```python
import jax
import jax.numpy as jnp

def _softmax(x, axis=-1):
    return jax.nn.softmax(x, axis=axis)

def _gelu(x):
    return jax.nn.gelu(x, approximate=True)

def _silu(x):
    return jax.nn.silu(x)

def _sigmoid(x):
    return jax.nn.sigmoid(x)

def _layernorm(x, axis=-1, eps=1e-05):
    m = jnp.mean(x, axis=axis, keepdims=True)
    v = jnp.var(x, axis=axis, keepdims=True)
    return (x - m) / jnp.sqrt(v + eps)

def _scatter_add(tgt, idx, src, axis=0):
    return tgt.at[idx].add(src)

def _segment_sum(src, seg, n):
    return jax.ops.segment_sum(src, seg, n)

class _Rng:

    def __init__(self, key):
        self._k = key

    def _next(self):
        self._k, sub = jax.random.split(self._k)
        return sub

    def normal(self, shape):
        return jax.random.normal(self._next(), shape, dtype=jnp.bfloat16)

    def randint(self, lo, hi, shape):
        return jax.random.randint(self._next(), shape, lo, hi, dtype=jnp.int32)

    def uniform(self, shape, lo=0.0, hi=1.0):
        return jax.random.uniform(self._next(), shape, jnp.bfloat16, lo, hi)

    def permutation(self, n):
        return jax.random.permutation(self._next(), n)
kernel_name = 'adaLN_cond__ssm_conv_h3__glu_gated_swiglu__prompt'

def setup_inputs():
    _rng = _Rng(jax.random.key(int.from_bytes(__import__("os").urandom(4), "little")))
    _w = lambda a: (lambda t: t.astype(jnp.bfloat16) if jnp.issubdtype(t.dtype, jnp.floating) else t)(jnp.asarray(a))

    def _A_setup():
        B, S, D = (1, 2048, 640)
        ks = 4
        return {'q': _w((lambda *s: _rng.normal(s) * 0.05)(B, S, D)), 'k': _w((lambda *s: _rng.normal(s) * 0.05)(B, S, D)), 'v': _w((lambda *s: _rng.normal(s) * 0.05)(B, S, D)), 'shift_k': _w((lambda *s: _rng.normal(s) * 0.05)(D, ks) * 0.5), 'ssm_k': _w((lambda *s: _rng.normal(s) * 0.05)(D, S) * (1.0 / S ** 0.5)), 'ssm_D': _w((lambda *s: _rng.normal(s) * 0.05)(D))}
    _A_in = _A_setup()

    def _B_setup():
        B, S, D, F = (1, 2048, 640, 1536)
        return {'x': _w((lambda *s: _rng.normal(s) * 0.05)(B, S, D)), 'w1': _w((lambda *s: _rng.normal(s) * 0.05)(D, F) * (2.0 / D) ** 0.5), 'w3': _w((lambda *s: _rng.normal(s) * 0.05)(D, F) * (2.0 / D) ** 0.5), 'w2': _w((lambda *s: _rng.normal(s) * 0.05)(F, D) * (2.0 / F) ** 0.5)}
    _B_in = _B_setup()
    return {'A_q': _A_in['q'], 'A_k': _A_in['k'], 'A_v': _A_in['v'], 'A_shift_k': _A_in['shift_k'], 'A_ssm_k': _A_in['ssm_k'], 'A_ssm_D': _A_in['ssm_D'], 'B_x': _B_in['x'], 'B_w1': _B_in['w1'], 'B_w3': _B_in['w3'], 'B_w2': _B_in['w2'], 'c': _w((lambda *s: _rng.normal(s) * 0.05)(1, 640)), 'w_mod': _w((lambda *s: _rng.normal(s) * 0.05)(640, 6 * 640) * 640 ** (-0.5))}

def reference(A_q, A_k, A_v, A_shift_k, A_ssm_k, A_ssm_D, B_x, B_w1, B_w3, B_w2, c, w_mod):

    def _A_ref(q, k, v, shift_k, ssm_k, ssm_D):
        B, S, D = q.shape
        ks = shift_k.shape[-1]
        k_pad = jnp.pad(k, ((0, 0), (ks - 1, 0), (0, 0)))
        k_shift = jnp.zeros_like(k)
        for t in range(ks):
            k_shift = k_shift + k_pad[:, t:t + S, :] * shift_k[:, ks - 1 - t][None, None, :]
        kv = k_shift * v
        L = 2 * S
        kv_pad = jnp.pad(kv, ((0, 0), (0, S), (0, 0)))
        kf_pad = jnp.pad(ssm_k, ((0, 0), (0, S)))
        kv_f = (lambda x, axes=(-2, -1): jnp.fft.rfft2(x.astype(jnp.float32), axes=axes))(kv_pad[:, None, :, :], axes=(1, 2))
        kf_f = (lambda x, axes=(-2, -1): jnp.fft.rfft2(x.astype(jnp.float32), axes=axes))(kf_pad[:, None, :], axes=(1, 2))
        kf_f = (lambda x, *d: x.transpose(*d))(kf_f, 1, 2, 0)
        y_f = kv_f * kf_f[None, :, :, :]
        y = (lambda x, s, axes=(-2, -1): jnp.fft.irfft2(x, s=s, axes=axes).astype(jnp.bfloat16))(y_f, (1, L), axes=(1, 2))[:, 0, :S, :]
        y = y + kv * ssm_D[None, None, :]
        return q * y

    def _B_ref(x, w1, w3, w2):
        gate = jnp.einsum('bsd,df->bsf', x, w1)
        up = jnp.einsum('bsd,df->bsf', x, w3)
        h = _silu(gate) * up
        out = jnp.einsum('bsf,fd->bsd', h, w2)
        return out
    x = A_q
    mod = (_silu(c) @ w_mod).reshape(c.shape[0], 6, 1, -1)
    sa, ca, ga, sb, cb, gb = (mod[:, 0].copy(), mod[:, 1].copy(), mod[:, 2].copy(), mod[:, 3].copy(), mod[:, 4].copy(), mod[:, 5].copy())
    h = _layernorm(x, axis=-1) * (1 + ca) + sa
    x = x + ga * _A_ref(h, A_k, A_v, A_shift_k, A_ssm_k, A_ssm_D)
    h = _layernorm(x, axis=-1) * (1 + cb) + sb
    x = x + gb * _B_ref(h, B_w1, B_w3, B_w2)
    return x
```

```python
import numpy as np

import jax
import jax.numpy as jnp
import jax.experimental.pallas as pl
import jax.experimental.pallas.tpu as pltpu

C = 128
R = 256
FB = 256
EPS = 1e-5

_F32 = jnp.float32
_BF16 = jnp.bfloat16
_NT = (((1,), (1,)), ((), ()))


def _dft_matrices():
    even = np.arange(0, C, 2)
    f = np.concatenate([even, C - 1 - even]).astype(np.float64)
    ang = 2.0 * np.pi * (f[:, None] + 0.5) * np.arange(C)[None, :] / (2 * C)
    fwd = np.concatenate([np.cos(ang), -np.sin(ang)], axis=0)
    inv = fwd.T / C
    return fwd.astype(np.float32), inv.astype(np.float32)


_FWD, _INV = _dft_matrices()


def _dot(a, b):
    return jnp.dot(a, b, preferred_element_type=_F32)


def _layernorm(x):
    inv_d = 1.0 / x.shape[-1]
    m = jnp.sum(x, axis=-1, keepdims=True) * inv_d
    xc = x - m
    v = jnp.sum(xc * xc, axis=-1, keepdims=True) * inv_d
    return xc * jax.lax.rsqrt(v + EPS)


def _silu(x):
    return x * jax.nn.sigmoid(x)


def _interleave(main, side):
    done = 0
    for i, step in enumerate(main):
        step()
        upto = (len(side) * (i + 1)) // len(main)
        for k in range(done, upto):
            side[k]()
        done = upto


def _kernel(q_hbm, k_hbm, v_hbm, shift_hbm, sk_hbm, d_hbm, w1_hbm, w3_hbm, w2_hbm,
            c_hbm, wm_hbm, fwd_hbm, inv_hbm, out_hbm,
            q_v, k_v, v_v, shift_v, sk_v, d_v, w1_v, w3_v, w2_v, c_v, wm_v, fwd_v, inv_v,
            u_s, kf_s, kraw_s, z_s, mod_s, x1_s, h2_s, act_s, out_v,
            in_sems, out_sems):
    S, D = q_hbm.shape
    FH = w1_hbm.shape[1]
    NB = S // R
    CPB = R // C
    NF = FH // FB
    H = C // 2

    copies = {}

    def start(name, src, dst):
        cp = pltpu.make_async_copy(src, dst, in_sems.at[len(copies)])
        cp.start()
        copies[name] = cp

    def wait(*names):
        for name in names:
            copies[name].wait()

    def start_block(b):
        rows = pl.ds(b * R, R)
        start(("sk", b), sk_hbm.at[:, rows], sk_v.at[:, rows])
        start(("k", b), k_hbm.at[rows, :], k_v.at[rows, :])
        start(("v", b), v_hbm.at[rows, :], v_v.at[rows, :])
        start(("q", b), q_hbm.at[rows, :], q_v.at[rows, :])

    start("fwd", fwd_hbm, fwd_v)
    start("shift", shift_hbm, shift_v)
    start("d", d_hbm, d_v)
    start("c", c_hbm, c_v)
    start("inv", inv_hbm, inv_v)
    start_block(0)
    for j in range(5):
        cols = pl.ds(j * D, D)
        start(("wm", j), wm_hbm.at[:, cols], wm_v.at[:, cols])
    for f in range(NF):
        cols = pl.ds(f * FB, FB)
        start(("w1", f), w1_hbm.at[:, cols], w1_v.at[:, cols])
        start(("w3", f), w3_hbm.at[:, cols], w3_v.at[:, cols])
    start_block(1)
    start("w2", w2_hbm, w2_v)
    start(("wm", 5), wm_hbm.at[:, pl.ds(5 * D, D)], wm_v.at[:, pl.ds(5 * D, D)])
    for b in range(2, NB):
        start_block(b)

    def mod(j):
        return mod_s[0:1, j * D:(j + 1) * D]

    def compute_mod(j):
        wait(("wm", j))
        sc = _silu(c_v[...].astype(_F32)).astype(_BF16)
        sc = jnp.broadcast_to(sc, (16, D))
        mod_s[:, j * D:(j + 1) * D] = _dot(sc, wm_v[:, j * D:(j + 1) * D])[0:8]

    def ssm_transform(m):
        raw = jax.lax.dot_general(fwd_v[...], sk_v[:, m * C:(m + 1) * C], _NT,
                                  preferred_element_type=_F32)
        if m == 0:
            kf_s[0, 0:C] = raw[0:C] + d_v[...].astype(_F32)
            kf_s[0, C:2 * C] = raw[C:2 * C]
        else:
            kf_s[m, 0:H] = raw[0:H] - kraw_s[C:C + H]
            kf_s[m, H:C] = raw[H:C] + kraw_s[C + H:2 * C]
            kf_s[m, C:C + H] = raw[C:C + H] + kraw_s[0:H]
            kf_s[m, C + H:2 * C] = raw[C + H:2 * C] - kraw_s[H:C]
        if m + 1 < S // C:
            kraw_s[...] = raw

    def kv_transform(i):
        r0 = i * C
        if i == 0:
            kk = jnp.concatenate(
                [jnp.zeros((16, D), _F32), k_v[0:C, :].astype(_F32)], axis=0)
        else:
            kk = k_v[r0 - 16:r0 + C, :].astype(_F32)
        w = shift_v[...].astype(_F32)
        ks = kk[16:16 + C] * w[0:1]
        for j in range(1, w.shape[0]):
            ks = ks + kk[16 - j:16 - j + C] * w[j:j + 1]
        kv = (ks * v_v[r0:r0 + C, :].astype(_F32)).astype(_BF16)
        u_s[i] = _dot(fwd_v[...], kv)

    def mac(b, g):
        chunks = range(b * CPB, (b + 1) * CPB)
        halves = []
        for half in range(2):
            re = slice(16 * g + 8 * half, 16 * g + 8 * half + 8)
            im = slice(C + re.start, C + re.stop)
            acc = {}
            for i in range(chunks[-1] + 1):
                ur, ui = u_s[i, re], u_s[i, im]
                for j in chunks:
                    if j < i:
                        continue
                    kr, ki = kf_s[j - i, re], kf_s[j - i, im]
                    pr = kr * ur - ki * ui
                    pi = kr * ui + ki * ur
                    acc[j] = (pr, pi) if j not in acc else (acc[j][0] + pr, acc[j][1] + pi)
            halves.append(acc)
        for j in chunks:
            for part in range(2):
                z = jnp.concatenate([halves[0][j][part], halves[1][j][part]], axis=0)
                z_s[j % CPB, part * C + 16 * g:part * C + 16 * g + 16] = z.astype(_BF16)

    def pre_ffn(b, jj):
        slot = b % 2
        r0 = b * R + jj * C
        y = _dot(inv_v[...], z_s[jj])
        x = q_v[r0:r0 + C, :].astype(_F32)
        h = _layernorm(x) * (1.0 + mod(1)) + mod(0)
        x1 = x + mod(2) * (h * y)
        h2 = _layernorm(x1) * (1.0 + mod(4)) + mod(3)
        x1_s[slot, jj * C:(jj + 1) * C] = x1
        h2_s[slot, jj * C:(jj + 1) * C] = h2.astype(_BF16)

    def ffn_up(b, f):
        if b == 0:
            wait(("w1", f), ("w3", f))
        h2 = h2_s[b % 2]
        cols = slice(f * FB, (f + 1) * FB)
        gate = _dot(h2, w1_v[:, cols])
        up = _dot(h2, w3_v[:, cols])
        act_s[:, cols] = (_silu(gate) * up).astype(_BF16)

    out_copies = []

    def ffn_down(b):
        if b == 0:
            wait("w2")
            compute_mod(5)
        rows = pl.ds(b * R, R)
        o = _dot(act_s[...], w2_v[...])
        out_v[rows, :] = (x1_s[b % 2] + mod(5) * o).astype(_BF16)
        cp = pltpu.make_async_copy(out_v.at[rows, :], out_hbm.at[rows, :], out_sems.at[b])
        cp.start()
        out_copies.append(cp)

    def conv_steps(b):
        steps = [lambda: wait(("sk", b))]
        steps += [lambda m=m: ssm_transform(m) for m in range(b * CPB, (b + 1) * CPB)]
        steps += [lambda: wait(("k", b), ("v", b))]
        steps += [lambda i=i: kv_transform(i) for i in range(b * CPB, (b + 1) * CPB)]
        steps += [lambda g=g: mac(b, g) for g in range(C // 16)]
        return steps

    def pre_steps(b):
        return [lambda: wait(("q", b))] + [lambda jj=jj: pre_ffn(b, jj) for jj in range(CPB)]

    def ffn_steps(b):
        return [lambda f=f: ffn_up(b, f) for f in range(NF)] + [lambda: ffn_down(b)]

    wait("fwd", "shift", "d")
    for step in conv_steps(0):
        step()
    wait("c", "inv")
    for j in range(5):
        compute_mod(j)
    for step in pre_steps(0):
        step()
    for b in range(NB):
        side = conv_steps(b + 1) + pre_steps(b + 1) if b + 1 < NB else []
        _interleave(ffn_steps(b), side)
    for cp in out_copies:
        cp.wait()


@jax.jit
def pallas_adaLN_cond__ssm_conv_h3__glu_gated_swiglu__prompt_kernel(
    A_q: jax.Array,
    A_k: jax.Array,
    A_v: jax.Array,
    A_shift_k: jax.Array,
    A_ssm_k: jax.Array,
    A_ssm_D: jax.Array,
    B_x: jax.Array,
    B_w1: jax.Array,
    B_w3: jax.Array,
    B_w2: jax.Array,
    c: jax.Array,
    w_mod: jax.Array,
):
    del B_x
    B, S, D = A_q.shape
    FH = B_w1.shape[1]
    KS = A_shift_k.shape[1]
    assert B == 1 and S % R == 0 and FH % FB == 0 and KS <= 16
    NB, NC = S // R, S // C
    n_in = 5 + 4 * NB + 6 + 2 * (FH // FB) + 1

    hbm = pl.BlockSpec(memory_space=pl.ANY)
    out = pl.pallas_call(
        _kernel,
        out_shape=jax.ShapeDtypeStruct((S, D), A_q.dtype),
        in_specs=[hbm] * 13,
        out_specs=hbm,
        scratch_shapes=[
            pltpu.VMEM((S, D), _BF16),
            pltpu.VMEM((S, D), _BF16),
            pltpu.VMEM((S, D), _BF16),
            pltpu.VMEM((KS, D), _BF16),
            pltpu.VMEM((D, S), _BF16),
            pltpu.VMEM((1, D), _BF16),
            pltpu.VMEM((D, FH), _BF16),
            pltpu.VMEM((D, FH), _BF16),
            pltpu.VMEM((FH, D), _BF16),
            pltpu.VMEM((1, D), _BF16),
            pltpu.VMEM((D, 6 * D), _BF16),
            pltpu.VMEM((2 * C, C), _BF16),
            pltpu.VMEM((C, 2 * C), _BF16),
            pltpu.VMEM((NC, 2 * C, D), _F32),
            pltpu.VMEM((NC, 2 * C, D), _F32),
            pltpu.VMEM((2 * C, D), _F32),
            pltpu.VMEM((R // C, 2 * C, D), _BF16),
            pltpu.VMEM((8, 6 * D), _F32),
            pltpu.VMEM((2, R, D), _F32),
            pltpu.VMEM((2, R, D), _BF16),
            pltpu.VMEM((R, FH), _BF16),
            pltpu.VMEM((S, D), _BF16),
            pltpu.SemaphoreType.DMA((n_in,)),
            pltpu.SemaphoreType.DMA((NB,)),
        ],
        compiler_params=pltpu.CompilerParams(vmem_limit_bytes=100 * 1024 * 1024),
    )(
        A_q.reshape(S, D), A_k.reshape(S, D), A_v.reshape(S, D),
        A_shift_k.T, A_ssm_k, A_ssm_D.reshape(1, D),
        B_w1, B_w3, B_w2, c, w_mod,
        jnp.asarray(_FWD, _BF16), jnp.asarray(_INV, _BF16),
    )
    return out.reshape(B, S, D)
```

```python
import numpy as np

import jax
import jax.numpy as jnp
import jax.experimental.pallas as pl
import jax.experimental.pallas.tpu as pltpu

C = 128
R = 256
L = 128
WG = 2
RP = 32
RN = 32
MAC_LAG = 4
NORM0, NORM_STRIDE, NORM_SPAN = 0, 5, 4
MR, ML = 16, 128
NPRO = 4
MPRO = 3
CONV_AT = {2: 4, 3: 5, 4: 6, 5: 7}
MAC_AT = {0: [(3, 0, 20)], 1: [(3, 20, 40)], 2: [(4, 0, 40)], 3: [(5, 0, 40)],
          4: [(6, 0, 40)], 5: [(7, 0, 40)]}
W2_GROUPS = ((0, 2), (2, 5))
TIE = 'zth'
KT = 4
EPS = 1e-5

_F32 = jnp.float32
_BF16 = jnp.bfloat16
_NT = (((1,), (1,)), ((), ()))


def _dft_matrices():
    even = np.arange(0, C, 2)
    f = np.concatenate([even, C - 1 - even]).astype(np.float64)
    ang = 2.0 * np.pi * (f[:, None] + 0.5) * np.arange(C)[None, :] / (2 * C)
    fwd = np.concatenate([np.cos(ang), -np.sin(ang)], axis=0)
    inv = fwd.T / C
    return fwd.astype(np.float32), inv.astype(np.float32)


_FWD, _INV = _dft_matrices()


def _dot(a, b):
    return jnp.dot(a, b, preferred_element_type=_F32)


def _row_mean(x):
    m = jnp.sum(x, axis=-1, keepdims=True) * (1.0 / x.shape[-1])
    return jnp.broadcast_to(m, (x.shape[0], 128))


def _silu(x):
    hx = 0.5 * x
    return hx * jnp.tanh(hx) + hx


def _spread(slots, steps, first, last):
    for k, step in enumerate(steps):
        slots[first + (k * (last - first)) // len(steps)].append(step)


def _fill(slots, sizes, steps, first):
    held = [sum(cost for _, cost in slot) for slot in slots]
    rate = (sum(held[first:]) + sum(cost for _, cost in steps)) / sum(sizes[first:])
    budget, k = 0.0, 0
    for s in range(first, len(slots)):
        budget += rate * sizes[s] - held[s]
        while k < len(steps) and (budget >= 0.5 * steps[k][1] or s == len(slots) - 1):
            slots[s].append(steps[k])
            budget -= steps[k][1]
            k += 1


def _kernel(q_hbm, k_hbm, v_hbm, shift_hbm, sk_hbm, d_hbm, w1_hbm, w3_hbm, w2_hbm,
            c_hbm, wm_hbm, fwd_hbm, inv_hbm, base_hbm, out_hbm,
            q_v, k_v, v_v, shift_v, sk_v, d_v, w1_v, w3_v, w2_v, c_v, wm_v, fwd_v, inv_v, base_sm,
            kv_s, spec_s, kraw_s, z_s, y_s, mod_s, stat_s, x1_s, h2_s, w1_p, w3_p, w2_p, out_v,
            in_sems, out_sems):
    S, D = q_hbm.shape
    FH = w1_hbm.shape[1]
    NB = S // R
    NC = S // C
    CPB = R // C
    NF = FH // L
    ND = D // L
    H = C // 2

    copies = {}

    def start(name, src, dst):
        cp = pltpu.make_async_copy(src, dst, in_sems.at[len(copies)])
        cp.start()
        copies[name] = cp

    def wait(*names):
        for name in names:
            copies[name].wait()

    def start_conv(b):
        rows = pl.ds(b * R, R)
        start(("sk", b), sk_hbm.at[:, rows], sk_v.at[:, rows])
        start(("k", b), k_hbm.at[rows, :], k_v.at[rows, :])
        start(("v", b), v_hbm.at[rows, :], v_v.at[rows, :])

    def wait_conv(b):
        wait(("sk", b), ("k", b), ("v", b))

    def start_q(b):
        rows = pl.ds(b * R, R)
        start(("q", b), q_hbm.at[rows, :], q_v.at[rows, :])

    start("base", base_hbm, base_sm)
    start("fwd", fwd_hbm, fwd_v)
    start("shift", shift_hbm, shift_v)
    start("d", d_hbm, d_v)
    start("c", c_hbm, c_v)
    start("inv", inv_hbm, inv_v)
    def start_mod(j):
        start(("wm", j), wm_hbm.at[:, pl.ds(j * D, D)], wm_v.at[j])

    start_conv(0)
    start_q(0)
    for b in range(1, NPRO):
        start_conv(b)
    for j in (1, 0, 2, 4, 3):
        start_mod(j)
    for g in range(NF // WG):
        cols = pl.ds(g * WG * L, WG * L)
        start(("w1", g), w1_hbm.at[:, cols], w1_v.at[:, cols])
        start(("w3", g), w3_hbm.at[:, cols], w3_v.at[:, cols])
        if g == 0:
            start_q(1)
    for n0, n1 in W2_GROUPS:
        cols = pl.ds(n0 * L, (n1 - n0) * L)
        start(("w2", n0), w2_hbm.at[:, cols], w2_v.at[:, cols])
    start_mod(5)
    for b in range(2, NB):
        start_q(b)
        if b >= NPRO:
            start_conv(b)

    wait("base")
    base = base_sm[0]

    z_s[NC, 0:8, 0:L] = jnp.zeros((8, 128), _F32)
    x1_s[2, 0:8, 0:128] = jnp.zeros((8, 128), _F32)
    stat_s[4, 0:8] = jnp.zeros((8, L), _F32)
    h2_s[2, 0:16, 0:L] = jnp.zeros((16, L), _BF16)

    def mod(j):
        return mod_s[0:1, j * D:(j + 1) * D]

    def compute_mod(j):
        wait(("wm", j))
        sc = _silu(c_v[...].astype(_F32)).astype(_BF16)
        sc = jnp.broadcast_to(sc, (16, D))
        mod_s[:, j * D:(j + 1) * D] = _dot(sc, wm_v[j])[0:8]

    def ssm_transform(m):
        raw = jax.lax.dot_general(fwd_v[...], sk_v[:, m * C:(m + 1) * C], _NT,
                                  preferred_element_type=_F32)
        if m == 0:
            spec_s[NC, 0:C] = raw[0:C] + d_v[...].astype(_F32).reshape(1, D)
            spec_s[NC, C:2 * C] = raw[C:2 * C]
        else:
            spec_s[NC + m, 0:H] = raw[0:H] - kraw_s[base, C:C + H]
            spec_s[NC + m, H:C] = raw[H:C] + kraw_s[base, C + H:2 * C]
            spec_s[NC + m, C:C + H] = raw[C:C + H] + kraw_s[base, 0:H]
            spec_s[NC + m, C + H:2 * C] = raw[C + H:2 * C] - kraw_s[base, H:C]
        if m + 1 < S // C:
            kraw_s[0] = raw

    def short_conv(i, p):
        r0 = i * C + p * RP
        if r0 == 0:
            kk = jnp.concatenate(
                [jnp.zeros((16, D), _F32), k_v[0:RP, :].astype(_F32)], axis=0)
        else:
            kk = k_v[r0 - 16:r0 + RP, :].astype(_F32)
        w = shift_v[...].astype(_F32)
        ks = kk[16:16 + RP] * w[0:1]
        for j in range(1, w.shape[0]):
            ks = ks + kk[16 - j:16 - j + RP] * w[j:j + 1]
        kv_s[i % CPB, p * RP:(p + 1) * RP] = (ks * v_v[r0:r0 + RP, :].astype(_F32)).astype(_BF16)

    def kv_transform(i):
        spec_s[i] = _dot(fwd_v[...], kv_s[i % CPB])

    def mac(b, g, n):
        chunks = range(b * CPB, (b + 1) * CPB)
        re = slice(MR * g, MR * (g + 1))
        im = slice(C + re.start, C + re.stop)
        ln = slice(n * ML, min(D, (n + 1) * ML))
        acc = {}
        kf = {}
        for i in range(chunks[-1] + 1):
            ur, ui = spec_s[base + i, re, ln], spec_s[base + i, im, ln]
            for j in chunks:
                if j < i:
                    continue
                if j - i not in kf:
                    kf[j - i] = (spec_s[base + (NC + j - i), re, ln], spec_s[base + (NC + j - i), im, ln])
                kr, ki = kf[j - i]
                if j not in acc:
                    acc[j] = (kr * ur - ki * ui, kr * ui + ki * ur)
                else:
                    acc[j] = (acc[j][0] + (kr * ur - ki * ui), acc[j][1] + (kr * ui + ki * ur))
        for j in chunks:
            z_s[j, re, ln] = acc[j][0]
            z_s[j, im, ln] = acc[j][1]

    def inverse_transform(b, jj):
        z = z_s[base + (b * CPB + jj)]
        r0 = b * R + jj * C
        y_s[0, r0:r0 + C] = _dot(inv_v[...], z.astype(_BF16))

    def stat(k, rows):
        return jnp.tile(stat_s[base + k, rows], (1, D // 128))

    def q_rows(b, rows):
        return q_v[b * R + rows.start:b * R + rows.stop, :].astype(_F32)

    def norm1_mean(b, rows):
        stat_s[0, rows] = _row_mean(q_rows(b, rows))

    def norm1_scale(b, rows):
        xc = q_rows(b, rows) - stat(0, rows)
        stat_s[1, rows] = jax.lax.rsqrt(_row_mean(xc * xc) + EPS)

    def residual(b, rows):
        x = q_rows(b, rows)
        y = y_s[base, b * R + rows.start:b * R + rows.stop]
        h = (x - stat(0, rows)) * stat(1, rows) * (1.0 + mod(1)) + mod(0)
        x1 = x + mod(2) * (h * y)
        x1_s[b % 2, rows] = x1
        stat_s[2, rows] = _row_mean(x1)

    def norm2_scale(b, rows):
        xc = x1_s[base + b % 2, rows] - stat(2, rows)
        stat_s[3, rows] = jax.lax.rsqrt(_row_mean(xc * xc) + EPS)

    def norm2_apply(b, rows):
        xc = x1_s[base + b % 2, rows] - stat(2, rows)
        h2 = xc * stat(3, rows) * (1.0 + mod(4)) + mod(3)
        h2_s[b % 2, rows] = h2.astype(_BF16)

    def tied(lhs):
        zero = None
        for key, ref, slot in (('z', z_s, NC), ('x', x1_s, 2), ('t', stat_s, 4), ('h', h2_s, 2)):
            if key in TIE:
                w = pltpu.bitcast(ref[base + slot, 0:32 // ref.dtype.itemsize, 0:L], jnp.uint32)
                zero = w if zero is None else zero | w
        if zero is None:
            return lhs
        tile = pltpu.bitcast(pltpu.bitcast(lhs[0:16, 0:L], jnp.uint32) | zero, _BF16)
        top = jnp.concatenate([tile, lhs[0:16, L:]], axis=1)
        return jnp.concatenate([top, lhs[16:]], axis=0)

    def weight(b, raw, packed, tile, rows):
        words = slice(rows.start // 2, rows.stop // 2)
        if b == 0:
            w = raw[rows, tile * L:(tile + 1) * L]
            packed[tile, words] = pltpu.bitcast(w, jnp.uint32)
            return w
        return pltpu.bitcast(packed[base + tile, words], _BF16)

    live = {}

    def ffn_gate(b, f):
        if b == 0 and f % WG == 0:
            wait(("w1", f // WG), ("w3", f // WG))
            if f == 0:
                wait(("q", 1))
        live["gate"] = _dot(tied(h2_s[b % 2]), weight(b, w1_v, w1_p, f, slice(0, D)))

    def ffn_up(b, f):
        up = _dot(tied(h2_s[b % 2]), weight(b, w3_v, w3_p, f, slice(0, D)))
        live["act", f] = (_silu(live.pop("gate")) * up).astype(_BF16)

    out_copies = []

    def write_out(b, n, o):
        rows = pl.ds(b * R, R)
        cols = slice(n * L, (n + 1) * L)
        out_v[rows, cols] = (x1_s[base + b % 2, :, cols] + mod(5)[:, cols] * o).astype(_BF16)
        if n + 1 == ND:
            cp = pltpu.make_async_copy(out_v.at[rows, :], out_hbm.at[rows, :], out_sems.at[b])
            cp.start()
            out_copies.append(cp)

    def ffn_down(b, n, kk):
        if b == 0 and kk == 0 and n in dict(W2_GROUPS):
            wait(("w2", n))
        act = jnp.concatenate([live["act", kk * KT + j] for j in range(KT)], axis=1)
        o = _dot(tied(act), weight(b, w2_v, w2_p, n, slice(kk * KT * L, (kk + 1) * KT * L)))
        if kk > 0:
            o = live.pop(("out", n)) + o
        if kk + 1 < NF // KT or b == 0:
            live["out", n] = o
        else:
            write_out(b, n, o)

    def ffn_steps(b):
        steps = []
        for f in range(NF):
            steps += [lambda f=f: ffn_gate(b, f), lambda f=f: ffn_up(b, f)]
        steps += [lambda n=n, kk=kk: ffn_down(b, n, kk)
                  for n in range(ND) for kk in range(NF // KT)]
        return steps

    def short_conv_steps(i):
        return [(lambda p=p: short_conv(i, p), 17 * RP * ND // 8) for p in range(C // RP)]

    def mac_steps(b):
        cost = sum(j + 1 for j in range(b * CPB, (b + 1) * CPB)) * MR * ML // 128
        return [(lambda g=g, n=n: mac(b, g, n), cost)
                for g in range(C // MR) for n in range(D // ML)]

    def norm_passes(b):
        return [[(lambda p=p, fn=fn: fn(b, slice(p * RN, (p + 1) * RN)), ops * RN * ND // 8)
                 for p in range(R // RN)]
                for fn, ops in ((norm1_mean, 2), (norm1_scale, 5), (residual, 9),
                                (norm2_scale, 4), (norm2_apply, 5))]

    def conv_steps(slots, b, first):
        for jj in range(CPB):
            i = b * CPB + jj
            s0 = first + 2 * jj
            slots[s0].append((lambda i=i: ssm_transform(i), 0))
            _spread(slots, short_conv_steps(i), s0, s0 + 2)
            slots[s0 + 3].append((lambda i=i: kv_transform(i), 0))

    def pipeline_step(b):
        main = ffn_steps(b)
        sizes = [ND] * (2 * NF) + [KT] * (len(main) - 2 * NF)
        slots = [[] for _ in main]
        if b == 1:
            for n in range(ND):
                slots[n].append((lambda n=n: write_out(0, n, live.pop(("out", n))), 3 * R // 8))
        if b + 1 < NB:
            for jj in range(CPB):
                slots[jj].append((lambda jj=jj: inverse_transform(b + 1, jj), 0))
            for k, steps in enumerate(norm_passes(b + 1)):
                _spread(slots, steps, NORM0 + k * NORM_STRIDE, NORM0 + k * NORM_STRIDE + NORM_SPAN)
        if b in CONV_AT:
            conv_steps(slots, CONV_AT[b], 0)
        macs = [step for blk, lo, hi in MAC_AT.get(b, ()) for step in mac_steps(blk)[lo:hi]]
        if macs:
            fresh = MAC_AT[b][0][0] == CONV_AT.get(b)
            _fill(slots, sizes, macs, 2 * CPB + MAC_LAG if fresh else 0)
        for step, side in zip(main, slots):
            step()
            for extra, _ in side:
                extra()

    wait("fwd", "shift", "d", "c", "inv")
    norm0 = norm_passes(0)
    for b in range(NPRO):
        wait_conv(b)
        slots = [[] for _ in range(2 * CPB + 2)]
        conv_steps(slots, b, 0)
        for step, _ in sum(slots, []) + (mac_steps(b) if b < MPRO else []):
            step()
        if b == 0:
            wait(("q", 0))
            for jj in range(CPB):
                inverse_transform(b, jj)
            for step, _ in norm0[0] + norm0[1]:
                step()
    for j in (1, 0, 2):
        compute_mod(j)
    for step, _ in norm0[2] + norm0[3]:
        step()
    for j in (4, 3):
        compute_mod(j)
    for step, _ in norm0[4]:
        step()
    for b in range(NB):
        if b == 1:
            compute_mod(5)
        if 1 <= b < NB - 1:
            wait(("q", b + 1))
        if b in CONV_AT:
            wait_conv(CONV_AT[b])
        pipeline_step(b)
    for cp in out_copies:
        cp.wait()


@jax.jit
def pallas_adaLN_cond__ssm_conv_h3__glu_gated_swiglu__prompt_kernel(
    A_q: jax.Array,
    A_k: jax.Array,
    A_v: jax.Array,
    A_shift_k: jax.Array,
    A_ssm_k: jax.Array,
    A_ssm_D: jax.Array,
    B_x: jax.Array,
    B_w1: jax.Array,
    B_w3: jax.Array,
    B_w2: jax.Array,
    c: jax.Array,
    w_mod: jax.Array,
):
    del B_x
    B, S, D = A_q.shape
    FH = B_w1.shape[1]
    KS = A_shift_k.shape[1]
    assert B == 1 and S % R == 0 and FH % (KT * L) == 0 and D % L == 0 and KS <= 16
    NB, NC = S // R, S // C
    NF, ND = FH // L, D // L
    n_in = 6 + 4 * NB + 6 + 2 * (NF // WG) + len(W2_GROUPS)

    hbm = pl.BlockSpec(memory_space=pl.ANY)
    out = pl.pallas_call(
        _kernel,
        out_shape=jax.ShapeDtypeStruct((S, D), A_q.dtype),
        in_specs=[hbm] * 14,
        out_specs=hbm,
        scratch_shapes=[
            pltpu.VMEM((S, D), _BF16),
            pltpu.VMEM((S, D), _BF16),
            pltpu.VMEM((S, D), _BF16),
            pltpu.VMEM((KS, D), _BF16),
            pltpu.VMEM((D, S), _BF16),
            pltpu.VMEM((D,), _BF16),
            pltpu.VMEM((D, FH), _BF16),
            pltpu.VMEM((D, FH), _BF16),
            pltpu.VMEM((FH, D), _BF16),
            pltpu.VMEM((1, D), _BF16),
            pltpu.VMEM((6, D, D), _BF16),
            pltpu.VMEM((2 * C, C), _BF16),
            pltpu.VMEM((C, 2 * C), _BF16),
            pltpu.SMEM((1,), jnp.int32),
            pltpu.VMEM((R // C, C, D), _BF16),
            pltpu.VMEM((2 * NC, 2 * C, D), _F32),
            pltpu.VMEM((1, 2 * C, D), _F32),
            pltpu.VMEM((NC + 1, 2 * C, D), _F32),
            pltpu.VMEM((1, S, D), _F32),
            pltpu.VMEM((8, 6 * D), _F32),
            pltpu.VMEM((5, R, 128), _F32),
            pltpu.VMEM((3, R, D), _F32),
            pltpu.VMEM((3, R, D), _BF16),
            pltpu.VMEM((NF, D // 2, L), jnp.uint32),
            pltpu.VMEM((NF, D // 2, L), jnp.uint32),
            pltpu.VMEM((ND, FH // 2, L), jnp.uint32),
            pltpu.VMEM((S, D), _BF16),
            pltpu.SemaphoreType.DMA((n_in,)),
            pltpu.SemaphoreType.DMA((NB,)),
        ],
        compiler_params=pltpu.CompilerParams(vmem_limit_bytes=112 * 1024 * 1024),
    )(
        A_q.reshape(S, D), A_k.reshape(S, D), A_v.reshape(S, D),
        A_shift_k.T, A_ssm_k, A_ssm_D,
        B_w1, B_w3, B_w2, c, w_mod,
        jnp.asarray(_FWD, _BF16), jnp.asarray(_INV, _BF16), np.zeros((1,), np.int32),
    )
    return out.reshape(B, S, D)
```

```python
import numpy as np

import jax
import jax.numpy as jnp
import jax.experimental.pallas as pl
import jax.experimental.pallas.tpu as pltpu

C = 128
R = 256
L = 128
WG = 2
HALO = 8
RW = 128
RP = 32
PPRO = 1
RN = 32
MAC_LAG = 3
MARK_LAG = 3
INV0 = 0
SC0, SC1 = 14, 24
NORM_AT = ((0, 3), (2, 5), (5, 9), (8, 11), (11, 14))
XFORM_AT = (3, 5, 11, 12)
MR, ML = 16, 128
NPRO = 4
MPRO = 4
CONV_AT = {2: 4, 3: 5, 4: 6, 5: 7}
MAC_AT = {2: [(4, 0, 40)], 3: [(5, 0, 40)],
          4: [(6, 0, 40)], 5: [(7, 0, 40)]}
SEND_AT = (1, 2, 3, 4, 5, 6, 7)
W2_GROUPS = ((0, 2), (2, 5))
KT = 4
EPS = 1e-5

_F32 = jnp.float32
_BF16 = jnp.bfloat16
_NT = (((1,), (1,)), ((), ()))


def _dft_matrices():
    even = np.arange(0, C, 2)
    f = np.concatenate([even, C - 1 - even]).astype(np.float64)
    ang = 2.0 * np.pi * (f[:, None] + 0.5) * np.arange(C)[None, :] / (2 * C)
    fwd = np.concatenate([np.cos(ang), -np.sin(ang)], axis=0)
    inv = fwd.T / C
    return fwd.astype(np.float32), inv.astype(np.float32)


_FWD, _INV = _dft_matrices()


def _dot(a, b):
    return jnp.dot(a, b, preferred_element_type=_F32)


def _row_mean(x, zero=None):
    acc = x[:, 0:L] if zero is None else x[:, 0:L] + zero
    for n in range(1, x.shape[1] // L):
        acc = acc + x[:, n * L:(n + 1) * L]
    m = jnp.sum(acc, axis=-1, keepdims=True) * (1.0 / x.shape[1])
    return jnp.broadcast_to(m, (x.shape[0], L))


def _silu(x):
    hx = 0.5 * x
    return hx * jnp.tanh(hx) + hx


def _spread(slots, steps, first, last):
    for k, step in enumerate(steps):
        slots[first + (k * (last - first)) // len(steps)].append(step)


def _fill(slots, sizes, steps, first):
    held = [sum(cost for _, cost in slot) for slot in slots]
    rate = (sum(held[first:]) + sum(cost for _, cost in steps)) / sum(sizes[first:])
    budget, k = 0.0, 0
    for s in range(first, len(slots)):
        budget += rate * sizes[s] - held[s]
        while k < len(steps) and (budget >= 0.5 * steps[k][1] or s == len(slots) - 1):
            slots[s].append(steps[k])
            budget -= steps[k][1]
            k += 1


def _kernel(q_hbm, k_hbm, v_hbm, shift_hbm, sk_hbm, d_hbm, w1_hbm, w3_hbm, w2_hbm,
            c_hbm, wm_hbm, fwd_hbm, inv_hbm, base_hbm, out_hbm,
            q_v, k_v, v_v, shift_v, sk_v, d_v, w1_v, w3_v, w2_v, c_v, wm_v, fwd_v, inv_v, base_sm,
            k_s, kv_s, spec_s, kraw_s, z_s, y_s, mod_s, stat_s, mark_s, x1_s, h2_s, w1_p, w3_p, w2_p, out_v,
            in_sems, out_sems):
    S, D = q_hbm.shape
    FH = w1_hbm.shape[1]
    NB = S // R
    NC = S // C
    CPB = R // C
    NF = FH // L
    ND = D // L
    H = C // 2

    copies = {}

    def start(name, src, dst):
        cp = pltpu.make_async_copy(src, dst, in_sems.at[len(copies)])
        cp.start()
        copies[name] = cp

    def wait(*names):
        for name in names:
            copies[name].wait()

    def start_ssm(b):
        cols = pl.ds(b * R, R)
        start(("sk", b), sk_hbm.at[:, cols], sk_v.at[:, cols])

    def start_kv(b):
        rows = pl.ds(b * R, R)
        start(("k", b), k_hbm.at[rows, :], k_v.at[rows, :])
        start(("v", b), v_hbm.at[rows, :], v_v.at[rows, :])

    def start_q(b):
        rows = pl.ds(b * R, R)
        start(("q", b), q_hbm.at[rows, :], q_v.at[rows, :])

    start("base", base_hbm, base_sm)
    start("fwd", fwd_hbm, fwd_v)
    start("shift", shift_hbm, shift_v)
    start("d", d_hbm, d_v)
    start("c", c_hbm, c_v)
    start("inv", inv_hbm, inv_v)
    def start_mod(j):
        start(("wm", j), wm_hbm.at[:, pl.ds(j * D, D)], wm_v.at[j])

    for b in range(NPRO):
        start_ssm(b)
        start_kv(b)
        if b == 1:
            for j in range(PPRO):
                start_q(j)
    for j in (1, 0, 2, 4, 3):
        start_mod(j)
    for g in range(NF // WG):
        cols = pl.ds(g * WG * L, WG * L)
        start(("w1", g), w1_hbm.at[:, cols], w1_v.at[:, cols])
        start(("w3", g), w3_hbm.at[:, cols], w3_v.at[:, cols])
        if g == 0 and PPRO < 2:
            start_q(1)
    for n0, n1 in W2_GROUPS:
        cols = pl.ds(n0 * L, (n1 - n0) * L)
        start(("w2", n0), w2_hbm.at[:, cols], w2_v.at[:, cols])
    start_mod(5)
    for b in range(1, NB - 1):
        start_q(b + 1)
        if b in CONV_AT:
            start_ssm(CONV_AT[b])
        if b + 1 in CONV_AT:
            start_kv(CONV_AT[b + 1])

    wait("base")
    base = base_sm[0]

    z_s[NC, 0:8, 0:L] = jnp.zeros((8, 128), _F32)
    for ref in stat_s:
        ref[1, 0:8] = jnp.zeros((8, L), _F32)
    for ref in h2_s:
        ref[1, 0:8, 0:L] = jnp.zeros((8, L), _F32)
    kv_s[NC, 0:8, 0:L] = jnp.zeros((8, L), _F32)
    k_s[:, 0:HALO] = jnp.zeros((ND, HALO, L), _F32)

    written = []

    def wrote(ref, slot):
        if not any(ref is r for r, _ in written):
            written.append((ref, slot))

    emitted = [0]

    def mark(result):
        mark_s[emitted[0] % len(mark_s)][0] = result[0:8, 0:L]
        emitted[0] += 1

    def after_mark(lag=MARK_LAG):
        return mark_s[(emitted[0] - 1 - lag) % len(mark_s)][base + 1, 0:1]

    for ref in mark_s:
        ref[1] = jnp.zeros((8, L), _F32)

    def mod(j):
        return mod_s[0:1, j * D:(j + 1) * D]

    def compute_mod(j):
        sc = _silu(c_v[...].astype(_F32)).astype(_BF16)
        sc = jnp.broadcast_to(sc, (16, D))
        mod_s[:, j * D:(j + 1) * D] = _dot(sc, wm_v[j])[0:8]

    def ssm_transform(m):
        raw = jax.lax.dot_general(fwd_v[...], sk_v[:, m * C:(m + 1) * C], _NT,
                                  preferred_element_type=_F32)
        prev = kraw_s[(m - 1) % 2]
        if m == 0:
            spec_s[NC, 0:C] = raw[0:C] + d_v[...].astype(_F32).reshape(1, D)
            spec_s[NC, C:2 * C] = raw[C:2 * C]
        else:
            spec_s[NC + m, 0:H] = raw[0:H] - prev[base, C:C + H]
            spec_s[NC + m, H:C] = raw[H:C] + prev[base, C + H:2 * C]
            spec_s[NC + m, C:C + H] = raw[C:C + H] + prev[base, 0:H]
            spec_s[NC + m, C + H:2 * C] = raw[C + H:2 * C] - prev[base, H:C]
        if m + 1 < S // C:
            kraw_s[m % 2][0] = raw

    def widen_k(r0):
        kk = k_v[r0:r0 + RW, :].astype(_F32) + jnp.tile(after_mark(), (1, ND))
        for n in range(ND):
            k_s[n, HALO + r0:HALO + r0 + RW] = kk[:, n * L:(n + 1) * L]

    def short_conv(i, p):
        r0 = i * C + p * RP
        w = shift_v[...].astype(_F32)
        ks = None
        for j in range(w.shape[0]):
            kj = jnp.concatenate([k_s[base + n, HALO + r0 - j:HALO + r0 - j + RP]
                                  for n in range(ND)], axis=1)
            ks = kj * w[j:j + 1] if ks is None else ks + kj * w[j:j + 1]
        kv_s[i, p * RP:(p + 1) * RP] = ks * v_v[r0:r0 + RP, :].astype(_F32)
        wrote(kv_s, NC)

    def kv_transform(i):
        spec_s[i] = _dot(fwd_v[...], kv_s[base + i].astype(_BF16))

    def mac(b, g, n):
        chunks = range(b * CPB, (b + 1) * CPB)
        re = slice(MR * g, MR * (g + 1))
        im = slice(C + re.start, C + re.stop)
        ln = slice(n * ML, min(D, (n + 1) * ML))
        acc = {}
        kf = {}
        for i in range(chunks[-1] + 1):
            ur, ui = spec_s[base + i, re, ln], spec_s[base + i, im, ln]
            for j in chunks:
                if j < i:
                    continue
                if j - i not in kf:
                    kf[j - i] = (spec_s[base + (NC + j - i), re, ln], spec_s[base + (NC + j - i), im, ln])
                kr, ki = kf[j - i]
                if j not in acc:
                    acc[j] = (kr * ur - ki * ui, kr * ui + ki * ur)
                else:
                    acc[j] = (acc[j][0] + (kr * ur - ki * ui), acc[j][1] + (kr * ui + ki * ur))
        for j in chunks:
            z_s[j, re, ln] = acc[j][0]
            z_s[j, im, ln] = acc[j][1]
        wrote(z_s, NC)

    def inverse_transform(b, jj):
        z = z_s[base + (b * CPB + jj)]
        r0 = b * R + jj * C
        y_s[0, r0:r0 + C] = _dot(inv_v[...], z.astype(_BF16))

    def stat(k, rows):
        s = stat_s[k][base, rows]
        return jnp.tile(s + after_mark() if k % 2 == 0 else s, (1, ND))

    def q_rows(b, rows):
        return q_v[b * R + rows.start:b * R + rows.stop, :].astype(_F32)

    def norm1_mean(b, rows):
        stat_s[0][0, rows] = _row_mean(q_rows(b, rows), after_mark())
        wrote(stat_s[0], 1)

    def norm1_scale(b, rows):
        xc = q_rows(b, rows) - stat(0, rows)
        stat_s[1][0, rows] = jax.lax.rsqrt(_row_mean(xc * xc) + EPS)
        wrote(stat_s[1], 1)

    def residual(b, rows):
        x = q_rows(b, rows)
        y = y_s[base, b * R + rows.start:b * R + rows.stop]
        h = (x - stat(0, rows)) * stat(1, rows) * (1.0 + mod(1)) + mod(0)
        x1 = x + mod(2) * (h * y)
        x1_s[b % 2, rows] = x1
        stat_s[2][0, rows] = _row_mean(x1)
        wrote(stat_s[2], 1)

    def norm2_scale(b, rows):
        xc = x1_s[base + b % 2, rows] - stat(2, rows)
        stat_s[3][0, rows] = jax.lax.rsqrt(_row_mean(xc * xc) + EPS)
        wrote(stat_s[3], 1)

    def norm2_apply(b, rows):
        xc = x1_s[base + b % 2, rows] - stat(2, rows)
        h2 = xc * stat(3, rows) * (1.0 + mod(4)) + mod(3)
        h2_s[b % 2][0, rows] = h2
        wrote(h2_s[b % 2], 1)

    def tied(lhs):
        zero = None
        for ref, slot in written:
            w = pltpu.bitcast(ref[base + slot, 0:8, 0:L], jnp.uint32)
            zero = w if zero is None else zero | w
        written.clear()
        if zero is None:
            return lhs
        tile = pltpu.bitcast(pltpu.bitcast(lhs[0:16, 0:L], jnp.uint32) | zero, _BF16)
        top = jnp.concatenate([tile, lhs[0:16, L:]], axis=1)
        return jnp.concatenate([top, lhs[16:]], axis=0)

    def weight(b, raw, packed, tile, rows):
        words = slice(rows.start // 2, rows.stop // 2)
        if b == 0:
            w = raw[rows, tile * L:(tile + 1) * L]
            packed[tile, words] = pltpu.bitcast(w, jnp.uint32)
            return w
        return pltpu.bitcast(packed[base + tile, words], _BF16)

    live = {}

    def ffn_gate(b, f):
        if f == 0:
            live["h2"] = h2_s[b % 2][base].astype(_BF16)
        if b == 0 and f % WG == 0:
            wait(("w1", f // WG), ("w3", f // WG))
            if f == 0 and PPRO < 2:
                wait(("q", 1))
        live["gate"] = _dot(tied(live["h2"]), weight(b, w1_v, w1_p, f, slice(0, D)))
        mark(live["gate"])

    def ffn_up(b, f):
        up = _dot(tied(live["h2"]), weight(b, w3_v, w3_p, f, slice(0, D)))
        mark(up)
        live["act", f] = (_silu(live.pop("gate")) * up).astype(_BF16)

    out_copies = []

    def write_out(b, n, o):
        rows = pl.ds(b * R, R)
        cols = slice(n * L, (n + 1) * L)
        out_v[rows, cols] = (x1_s[base + b % 2, :, cols] + mod(5)[:, cols] * o).astype(_BF16)

    def send_out(b):
        first = max([s + 1 for s in SEND_AT if s < b], default=0)
        rows = pl.ds(first * R, (b + 1 - first) * R)
        cp = pltpu.make_async_copy(out_v.at[rows, :], out_hbm.at[rows, :], out_sems.at[b])
        cp.start()
        out_copies.append(cp)

    def ffn_down(b, n, kk):
        if b == 0 and kk == 0 and n in dict(W2_GROUPS):
            wait(("w2", n))
        act = jnp.concatenate([live["act", kk * KT + j] for j in range(KT)], axis=1)
        o = _dot(tied(act), weight(b, w2_v, w2_p, n, slice(kk * KT * L, (kk + 1) * KT * L)))
        mark(o)
        if kk > 0:
            o = live.pop(("out", n)) + o
        if kk + 1 < NF // KT or b == 0:
            live["out", n] = o
        else:
            write_out(b, n, o)

    def ffn_steps(b):
        steps = []
        for f in range(NF):
            steps += [lambda f=f: ffn_gate(b, f), lambda f=f: ffn_up(b, f)]
        steps += [lambda n=n, kk=kk: ffn_down(b, n, kk)
                  for n in range(ND) for kk in range(NF // KT)]
        return steps

    def short_conv_steps(b):
        return ([(lambda r0=r0: widen_k(r0), 2 * RW * ND // 8)
                 for r0 in range(b * R, (b + 1) * R, RW)]
                + [(lambda i=i, p=p: short_conv(i, p), 9 * RP * ND // 8)
                   for i in range(b * CPB, (b + 1) * CPB) for p in range(C // RP)])

    def mac_steps(b):
        cost = sum(j + 1 for j in range(b * CPB, (b + 1) * CPB)) * MR * ML // 128
        return [(lambda g=g, n=n: mac(b, g, n), cost)
                for g in range(C // MR) for n in range(D // ML)]

    def norm_passes(b, rn=RN):
        return [[(lambda p=p, fn=fn: fn(b, slice(p * rn, (p + 1) * rn)), ops * rn * ND // 8)
                 for p in range(R // rn)]
                for fn, ops in ((norm1_mean, 2), (norm1_scale, 5), (residual, 9),
                                (norm2_scale, 4), (norm2_apply, 5))]

    def transform_steps(b):
        return [(lambda i=i, fn=fn: fn(i), 0)
                for fn in (ssm_transform, kv_transform) for i in range(b * CPB, (b + 1) * CPB)]

    def pipeline_step(b):
        main = ffn_steps(b)
        sizes = [ND] * (2 * NF) + [KT] * (len(main) - 2 * NF)
        slots = [[] for _ in main]
        if b == 1:
            for n in range(ND):
                slots[n].append((lambda n=n: write_out(0, n, live.pop(("out", n))), 3 * R // 8))
        if b in CONV_AT:
            for step, at in zip(transform_steps(CONV_AT[b]), XFORM_AT):
                slots[at].append(step)
        if PPRO <= b + 1 < NB:
            for jj in range(CPB):
                slots[INV0 + jj].append((lambda jj=jj: inverse_transform(b + 1, jj), 0))
            for steps, (first, stop) in zip(norm_passes(b + 1), NORM_AT):
                _spread(slots, steps, first, stop)
        if b + 1 in CONV_AT:
            _spread(slots, short_conv_steps(CONV_AT[b + 1]), SC0, SC1)
        macs = [step for blk, lo, hi in MAC_AT.get(b, ()) for step in mac_steps(blk)[lo:hi]]
        if macs:
            fresh = MAC_AT[b][0][0] == CONV_AT.get(b)
            _fill(slots, sizes, macs, XFORM_AT[-1] + MAC_LAG if fresh else 0)
        for step, side in zip(main, slots):
            step()
            for extra, _ in side:
                extra()
        if b in SEND_AT:
            send_out(b)

    def run(steps):
        for step, _ in steps:
            step()

    wait("fwd", "shift", "d", "c", "inv")
    early = [norm_passes(b, R) for b in range(PPRO)]
    last = max(NPRO + 1, MPRO + 2)
    for r in range(last):
        if r < NPRO:
            wait(("sk", r), ("k", r), ("v", r))
        if r == 1:
            wait(*[("q", b) for b in range(PPRO)])
        if r == last - 1:
            wait(("wm", 1), ("wm", 0), ("wm", 2))
            for j in (1, 0, 2):
                compute_mod(j)
            for passes in early:
                run(passes[2] + passes[3])
        if 1 <= r <= NPRO:
            run(transform_steps(r - 1))
        if 3 <= r < PPRO + 3:
            for jj in range(CPB):
                inverse_transform(r - 3, jj)
        if r == 1:
            for passes in early:
                run(passes[0] + passes[1])
        if r < NPRO + 1:
            run(short_conv_steps(r) if r < NPRO else [])
        if 2 <= r < MPRO + 2:
            run(mac_steps(r - 2))
    wait(("wm", 4), ("wm", 3))
    for j in (4, 3):
        compute_mod(j)
    for passes in early:
        run(passes[4])
    for b in range(NB):
        if 1 <= b < NB - 1:
            wait(("q", b + 1))
        if b in CONV_AT:
            wait(("sk", CONV_AT[b]))
        if b + 1 in CONV_AT:
            wait(("k", CONV_AT[b + 1]), ("v", CONV_AT[b + 1]))
        if b == 1:
            wait(("wm", 5))
            compute_mod(5)
        pipeline_step(b)
    for cp in out_copies:
        cp.wait()


@jax.jit
def pallas_adaLN_cond__ssm_conv_h3__glu_gated_swiglu__prompt_kernel(
    A_q: jax.Array,
    A_k: jax.Array,
    A_v: jax.Array,
    A_shift_k: jax.Array,
    A_ssm_k: jax.Array,
    A_ssm_D: jax.Array,
    B_x: jax.Array,
    B_w1: jax.Array,
    B_w3: jax.Array,
    B_w2: jax.Array,
    c: jax.Array,
    w_mod: jax.Array,
):
    del B_x
    B, S, D = A_q.shape
    FH = B_w1.shape[1]
    KS = A_shift_k.shape[1]
    assert B == 1 and S % R == 0 and FH % (KT * L) == 0 and D % L == 0 and KS <= HALO + 1
    NB, NC = S // R, S // C
    NF, ND = FH // L, D // L
    n_in = 6 + 4 * NB + 6 + 2 * (NF // WG) + len(W2_GROUPS)

    hbm = pl.BlockSpec(memory_space=pl.ANY)
    out = pl.pallas_call(
        _kernel,
        out_shape=jax.ShapeDtypeStruct((S, D), A_q.dtype),
        in_specs=[hbm] * 14,
        out_specs=hbm,
        scratch_shapes=[
            pltpu.VMEM((S, D), _BF16),
            pltpu.VMEM((S, D), _BF16),
            pltpu.VMEM((S, D), _BF16),
            pltpu.VMEM((KS, D), _BF16),
            pltpu.VMEM((D, S), _BF16),
            pltpu.VMEM((D,), _BF16),
            pltpu.VMEM((D, FH), _BF16),
            pltpu.VMEM((D, FH), _BF16),
            pltpu.VMEM((FH, D), _BF16),
            pltpu.VMEM((1, D), _BF16),
            pltpu.VMEM((6, D, D), _BF16),
            pltpu.VMEM((2 * C, C), _BF16),
            pltpu.VMEM((C, 2 * C), _BF16),
            pltpu.SMEM((1,), jnp.int32),
            pltpu.VMEM((ND, HALO + S, L), _F32),
            pltpu.VMEM((NC + 1, C, D), _F32),
            pltpu.VMEM((2 * NC, 2 * C, D), _F32),
            [pltpu.VMEM((1, 2 * C, D), _F32)] * 2,
            pltpu.VMEM((NC + 1, 2 * C, D), _F32),
            pltpu.VMEM((1, S, D), _F32),
            pltpu.VMEM((8, 6 * D), _F32),
            [pltpu.VMEM((2, R, L), _F32)] * 4,
            [pltpu.VMEM((2, 8, L), _F32)] * 8,
            pltpu.VMEM((2, R, D), _F32),
            [pltpu.VMEM((2, R, D), _F32)] * 2,
            pltpu.VMEM((NF, D // 2, L), jnp.uint32),
            pltpu.VMEM((NF, D // 2, L), jnp.uint32),
            pltpu.VMEM((ND, FH // 2, L), jnp.uint32),
            pltpu.VMEM((S, D), _BF16),
            pltpu.SemaphoreType.DMA((n_in,)),
            pltpu.SemaphoreType.DMA((NB,)),
        ],
        compiler_params=pltpu.CompilerParams(vmem_limit_bytes=112 * 1024 * 1024),
    )(
        A_q.reshape(S, D), A_k.reshape(S, D), A_v.reshape(S, D),
        A_shift_k.T, A_ssm_k, A_ssm_D,
        B_w1, B_w3, B_w2, c, w_mod,
        jnp.asarray(_FWD, _BF16), jnp.asarray(_INV, _BF16), np.zeros((1,), np.int32),
    )
    return out.reshape(B, S, D)
```

```python
import numpy as np

import jax
import jax.numpy as jnp
import jax.experimental.pallas as pl
import jax.experimental.pallas.tpu as pltpu

C = 128
R = 256
L = 128
WG = 2
HALO = 8
RW = 128
RP = 32
PPRO = 1
RN = 32
MAC_LAG = 3
MARK_LAG = 3
MARK_SLOT = 0
TIE = 'zcth'
INV0 = 0
SC0, SC1 = 14, 24
NORM_AT = ((0, 3), (2, 5), (5, 9), (8, 11), (11, 14))
XFORM_AT = (3, 5, 11, 12)
MR = 16
NPRO = 4
MPRO = 4
CONV_AT = {2: 4, 3: 5, 4: 6, 5: 7}
MAC_AT = {2: [(4, 0, 40)], 3: [(5, 0, 40)],
          4: [(6, 0, 40)], 5: [(7, 0, 40)]}
SEND_AT = (1, 2, 3, 4, 5, 6, 7)
W2_GROUPS = ((0, 2), (2, 5))
KT = 4
EPS = 1e-5

_F32 = jnp.float32
_BF16 = jnp.bfloat16
_NT = (((1,), (1,)), ((), ()))


def _dft_matrices():
    even = np.arange(0, C, 2)
    f = np.concatenate([even, C - 1 - even]).astype(np.float64)
    ang = 2.0 * np.pi * (f[:, None] + 0.5) * np.arange(C)[None, :] / (2 * C)
    fwd = np.concatenate([np.cos(ang), -np.sin(ang)], axis=0)
    inv = fwd.T / C
    return fwd.astype(np.float32), inv.astype(np.float32)


_FWD, _INV = _dft_matrices()


def _dot(a, b):
    return jnp.dot(a, b, preferred_element_type=_F32)


def _row_mean(x, zero=None):
    acc = x[:, 0:L] if zero is None else x[:, 0:L] + zero
    for n in range(1, x.shape[1] // L):
        acc = acc + x[:, n * L:(n + 1) * L]
    m = jnp.sum(acc, axis=-1, keepdims=True) * (1.0 / x.shape[1])
    return jnp.broadcast_to(m, (x.shape[0], L))


def _silu(x):
    hx = 0.5 * x
    return hx * jnp.tanh(hx) + hx


def _spread(slots, steps, first, last):
    for k, step in enumerate(steps):
        slots[first + (k * (last - first)) // len(steps)].append(step)


def _fill(slots, sizes, steps, first):
    held = [sum(cost for _, cost in slot) for slot in slots]
    rate = (sum(held[first:]) + sum(cost for _, cost in steps)) / sum(sizes[first:])
    budget, k = 0.0, 0
    for s in range(first, len(slots)):
        budget += rate * sizes[s] - held[s]
        while k < len(steps) and (budget >= 0.5 * steps[k][1] or s == len(slots) - 1):
            slots[s].append(steps[k])
            budget -= steps[k][1]
            k += 1


def _kernel(q_hbm, k_hbm, v_hbm, shift_hbm, sk_hbm, d_hbm, w1_hbm, w3_hbm, w2_hbm,
            c_hbm, wm_hbm, fwd_hbm, inv_hbm, base_hbm, out_hbm,
            q_v, k_v, v_v, shift_v, sk_v, d_v, w1_v, w3_v, w2_v, c_v, wm_v, fwd_v, inv_v, base_sm,
            k_s, kv_s, u_s, kf_s, carry_s, z_s, y_s, mod_s, stat_s, mark_s, x1_s, h2_s, w1_p, w3_p, w2_p, out_v,
            in_sems, out_sems):
    S, D = q_hbm.shape
    FH = w1_hbm.shape[1]
    NB = S // R
    NC = S // C
    CPB = R // C
    NF = FH // L
    ND = D // L

    copies = {}

    def start(name, src, dst):
        cp = pltpu.make_async_copy(src, dst, in_sems.at[len(copies)])
        cp.start()
        copies[name] = cp

    def wait(*names):
        for name in names:
            copies[name].wait()

    def start_ssm(b):
        cols = pl.ds(b * R, R)
        start(("sk", b), sk_hbm.at[:, cols], sk_v.at[:, cols])

    def start_kv(b):
        rows = pl.ds(b * R, R)
        start(("k", b), k_hbm.at[rows, :], k_v.at[rows, :])
        start(("v", b), v_hbm.at[rows, :], v_v.at[rows, :])

    def start_q(b):
        rows = pl.ds(b * R, R)
        start(("q", b), q_hbm.at[rows, :], q_v.at[rows, :])

    start("base", base_hbm, base_sm)
    start("fwd", fwd_hbm, fwd_v)
    start("shift", shift_hbm, shift_v)
    start("d", d_hbm, d_v)
    start("c", c_hbm, c_v)
    start("inv", inv_hbm, inv_v)
    def start_mod(j):
        start(("wm", j), wm_hbm.at[:, pl.ds(j * D, D)], wm_v.at[j])

    for b in range(NPRO):
        start_ssm(b)
        start_kv(b)
        if b == 1:
            for j in range(PPRO):
                start_q(j)
    for j in (1, 0, 2, 4, 3):
        start_mod(j)
    for g in range(NF // WG):
        cols = pl.ds(g * WG * L, WG * L)
        start(("w1", g), w1_hbm.at[:, cols], w1_v.at[:, cols])
        start(("w3", g), w3_hbm.at[:, cols], w3_v.at[:, cols])
        if g == 0 and PPRO < 2:
            start_q(1)
    for n0, n1 in W2_GROUPS:
        cols = pl.ds(n0 * L, (n1 - n0) * L)
        start(("w2", n0), w2_hbm.at[:, cols], w2_v.at[:, cols])
    start_mod(5)
    for b in range(1, NB - 1):
        start_q(b + 1)
        if b in CONV_AT:
            start_ssm(CONV_AT[b])
        if b + 1 in CONV_AT:
            start_kv(CONV_AT[b + 1])

    wait("base")
    base = base_sm[0]

    for ref in (*z_s, *kv_s):
        ref[0, 0:8, 0:L] = jnp.zeros((8, L), _F32)
    for ref in stat_s:
        ref[0, 0:8] = jnp.zeros((8, L), _F32)
    for ref in h2_s:
        ref[0, 0:8, 0:L] = jnp.zeros((8, L), _F32)
    k_s[:, 0:HALO] = jnp.zeros((ND, HALO, L), _F32)

    written = []

    def wrote(ref, slot):
        if slot in TIE and not any(ref is r for r, _ in written):
            written.append((ref, slot))

    emitted = [0]

    def mark(result):
        mark_s[emitted[0] % len(mark_s)][1] = result[0:8, 0:L]
        emitted[0] += 1

    def after_mark(lag=MARK_LAG):
        return mark_s[(emitted[0] - 1 - lag) % len(mark_s)][base + MARK_SLOT, 0:1]

    for ref in mark_s:
        ref[0] = jnp.zeros((8, L), _F32)

    def mod(j):
        return mod_s[0:1, j * D:(j + 1) * D]

    def compute_mod(j):
        sc = _silu(c_v[...].astype(_F32)).astype(_BF16)
        sc = jnp.broadcast_to(sc, (16, D))
        mod_s[:, j * D:(j + 1) * D] = _dot(sc, wm_v[j])[0:8]

    def ssm_transform(m):
        spec = jax.lax.dot_general(tied(fwd_v[...]), sk_v[:, m * C:(m + 1) * C], _NT,
                                   preferred_element_type=_F32)
        if m == 0:
            kf_s[0][0, 0:C] = spec[0:C] + d_v[...].astype(_F32).reshape(1, D)
            kf_s[0][0, C:2 * C] = spec[C:2 * C]
        else:
            kf_s[m // CPB][m % CPB] = spec

    def widen_k(r0):
        kk = k_v[r0:r0 + RW, :].astype(_F32) + jnp.tile(after_mark(), (1, ND))
        for n in range(ND):
            k_s[n, HALO + r0:HALO + r0 + RW] = kk[:, n * L:(n + 1) * L]

    def short_conv(i, p):
        r0 = i * C + p * RP
        w = shift_v[...].astype(_F32)
        ks = None
        for j in range(w.shape[0]):
            kj = jnp.concatenate([k_s[base + n, HALO + r0 - j:HALO + r0 - j + RP]
                                  for n in range(ND)], axis=1)
            ks = kj * w[j:j + 1] if ks is None else ks + kj * w[j:j + 1]
        kv_s[i // CPB][1 + i % CPB, p * RP:(p + 1) * RP] = ks * v_v[r0:r0 + RP, :].astype(_F32)
        wrote(kv_s[i // CPB], 'c')

    def kv_transform(i):
        kv = kv_s[i // CPB][base + (1 + i % CPB)].astype(_BF16)
        u_s[i // CPB][i % CPB] = _dot(tied(fwd_v[...]), kv)

    def mac(b, g, n):
        chunks = range(b * CPB, (b + 1) * CPB)
        re = slice(MR * g, MR * (g + 1))
        im = slice(C + re.start, C + re.stop)
        ln = slice(n * L, (n + 1) * L)

        def tile(refs, i):
            return refs[i // CPB][base + i % CPB, re, ln], refs[i // CPB][base + i % CPB, im, ln]

        acc = {}
        kf = {}
        for i in range(chunks[-1] + 1):
            ur, ui = tile(u_s, i)
            for j in chunks:
                if j < i:
                    continue
                if j - i not in kf:
                    kf[j - i] = tile(kf_s, j - i)
                kr, ki = kf[j - i]
                pr, pi = kr * ur - ki * ui, kr * ui + ki * ur
                acc[j] = (acc[j][0] + pr, acc[j][1] + pi) if j in acc else (pr, pi)
        if b > 0:
            carry = carry_s[(b - 1) % 2]
            acc[chunks[0] - 1] = (carry[base, re, ln], carry[base, im, ln])
        if b + 1 < NB:
            carry_s[b % 2][0, re, ln], carry_s[b % 2][0, im, ln] = acc[chunks[-1]]
        for j in chunks:
            zr, zi = acc[j]
            if j > 0:
                pr, pi = acc[j - 1]
                zr, zi = (zr - pi, zi + pr) if re.start < C // 2 else (zr + pi, zi - pr)
            z_s[b][1 + j % CPB, re, ln] = zr
            z_s[b][1 + j % CPB, im, ln] = zi
        wrote(z_s[b], 'z')

    def inverse_transform(b, jj):
        z = z_s[b][base + (1 + jj)]
        y_s[b][0, jj * C:(jj + 1) * C] = _dot(tied(inv_v[...]), z.astype(_BF16))

    def stat(k, rows):
        s = stat_s[k][base + 1, rows]
        return jnp.tile(s + after_mark() if k % 2 == 0 else s, (1, ND))

    def q_rows(b, rows):
        return q_v[b * R + rows.start:b * R + rows.stop, :].astype(_F32)

    def norm1_mean(b, rows):
        stat_s[0][1, rows] = _row_mean(q_rows(b, rows), after_mark())
        wrote(stat_s[0], 't')

    def norm1_scale(b, rows):
        xc = q_rows(b, rows) - stat(0, rows)
        stat_s[1][1, rows] = jax.lax.rsqrt(_row_mean(xc * xc) + EPS)
        wrote(stat_s[1], 't')

    def residual(b, rows):
        x = q_rows(b, rows)
        y = y_s[b][base, rows]
        h = (x - stat(0, rows)) * stat(1, rows) * (1.0 + mod(1)) + mod(0)
        x1 = x + mod(2) * (h * y)
        x1_s[b % 2, rows] = x1
        stat_s[2][1, rows] = _row_mean(x1)
        wrote(stat_s[2], 't')

    def norm2_scale(b, rows):
        xc = x1_s[base + b % 2, rows] - stat(2, rows)
        stat_s[3][1, rows] = jax.lax.rsqrt(_row_mean(xc * xc) + EPS)
        wrote(stat_s[3], 't')

    def norm2_apply(b, rows):
        xc = x1_s[base + b % 2, rows] - stat(2, rows)
        h2 = xc * stat(3, rows) * (1.0 + mod(4)) + mod(3)
        h2_s[b % 2][1, rows] = h2
        wrote(h2_s[b % 2], 'h')

    def tied(lhs):
        zero = None
        for ref, slot in written:
            w = pltpu.bitcast(ref[base, 0:8, 0:L], jnp.uint32)
            zero = w if zero is None else zero | w
        written.clear()
        if zero is None:
            return lhs
        tile = pltpu.bitcast(pltpu.bitcast(lhs[0:16, 0:L], jnp.uint32) | zero, _BF16)
        if lhs.shape[1] > L:
            tile = jnp.concatenate([tile, lhs[0:16, L:]], axis=1)
        return jnp.concatenate([tile, lhs[16:]], axis=0)

    def weight(b, raw, packed, tile, rows):
        words = slice(rows.start // 2, rows.stop // 2)
        if b == 0:
            w = raw[rows, tile * L:(tile + 1) * L]
            packed[tile, words] = pltpu.bitcast(w, jnp.uint32)
            return w
        return pltpu.bitcast(packed[base + tile, words], _BF16)

    live = {}

    def ffn_gate(b, f):
        if f == 0:
            live["h2"] = h2_s[b % 2][base + 1].astype(_BF16)
        if b == 0 and f % WG == 0:
            wait(("w1", f // WG), ("w3", f // WG))
            if f == 0 and PPRO < 2:
                wait(("q", 1))
        live["gate"] = _dot(tied(live["h2"]), weight(b, w1_v, w1_p, f, slice(0, D)))
        mark(live["gate"])

    def ffn_up(b, f):
        up = _dot(tied(live["h2"]), weight(b, w3_v, w3_p, f, slice(0, D)))
        mark(up)
        live["act", f] = (_silu(live.pop("gate")) * up).astype(_BF16)

    out_copies = []

    def write_out(b, n, o):
        rows = pl.ds(b * R, R)
        cols = slice(n * L, (n + 1) * L)
        out_v[rows, cols] = (x1_s[base + b % 2, :, cols] + mod(5)[:, cols] * o).astype(_BF16)

    def send_out(b):
        first = max([s + 1 for s in SEND_AT if s < b], default=0)
        rows = pl.ds(first * R, (b + 1 - first) * R)
        cp = pltpu.make_async_copy(out_v.at[rows, :], out_hbm.at[rows, :], out_sems.at[b])
        cp.start()
        out_copies.append(cp)

    def ffn_down(b, n, kk):
        if b == 0 and kk == 0 and n in dict(W2_GROUPS):
            wait(("w2", n))
        act = jnp.concatenate([live["act", kk * KT + j] for j in range(KT)], axis=1)
        o = _dot(tied(act), weight(b, w2_v, w2_p, n, slice(kk * KT * L, (kk + 1) * KT * L)))
        mark(o)
        if kk > 0:
            o = live.pop(("out", n)) + o
        if kk + 1 < NF // KT or b == 0:
            live["out", n] = o
        else:
            write_out(b, n, o)

    def ffn_steps(b):
        steps = []
        for f in range(NF):
            steps += [lambda f=f: ffn_gate(b, f), lambda f=f: ffn_up(b, f)]
        steps += [lambda n=n, kk=kk: ffn_down(b, n, kk)
                  for n in range(ND) for kk in range(NF // KT)]
        return steps

    def short_conv_steps(b):
        return ([(lambda r0=r0: widen_k(r0), 2 * RW * ND // 8)
                 for r0 in range(b * R, (b + 1) * R, RW)]
                + [(lambda i=i, p=p: short_conv(i, p), 9 * RP * ND // 8)
                   for i in range(b * CPB, (b + 1) * CPB) for p in range(C // RP)])

    def mac_steps(b):
        cost = sum(j + 1 for j in range(b * CPB, (b + 1) * CPB)) * MR
        return [(lambda g=g, n=n: mac(b, g, n), cost)
                for g in range(C // MR) for n in range(ND)]

    def norm_passes(b, rn=RN):
        return [[(lambda p=p, fn=fn: fn(b, slice(p * rn, (p + 1) * rn)), ops * rn * ND // 8)
                 for p in range(R // rn)]
                for fn, ops in ((norm1_mean, 2), (norm1_scale, 5), (residual, 9),
                                (norm2_scale, 4), (norm2_apply, 5))]

    def transform_steps(b):
        return [(lambda i=i, fn=fn: fn(i), 0)
                for fn in (ssm_transform, kv_transform) for i in range(b * CPB, (b + 1) * CPB)]

    def pipeline_step(b):
        main = ffn_steps(b)
        sizes = [ND] * (2 * NF) + [KT] * (len(main) - 2 * NF)
        slots = [[] for _ in main]
        if b == 1:
            for n in range(ND):
                slots[n].append((lambda n=n: write_out(0, n, live.pop(("out", n))), 3 * R // 8))
        if b in CONV_AT:
            for step, at in zip(transform_steps(CONV_AT[b]), XFORM_AT):
                slots[at].append(step)
        if PPRO <= b + 1 < NB:
            for jj in range(CPB):
                slots[INV0 + jj].append((lambda jj=jj: inverse_transform(b + 1, jj), 0))
            for steps, (first, stop) in zip(norm_passes(b + 1), NORM_AT):
                _spread(slots, steps, first, stop)
        if b + 1 in CONV_AT:
            _spread(slots, short_conv_steps(CONV_AT[b + 1]), SC0, SC1)
        macs = [step for blk, lo, hi in MAC_AT.get(b, ()) for step in mac_steps(blk)[lo:hi]]
        if macs:
            fresh = MAC_AT[b][0][0] == CONV_AT.get(b)
            _fill(slots, sizes, macs, XFORM_AT[-1] + MAC_LAG if fresh else 0)
        for step, side in zip(main, slots):
            step()
            for extra, _ in side:
                extra()
        if b in SEND_AT:
            send_out(b)

    def run(steps):
        for step, _ in steps:
            step()

    wait("fwd", "shift", "d", "c", "inv")
    early = [norm_passes(b, R) for b in range(PPRO)]
    last = max(NPRO + 1, MPRO + 2)
    for r in range(last):
        if r < NPRO:
            wait(("sk", r), ("k", r), ("v", r))
        if r == 1:
            wait(*[("q", b) for b in range(PPRO)])
        if r == last - 1:
            wait(("wm", 1), ("wm", 0), ("wm", 2))
            for j in (1, 0, 2):
                compute_mod(j)
            for passes in early:
                run(passes[2] + passes[3])
        main = transform_steps(r - 1) if 1 <= r <= NPRO else []
        if 3 <= r < PPRO + 3:
            main += [(lambda jj=jj: inverse_transform(r - 3, jj), 0) for jj in range(CPB)]
        side = mac_steps(r - 2) if 2 <= r < MPRO + 2 else []
        slots = [[step] for step in main] or [[]]
        if side:
            _spread(slots, side, 0, len(slots))
        run(sum(slots, []))
        if r == 1:
            for passes in early:
                run(passes[0] + passes[1])
        if r < NPRO:
            run(short_conv_steps(r))
        written.clear()
    wait(("wm", 4), ("wm", 3))
    for j in (4, 3):
        compute_mod(j)
    for passes in early:
        run(passes[4])
    for b in range(NB):
        if 1 <= b < NB - 1:
            wait(("q", b + 1))
        if b in CONV_AT:
            wait(("sk", CONV_AT[b]))
        if b + 1 in CONV_AT:
            wait(("k", CONV_AT[b + 1]), ("v", CONV_AT[b + 1]))
        if b == 1:
            wait(("wm", 5))
            compute_mod(5)
        pipeline_step(b)
    for cp in out_copies:
        cp.wait()


@jax.jit
def pallas_adaLN_cond__ssm_conv_h3__glu_gated_swiglu__prompt_kernel(
    A_q: jax.Array,
    A_k: jax.Array,
    A_v: jax.Array,
    A_shift_k: jax.Array,
    A_ssm_k: jax.Array,
    A_ssm_D: jax.Array,
    B_x: jax.Array,
    B_w1: jax.Array,
    B_w3: jax.Array,
    B_w2: jax.Array,
    c: jax.Array,
    w_mod: jax.Array,
):
    del B_x
    B, S, D = A_q.shape
    FH = B_w1.shape[1]
    KS = A_shift_k.shape[1]
    assert B == 1 and S % R == 0 and FH % (KT * L) == 0 and D % L == 0 and KS <= HALO + 1
    NB, CPB = S // R, R // C
    NF, ND = FH // L, D // L
    n_in = 6 + 4 * NB + 6 + 2 * (NF // WG) + len(W2_GROUPS)

    hbm = pl.BlockSpec(memory_space=pl.ANY)
    out = pl.pallas_call(
        _kernel,
        out_shape=jax.ShapeDtypeStruct((S, D), A_q.dtype),
        in_specs=[hbm] * 14,
        out_specs=hbm,
        scratch_shapes=[
            pltpu.VMEM((S, D), _BF16),
            pltpu.VMEM((S, D), _BF16),
            pltpu.VMEM((S, D), _BF16),
            pltpu.VMEM((KS, D), _BF16),
            pltpu.VMEM((D, S), _BF16),
            pltpu.VMEM((D,), _BF16),
            pltpu.VMEM((D, FH), _BF16),
            pltpu.VMEM((D, FH), _BF16),
            pltpu.VMEM((FH, D), _BF16),
            pltpu.VMEM((1, D), _BF16),
            pltpu.VMEM((6, D, D), _BF16),
            pltpu.VMEM((2 * C, C), _BF16),
            pltpu.VMEM((C, 2 * C), _BF16),
            pltpu.SMEM((1,), jnp.int32),
            pltpu.VMEM((ND, HALO + S, L), _F32),
            [pltpu.VMEM((CPB + 1, C, D), _F32)] * NB,
            [pltpu.VMEM((CPB, 2 * C, D), _F32)] * NB,
            [pltpu.VMEM((CPB, 2 * C, D), _F32)] * NB,
            [pltpu.VMEM((1, 2 * C, D), _F32)] * 2,
            [pltpu.VMEM((CPB + 1, 2 * C, D), _F32)] * NB,
            [pltpu.VMEM((1, R, D), _F32)] * NB,
            pltpu.VMEM((8, 6 * D), _F32),
            [pltpu.VMEM((2, R, L), _F32)] * 4,
            [pltpu.VMEM((2, 8, L), _F32)] * 8,
            pltpu.VMEM((2, R, D), _F32),
            [pltpu.VMEM((2, R, D), _F32)] * 2,
            pltpu.VMEM((NF, D // 2, L), jnp.uint32),
            pltpu.VMEM((NF, D // 2, L), jnp.uint32),
            pltpu.VMEM((ND, FH // 2, L), jnp.uint32),
            pltpu.VMEM((S, D), _BF16),
            pltpu.SemaphoreType.DMA((n_in,)),
            pltpu.SemaphoreType.DMA((NB,)),
        ],
        compiler_params=pltpu.CompilerParams(vmem_limit_bytes=120 * 1024 * 1024),
    )(
        A_q.reshape(S, D), A_k.reshape(S, D), A_v.reshape(S, D),
        A_shift_k.T, A_ssm_k, A_ssm_D,
        B_w1, B_w3, B_w2, c, w_mod,
        jnp.asarray(_FWD, _BF16), jnp.asarray(_INV, _BF16), np.zeros((1,), np.int32),
    )
    return out.reshape(B, S, D)
```

```python
import numpy as np

import jax
import jax.numpy as jnp
import jax.experimental.pallas as pl
import jax.experimental.pallas.tpu as pltpu

C = 128
R = 256
L = 128
WG = 2
HALO = 8
RW = 128
RP = 32
RN = 32
MAC_LAG = 3
MARK_LAG = 3
TIE = 'zcth'
INV0 = 0
SC0, SC1 = 14, 24
NORM_AT = ((0, 3), (2, 5), (5, 9), (8, 11), (11, 14))
XFORM_AT = (3, 5, 11, 12)
NPRO = 4
CONV_AT = {2: 4, 3: 5, 4: 6, 5: 7}
MAC_AT = {2: [(4, 0, 40)], 3: [(5, 0, 40)],
          4: [(6, 0, 40)], 5: [(7, 0, 40)]}
SEND_AT = (1, 2, 3, 4, 5, 6, 7)
W2_GROUPS = ((0, 2), (2, 5))
KT = 4
EPS = 1e-5

_F32 = jnp.float32
_BF16 = jnp.bfloat16
_NT = (((1,), (1,)), ((), ()))


def _packed_bf16(x):
    bits = np.ascontiguousarray(x, np.float32).view(np.uint32)
    bits = (bits + 0x7FFF + ((bits >> 16) & 1)) >> 16
    return bits[0::2] | (bits[1::2] << 16)


def _dft_matrices():
    even = np.arange(0, C, 2)
    f = np.stack([even.reshape(-1, 8), C - 1 - even.reshape(-1, 8)], axis=1).reshape(-1)
    step = 2.0 * np.pi / (2 * C)
    ang = step * (f[:, None] + 0.5) * np.arange(C)[None, :]
    fwd = np.concatenate([np.cos(ang), -np.sin(ang)], axis=0)
    n = np.concatenate([even, even + 1])
    ang = step * n[:, None] * (even[None, :] + 0.5)
    inv = np.concatenate([np.cos(ang), -np.sin(ang)], axis=1) / C
    return _packed_bf16(fwd), _packed_bf16(inv)


_FWD, _INV = _dft_matrices()


def _dot(a, b):
    return jnp.dot(a, b, preferred_element_type=_F32)


def _row_mean(x, zero=None):
    acc = x[:, 0:L] if zero is None else x[:, 0:L] + zero
    for n in range(1, x.shape[1] // L):
        acc = acc + x[:, n * L:(n + 1) * L]
    m = jnp.sum(acc, axis=-1, keepdims=True) * (1.0 / x.shape[1])
    return jnp.broadcast_to(m, (x.shape[0], L))


def _silu(x):
    hx = 0.5 * x
    return hx * jnp.tanh(hx) + hx


def _spread(slots, steps, first, last):
    for k, step in enumerate(steps):
        slots[first + (k * (last - first)) // len(steps)].append(step)


def _fill(slots, sizes, steps, first):
    held = [sum(cost for _, cost in slot) for slot in slots]
    rate = (sum(held[first:]) + sum(cost for _, cost in steps)) / sum(sizes[first:])
    budget, k = 0.0, 0
    for s in range(first, len(slots)):
        budget += rate * sizes[s] - held[s]
        while k < len(steps) and (budget >= 0.5 * steps[k][1] or s == len(slots) - 1):
            slots[s].append(steps[k])
            budget -= steps[k][1]
            k += 1


def _kernel(q_hbm, k_hbm, v_hbm, shift_hbm, sk_hbm, d_hbm, w1_hbm, w3_hbm, w2_hbm,
            c_hbm, wm_hbm, fwd_hbm, inv_hbm, base_hbm, out_hbm,
            q_v, k_v, v_v, shift_v, sk_v, d_v, w1_v, w3_v, w2_v, c_v, wm_v, fwd_v, inv_v, base_sm,
            k_s, kv_s, u_s, kf_s, carry_s, z_s, y_s, mod_s, stat_s, mark_s, x1_s, h2_s, w1_p, w3_p, w2_p, out_v,
            in_sems, out_sems):
    S, D = q_hbm.shape
    FH = w1_hbm.shape[1]
    NB = S // R
    NC = S // C
    CPB = R // C
    NF = FH // L
    ND = D // L

    copies = {}

    def start(name, src, dst):
        cp = pltpu.make_async_copy(src, dst, in_sems.at[len(copies)])
        cp.start()
        copies[name] = cp

    def wait(*names):
        for name in names:
            copies[name].wait()

    def start_ssm(b):
        cols = pl.ds(b * R, R)
        start(("sk", b), sk_hbm.at[:, cols], sk_v.at[:, cols])

    def start_kv(b):
        rows = pl.ds(b * R, R)
        start(("k", b), k_hbm.at[rows, :], k_v.at[rows, :])
        start(("v", b), v_hbm.at[rows, :], v_v.at[rows, :])

    def start_q(b):
        rows = pl.ds(b * R, R)
        start(("q", b), q_hbm.at[rows, :], q_v.at[rows, :])

    start("base", base_hbm, base_sm)
    start("fwd", fwd_hbm, fwd_v)
    start("shift", shift_hbm, shift_v)
    start("d", d_hbm, d_v)
    start("c", c_hbm, c_v)
    start("inv", inv_hbm, inv_v)
    def start_mod(j):
        start(("wm", j), wm_hbm.at[:, pl.ds(j * D, D)], wm_v.at[j])

    for b in range(NPRO):
        start_kv(b)
        start_ssm(b)
    start_q(0)
    for j in (1, 0, 2, 4, 3):
        start_mod(j)
    for g in range(NF // WG):
        cols = pl.ds(g * WG * L, WG * L)
        start(("w1", g), w1_hbm.at[:, cols], w1_v.at[:, cols])
        start(("w3", g), w3_hbm.at[:, cols], w3_v.at[:, cols])
        if g == 0:
            start_q(1)
    for n0, n1 in W2_GROUPS:
        cols = pl.ds(n0 * L, (n1 - n0) * L)
        start(("w2", n0), w2_hbm.at[:, cols], w2_v.at[:, cols])
    start_mod(5)
    for b in range(1, NB - 1):
        start_q(b + 1)
        if b in CONV_AT:
            start_ssm(CONV_AT[b])
        if b + 1 in CONV_AT:
            start_kv(CONV_AT[b + 1])

    wait("base")
    base = base_sm[0]

    for ref in (*z_s, *kv_s):
        ref[0, 0:8, 0:L] = jnp.zeros((8, L), _F32)
    for ref in stat_s:
        ref[0, 0:8] = jnp.zeros((8, L), _F32)
    for ref in h2_s:
        ref[0, 0:8, 0:L] = jnp.zeros((8, L), _F32)
    k_s[:, 0:HALO] = jnp.zeros((ND, HALO, L), _F32)

    written = []

    def wrote(ref, slot):
        if slot in TIE and not any(ref is r for r in written):
            written.append(ref)

    emitted = [0]

    def mark(result):
        mark_s[emitted[0] % len(mark_s)][1] = result[0:8, 0:L]
        emitted[0] += 1

    def after_mark(lag=MARK_LAG):
        return mark_s[(emitted[0] - 1 - lag) % len(mark_s)][base, 0:1]

    for ref in mark_s:
        ref[0] = jnp.zeros((8, L), _F32)

    def mod(j):
        return mod_s[0:1, j * D:(j + 1) * D]

    def compute_mod(j):
        sc = _silu(c_v[...].astype(_F32)).astype(_BF16)
        sc = jnp.broadcast_to(sc, (16, D))
        mod_s[:, j * D:(j + 1) * D] = _dot(sc, wm_v[j])[0:8]

    def ssm_transform(m):
        spec = jax.lax.dot_general(tied(fwd_v[...]), sk_v[:, m * C:(m + 1) * C], _NT,
                                   preferred_element_type=_F32)
        if m == 0:
            kf_s[0][0, 0:C] = spec[0:C] + d_v[...].astype(_F32).reshape(1, D)
            kf_s[0][0, C:2 * C] = spec[C:2 * C]
        else:
            kf_s[m // CPB][m % CPB] = spec

    def widen_k(r0):
        kk = k_v[r0:r0 + RW, :].astype(_F32) + jnp.tile(after_mark(), (1, ND))
        for n in range(ND):
            k_s[n, HALO + r0:HALO + r0 + RW] = kk[:, n * L:(n + 1) * L]

    def short_conv(i, p):
        r0 = i * C + p * RP
        w = shift_v[...].astype(_F32)
        ks = None
        for j in range(w.shape[0]):
            kj = jnp.concatenate([k_s[base + n, HALO + r0 - j:HALO + r0 - j + RP]
                                  for n in range(ND)], axis=1)
            ks = kj * w[j:j + 1] if ks is None else ks + kj * w[j:j + 1]
        kv_s[i // CPB][1 + i % CPB, p * RP:(p + 1) * RP] = ks * v_v[r0:r0 + RP, :].astype(_F32)
        wrote(kv_s[i // CPB], 'c')

    def kv_transform(i):
        kv = kv_s[i // CPB][base + (1 + i % CPB)].astype(_BF16)
        u_s[i // CPB][i % CPB] = _dot(tied(fwd_v[...]), kv)

    def mac(b, g, n):
        chunks = range(b * CPB, (b + 1) * CPB)
        re = pl.ds(16 * g, 16)
        im = pl.ds(C + 16 * g, 16)
        ln = slice(n * L, (n + 1) * L)

        def tile(refs, i):
            return refs[i // CPB][base + i % CPB, re, ln], refs[i // CPB][base + i % CPB, im, ln]

        acc = {}
        kf = {}
        for i in range(chunks[-1] + 1):
            ur, ui = tile(u_s, i)
            for j in chunks:
                if j < i:
                    continue
                if j - i not in kf:
                    kf[j - i] = tile(kf_s, j - i)
                kr, ki = kf[j - i]
                pr, pi = kr * ur - ki * ui, kr * ui + ki * ur
                acc[j] = (acc[j][0] + pr, acc[j][1] + pi) if j in acc else (pr, pi)
        if b > 0:
            carry = carry_s[(b - 1) % 2]
            acc[chunks[0] - 1] = (carry[base, re, ln], carry[base, im, ln])
        if b + 1 < NB:
            carry_s[b % 2][0, re, ln], carry_s[b % 2][0, im, ln] = acc[chunks[-1]]
        for j in chunks:
            (ar, br), (ai, bi) = ((x[0:8], x[8:16]) for x in acc[j])
            if j > 0:
                pr, pi = acc[j - 1]
                ar, ai = ar - pi[0:8], ai + pr[0:8]
                br, bi = br + pi[8:16], bi - pr[8:16]
            for k, x in enumerate((ar + br, ai - bi, ar - br, ai + bi)):
                z_s[b][1 + j % CPB, pl.ds(k * (C // 2) + 8 * g, 8), ln] = x
        wrote(z_s[b], 'z')

    def inverse_transform(b, jj):
        for odd in range(2):
            z = z_s[b][base + (1 + jj), odd * C:(odd + 1) * C].astype(_BF16)
            y = _dot(tied(inv_v[odd * C // 4:(odd + 1) * C // 4]), z)
            for n in range(ND):
                y_s[b][n, pl.ds(jj * C + odd, C // 2, stride=2), :] = y[:, n * L:(n + 1) * L]

    def stat(k, rows):
        s = stat_s[k][base + 1, rows]
        return jnp.tile(s + after_mark() if k % 2 == 0 else s, (1, ND))

    def q_rows(b, rows):
        return q_v[b * R + rows.start:b * R + rows.stop, :].astype(_F32)

    def norm1_mean(b, rows):
        stat_s[0][1, rows] = _row_mean(q_rows(b, rows), after_mark())
        wrote(stat_s[0], 't')

    def norm1_scale(b, rows):
        xc = q_rows(b, rows) - stat(0, rows)
        stat_s[1][1, rows] = jax.lax.rsqrt(_row_mean(xc * xc) + EPS)
        wrote(stat_s[1], 't')

    def residual(b, rows):
        x = q_rows(b, rows)
        y = jnp.concatenate([y_s[b][base + n, rows] for n in range(ND)], axis=1)
        h = (x - stat(0, rows)) * stat(1, rows) * (1.0 + mod(1)) + mod(0)
        x1 = x + mod(2) * (h * y)
        x1_s[b % 2, rows] = x1
        stat_s[2][1, rows] = _row_mean(x1)
        wrote(stat_s[2], 't')

    def norm2_scale(b, rows):
        xc = x1_s[base + b % 2, rows] - stat(2, rows)
        stat_s[3][1, rows] = jax.lax.rsqrt(_row_mean(xc * xc) + EPS)
        wrote(stat_s[3], 't')

    def norm2_apply(b, rows):
        xc = x1_s[base + b % 2, rows] - stat(2, rows)
        h2 = xc * stat(3, rows) * (1.0 + mod(4))
        h2_s[b % 2][1, rows] = h2
        wrote(h2_s[b % 2], 'h')

    def tied(words):
        if written:
            top = words[0:8, 0:L]
            for ref in written:
                top = top | pltpu.bitcast(ref[base, 0:8, 0:L], jnp.uint32)
            written.clear()
            if words.shape[1] > L:
                top = jnp.concatenate([top, words[0:8, L:]], axis=1)
            words = jnp.concatenate([top, words[8:]], axis=0)
        return pltpu.bitcast(words, _BF16)

    def weight(b, raw, packed, tile, rows):
        words = slice(rows.start // 2, rows.stop // 2)
        if b == 0:
            w = raw[rows, tile * L:(tile + 1) * L]
            packed[tile, words] = pltpu.bitcast(w, jnp.uint32)
            return w
        return tied(packed[base + tile, words])

    live = {}

    def ffn_gate(b, f):
        if f == 0:
            live["h2"] = (h2_s[b % 2][base + 1] + mod(3)).astype(_BF16)
        if b == 0 and f % WG == 0:
            wait(("w1", f // WG), ("w3", f // WG))
            if f == 0:
                wait(("q", 1))
        live["gate"] = _dot(live["h2"], weight(b, w1_v, w1_p, f, slice(0, D)))
        mark(live["gate"])

    def ffn_up(b, f):
        up = _dot(live["h2"], weight(b, w3_v, w3_p, f, slice(0, D)))
        mark(up)
        live["act", f] = (_silu(live.pop("gate")) * up).astype(_BF16)

    out_copies = []

    def write_out(b, n, o):
        rows = pl.ds(b * R, R)
        cols = slice(n * L, (n + 1) * L)
        out_v[rows, cols] = (x1_s[base + b % 2, :, cols] + mod(5)[:, cols] * o).astype(_BF16)

    def send_out(b):
        first = max([s + 1 for s in SEND_AT if s < b], default=0)
        rows = pl.ds(first * R, (b + 1 - first) * R)
        cp = pltpu.make_async_copy(out_v.at[rows, :], out_hbm.at[rows, :], out_sems.at[b])
        cp.start()
        out_copies.append(cp)

    def ffn_down(b, n, kk):
        if b == 0 and kk == 0 and n in dict(W2_GROUPS):
            wait(("w2", n))
        act = jnp.concatenate([live["act", kk * KT + j] for j in range(KT)], axis=1)
        o = _dot(act, weight(b, w2_v, w2_p, n, slice(kk * KT * L, (kk + 1) * KT * L)))
        mark(o)
        if kk > 0:
            o = live.pop(("out", n)) + o
        if kk + 1 < NF // KT or b == 0:
            live["out", n] = o
        else:
            write_out(b, n, o)

    def ffn_steps(b):
        steps = []
        for f in range(NF):
            steps += [lambda f=f: ffn_gate(b, f), lambda f=f: ffn_up(b, f)]
        steps += [lambda n=n, kk=kk: ffn_down(b, n, kk)
                  for n in range(ND) for kk in range(NF // KT)]
        return steps

    def short_conv_steps(b):
        return ([(lambda r0=r0: widen_k(r0), 2 * RW * ND // 8)
                 for r0 in range(b * R, (b + 1) * R, RW)]
                + [(lambda i=i, p=p: short_conv(i, p), 9 * RP * ND // 8)
                   for i in range(b * CPB, (b + 1) * CPB) for p in range(C // RP)])

    def mac_steps(b):
        cost = sum(j + 1 for j in range(b * CPB, (b + 1) * CPB)) * 16
        return [(lambda g=g, n=n: mac(b, g, n), cost)
                for g in range(C // 16) for n in range(ND)]

    def norm_passes(b, rn=RN):
        return [[(lambda p=p, fn=fn: fn(b, slice(p * rn, (p + 1) * rn)), ops * rn * ND // 8)
                 for p in range(R // rn)]
                for fn, ops in ((norm1_mean, 2), (norm1_scale, 5), (residual, 9),
                                (norm2_scale, 4), (norm2_apply, 5))]

    def transform_steps(b):
        return [(lambda i=i, fn=fn: fn(i), 0)
                for fn in (ssm_transform, kv_transform) for i in range(b * CPB, (b + 1) * CPB)]

    def pipeline_step(b):
        main = ffn_steps(b)
        sizes = [ND] * (2 * NF) + [KT] * (len(main) - 2 * NF)
        slots = [[] for _ in main]
        if b == 1:
            for n in range(ND):
                slots[n].append((lambda n=n: write_out(0, n, live.pop(("out", n))), 3 * R // 8))
        if b in CONV_AT:
            for step, at in zip(transform_steps(CONV_AT[b]), XFORM_AT):
                slots[at].append(step)
        if b + 1 < NB:
            for jj in range(CPB):
                slots[INV0 + jj].append((lambda jj=jj: inverse_transform(b + 1, jj), 0))
            for steps, (first, stop) in zip(norm_passes(b + 1), NORM_AT):
                _spread(slots, steps, first, stop)
        if b + 1 in CONV_AT:
            _spread(slots, short_conv_steps(CONV_AT[b + 1]), SC0, SC1)
        macs = [step for blk, lo, hi in MAC_AT.get(b, ()) for step in mac_steps(blk)[lo:hi]]
        if macs:
            fresh = MAC_AT[b][0][0] == CONV_AT.get(b)
            _fill(slots, sizes, macs, XFORM_AT[-1] + MAC_LAG if fresh else 0)
        for step, side in zip(main, slots):
            step()
            for extra, _ in side:
                extra()
        if b in SEND_AT:
            send_out(b)

    def run(steps):
        for step, _ in steps:
            step()

    wait("fwd", "shift", "d", "c", "inv")
    norm0 = norm_passes(0, R)
    for r in range(NPRO + 2):
        if r < NPRO:
            wait(("k", r), ("v", r), ("sk", r))
        elif r == NPRO:
            wait(("q", 0))
            run(norm0[0] + norm0[1])
        else:
            wait(("wm", 1), ("wm", 0), ("wm", 2))
            for j in (1, 0, 2):
                compute_mod(j)
            run(norm0[2] + norm0[3])
        if 1 <= r <= NPRO:
            run(transform_steps(r - 1)[CPB:])
        if r < NPRO:
            run(transform_steps(r)[:CPB] + short_conv_steps(r))
        if r == 3:
            for jj in range(CPB):
                inverse_transform(0, jj)
        if r >= 2:
            run(mac_steps(r - 2))
        written.clear()
    wait(("wm", 4))
    compute_mod(4)
    run(norm0[4])
    wait(("wm", 3))
    compute_mod(3)
    for b in range(NB):
        if 1 <= b < NB - 1:
            wait(("q", b + 1))
        if b in CONV_AT:
            wait(("sk", CONV_AT[b]))
        if b + 1 in CONV_AT:
            wait(("k", CONV_AT[b + 1]), ("v", CONV_AT[b + 1]))
        if b == 1:
            wait(("wm", 5))
            compute_mod(5)
        pipeline_step(b)
    for cp in out_copies:
        cp.wait()


@jax.jit
def pallas_adaLN_cond__ssm_conv_h3__glu_gated_swiglu__prompt_kernel(
    A_q: jax.Array,
    A_k: jax.Array,
    A_v: jax.Array,
    A_shift_k: jax.Array,
    A_ssm_k: jax.Array,
    A_ssm_D: jax.Array,
    B_x: jax.Array,
    B_w1: jax.Array,
    B_w3: jax.Array,
    B_w2: jax.Array,
    c: jax.Array,
    w_mod: jax.Array,
):
    del B_x
    B, S, D = A_q.shape
    FH = B_w1.shape[1]
    KS = A_shift_k.shape[1]
    assert B == 1 and S % R == 0 and FH % (KT * L) == 0 and D % L == 0 and KS <= HALO + 1
    NB, CPB = S // R, R // C
    NF, ND = FH // L, D // L
    n_in = 6 + 4 * NB + 6 + 2 * (NF // WG) + len(W2_GROUPS)

    hbm = pl.BlockSpec(memory_space=pl.ANY)
    out = pl.pallas_call(
        _kernel,
        out_shape=jax.ShapeDtypeStruct((S, D), A_q.dtype),
        in_specs=[hbm] * 14,
        out_specs=hbm,
        scratch_shapes=[
            pltpu.VMEM((S, D), _BF16),
            pltpu.VMEM((S, D), _BF16),
            pltpu.VMEM((S, D), _BF16),
            pltpu.VMEM((KS, D), _BF16),
            pltpu.VMEM((D, S), _BF16),
            pltpu.VMEM((D,), _BF16),
            pltpu.VMEM((D, FH), _BF16),
            pltpu.VMEM((D, FH), _BF16),
            pltpu.VMEM((FH, D), _BF16),
            pltpu.VMEM((1, D), _BF16),
            pltpu.VMEM((6, D, D), _BF16),
            pltpu.VMEM(_FWD.shape, jnp.uint32),
            pltpu.VMEM(_INV.shape, jnp.uint32),
            pltpu.SMEM((1,), jnp.int32),
            pltpu.VMEM((ND, HALO + S, L), _F32),
            [pltpu.VMEM((CPB + 1, C, D), _F32)] * NB,
            [pltpu.VMEM((CPB, 2 * C, D), _F32)] * NB,
            [pltpu.VMEM((CPB, 2 * C, D), _F32)] * NB,
            [pltpu.VMEM((1, 2 * C, D), _F32)] * 2,
            [pltpu.VMEM((CPB + 1, 2 * C, D), _F32)] * NB,
            [pltpu.VMEM((ND, R, L), _F32)] * NB,
            pltpu.VMEM((8, 6 * D), _F32),
            [pltpu.VMEM((2, R, L), _F32)] * 4,
            [pltpu.VMEM((2, 8, L), _F32)] * 8,
            pltpu.VMEM((2, R, D), _F32),
            [pltpu.VMEM((2, R, D), _F32)] * 2,
            pltpu.VMEM((NF, D // 2, L), jnp.uint32),
            pltpu.VMEM((NF, D // 2, L), jnp.uint32),
            pltpu.VMEM((ND, FH // 2, L), jnp.uint32),
            pltpu.VMEM((S, D), _BF16),
            pltpu.SemaphoreType.DMA((n_in,)),
            pltpu.SemaphoreType.DMA((NB,)),
        ],
        compiler_params=pltpu.CompilerParams(vmem_limit_bytes=120 * 1024 * 1024),
    )(
        A_q.reshape(S, D), A_k.reshape(S, D), A_v.reshape(S, D),
        A_shift_k.T, A_ssm_k, A_ssm_D,
        B_w1, B_w3, B_w2, c, w_mod,
        _FWD, _INV, np.zeros((1,), np.int32),
    )
    return out.reshape(B, S, D)
```

```python
import numpy as np

import jax
import jax.numpy as jnp
import jax.experimental.pallas as pl
import jax.experimental.pallas.tpu as pltpu

C = 128
R = 256
L = 128
WG = 2
HALO = 8
RW = 128
RP = 32
RN = 32
MAC_LAG = 3
MARK_LAG = 3
TIE = 'zcth'
INV0 = 0
SC0, SC1 = 14, 24
NORM_AT = ((0, 3), (2, 5), (5, 9), (8, 11), (11, 14))
XFORM_AT = (3, 5, 11, 12)
NPRO = 4
MPRO = 3
CONV_AT = {2: 4, 3: 5, 4: 6, 5: 7}
MAC_AT = {0: [(3, 0, 40)], 2: [(4, 0, 40)], 3: [(5, 0, 40)],
          4: [(6, 0, 40)], 5: [(7, 0, 40)]}
SEND_AT = (1, 2, 3, 4, 5, 6, 7)
CUTS = ()
Q1_AFTER = 2
W2_GROUPS = ((0, 2), (2, 5))
KT = 4
EPS = 1e-5

_F32 = jnp.float32
_BF16 = jnp.bfloat16
_NT = (((1,), (1,)), ((), ()))


def _packed_bf16(x):
    bits = np.ascontiguousarray(x, np.float32).view(np.uint32)
    bits = (bits + 0x7FFF + ((bits >> 16) & 1)) >> 16
    return bits[0::2] | (bits[1::2] << 16)


def _dft_matrices():
    even = np.arange(0, C, 2)
    f = np.stack([even.reshape(-1, 8), C - 1 - even.reshape(-1, 8)], axis=1).reshape(-1)
    step = 2.0 * np.pi / (2 * C)
    ang = step * (f[:, None] + 0.5) * np.arange(C)[None, :]
    fwd = np.concatenate([np.cos(ang), -np.sin(ang)], axis=0)
    n = np.concatenate([even, even + 1])
    ang = step * n[:, None] * (even[None, :] + 0.5)
    inv = np.concatenate([np.cos(ang), -np.sin(ang)], axis=1) / C
    return _packed_bf16(fwd), _packed_bf16(inv)


_FWD, _INV = _dft_matrices()


def _dot(a, b):
    return jnp.dot(a, b, preferred_element_type=_F32)


def _row_mean(x, zero=None):
    acc = x[:, 0:L] if zero is None else x[:, 0:L] + zero
    for n in range(1, x.shape[1] // L):
        acc = acc + x[:, n * L:(n + 1) * L]
    m = jnp.sum(acc, axis=-1, keepdims=True) * (1.0 / x.shape[1])
    return jnp.broadcast_to(m, (x.shape[0], L))


def _silu(x):
    hx = 0.5 * x
    return hx * jnp.tanh(hx) + hx


def _spread(slots, steps, first, last):
    for k, step in enumerate(steps):
        slots[first + (k * (last - first)) // len(steps)].append(step)


def _fill(slots, sizes, steps, first):
    held = [sum(cost for _, cost in slot) for slot in slots]
    rate = (sum(held[first:]) + sum(cost for _, cost in steps)) / sum(sizes[first:])
    budget, k = 0.0, 0
    for s in range(first, len(slots)):
        budget += rate * sizes[s] - held[s]
        while k < len(steps) and (budget >= 0.5 * steps[k][1] or s == len(slots) - 1):
            slots[s].append(steps[k])
            budget -= steps[k][1]
            k += 1


def _kernel(q_hbm, k_hbm, v_hbm, shift_hbm, sk_hbm, d_hbm, w1_hbm, w3_hbm, w2_hbm,
            c_hbm, wm_hbm, fwd_hbm, inv_hbm, base_hbm, out_hbm,
            q_v, k_v, v_v, shift_v, sk_v, d_v, w1_v, w3_v, w2_v, c_v, wm_v, fwd_v, inv_v, base_sm,
            k_s, kv_s, u_s, kf_s, carry_s, z_s, y_s, mod_s, stat_s, mark_s, x1_s, h2_s, w1_p, w3_p, w2_p, out_v,
            in_sems, out_sems):
    S, D = q_hbm.shape
    FH = w1_hbm.shape[1]
    NB = S // R
    NC = S // C
    CPB = R // C
    NF = FH // L
    ND = D // L

    copies = {}

    def start(name, src, dst):
        cp = pltpu.make_async_copy(src, dst, in_sems.at[len(copies)])
        cp.start()
        copies[name] = cp

    def start_ssm(b):
        cols = pl.ds(b * R, R)
        start(("sk", b), sk_hbm.at[:, cols], sk_v.at[:, cols])

    def start_kv(b):
        rows = pl.ds(b * R, R)
        start(("k", b), k_hbm.at[rows, :], k_v.at[rows, :])
        start(("v", b), v_hbm.at[rows, :], v_v.at[rows, :])

    def start_q(b):
        rows = pl.ds(b * R, R)
        start(("q", b), q_hbm.at[rows, :], q_v.at[rows, :])

    start("base", base_hbm, base_sm)
    start("fwd", fwd_hbm, fwd_v)
    start("shift", shift_hbm, shift_v)
    start("d", d_hbm, d_v)
    start("c", c_hbm, c_v)
    start("inv", inv_hbm, inv_v)
    def start_mod(j):
        start(("wm", j), wm_hbm.at[:, pl.ds(j * D, D)], wm_v.at[j])

    for b in range(NPRO):
        start_kv(b)
        start_ssm(b)
    start_q(0)
    for j in (1, 0, 2, 4, 3):
        start_mod(j)
    for g in range(NF // WG):
        cols = pl.ds(g * WG * L, WG * L)
        start(("w1", g), w1_hbm.at[:, cols], w1_v.at[:, cols])
        start(("w3", g), w3_hbm.at[:, cols], w3_v.at[:, cols])
        if g == Q1_AFTER:
            start_q(1)
    for n0, n1 in W2_GROUPS:
        cols = pl.ds(n0 * L, (n1 - n0) * L)
        start(("w2", n0), w2_hbm.at[:, cols], w2_v.at[:, cols])
    start_mod(5)
    for b in range(1, NB - 1):
        start_q(b + 1)
        if b in CONV_AT:
            start_ssm(CONV_AT[b])
        if b + 1 in CONV_AT:
            start_kv(CONV_AT[b + 1])

    copies["base"].wait()
    base = base_sm[0]

    def fence():
        @pl.loop(0, base)
        def _(i):
            mark_s[0][1] = jnp.zeros((8, L), _F32)

    def wait(*names):
        for name in names:
            copies[name].wait()
        fence()

    for ref in (*z_s, *kv_s):
        ref[0, 0:8, 0:L] = jnp.zeros((8, L), _F32)
    for ref in stat_s:
        ref[0, 0:8] = jnp.zeros((8, L), _F32)
    for ref in h2_s:
        ref[0, 0:8, 0:L] = jnp.zeros((8, L), _F32)
    k_s[:, 0:HALO] = jnp.zeros((ND, HALO, L), _F32)

    written = []

    def wrote(ref, slot):
        if slot in TIE and not any(ref is r for r in written):
            written.append(ref)

    emitted = [0]

    def mark(result):
        mark_s[emitted[0] % len(mark_s)][1] = result[0:8, 0:L]
        emitted[0] += 1

    def after_mark(lag=MARK_LAG):
        return mark_s[(emitted[0] - 1 - lag) % len(mark_s)][base, 0:1]

    for ref in mark_s:
        ref[0] = jnp.zeros((8, L), _F32)

    def mod(j):
        return mod_s[0:1, j * D:(j + 1) * D]

    def compute_mod(j):
        sc = _silu(c_v[...].astype(_F32)).astype(_BF16)
        sc = jnp.broadcast_to(sc, (16, D))
        mod_s[:, j * D:(j + 1) * D] = _dot(sc, wm_v[j])[0:8]

    def ssm_transform(m):
        spec = jax.lax.dot_general(tied(fwd_v[...]), sk_v[:, m * C:(m + 1) * C], _NT,
                                   preferred_element_type=_F32)
        if m == 0:
            kf_s[0][0, 0:C] = spec[0:C] + d_v[...].astype(_F32).reshape(1, D)
            kf_s[0][0, C:2 * C] = spec[C:2 * C]
        else:
            kf_s[m // CPB][m % CPB] = spec

    def widen_k(r0):
        kk = k_v[r0:r0 + RW, :].astype(_F32) + jnp.tile(after_mark(), (1, ND))
        for n in range(ND):
            k_s[n, HALO + r0:HALO + r0 + RW] = kk[:, n * L:(n + 1) * L]

    def short_conv(i, p):
        r0 = i * C + p * RP
        w = shift_v[...].astype(_F32)
        ks = None
        for j in range(w.shape[0]):
            kj = jnp.concatenate([k_s[base + n, HALO + r0 - j:HALO + r0 - j + RP]
                                  for n in range(ND)], axis=1)
            ks = kj * w[j:j + 1] if ks is None else ks + kj * w[j:j + 1]
        kv_s[i // CPB][1 + i % CPB, p * RP:(p + 1) * RP] = ks * v_v[r0:r0 + RP, :].astype(_F32)
        wrote(kv_s[i // CPB], 'c')

    def kv_transform(i):
        kv = kv_s[i // CPB][base + (1 + i % CPB)].astype(_BF16)
        u_s[i // CPB][i % CPB] = _dot(tied(fwd_v[...]), kv)

    def mac(b, g, n):
        chunks = range(b * CPB, (b + 1) * CPB)
        re = pl.ds(16 * g, 16)
        im = pl.ds(C + 16 * g, 16)
        ln = slice(n * L, (n + 1) * L)

        def tile(refs, i):
            return refs[i // CPB][base + i % CPB, re, ln], refs[i // CPB][base + i % CPB, im, ln]

        acc = {}
        kf = {}
        for i in range(chunks[-1] + 1):
            ur, ui = tile(u_s, i)
            for j in chunks:
                if j < i:
                    continue
                if j - i not in kf:
                    kf[j - i] = tile(kf_s, j - i)
                kr, ki = kf[j - i]
                pr, pi = kr * ur - ki * ui, kr * ui + ki * ur
                acc[j] = (acc[j][0] + pr, acc[j][1] + pi) if j in acc else (pr, pi)
        if b > 0:
            carry = carry_s[(b - 1) % 2]
            acc[chunks[0] - 1] = (carry[base, re, ln], carry[base, im, ln])
        if b + 1 < NB:
            carry_s[b % 2][0, re, ln], carry_s[b % 2][0, im, ln] = acc[chunks[-1]]
        for j in chunks:
            (ar, br), (ai, bi) = ((x[0:8], x[8:16]) for x in acc[j])
            if j > 0:
                pr, pi = acc[j - 1]
                ar, ai = ar - pi[0:8], ai + pr[0:8]
                br, bi = br + pi[8:16], bi - pr[8:16]
            for k, x in enumerate((ar + br, ai - bi, ar - br, ai + bi)):
                z_s[b][1 + j % CPB, pl.ds(k * (C // 2) + 8 * g, 8), ln] = x
        wrote(z_s[b], 'z')

    def inverse_transform(b, jj):
        for odd in range(2):
            z = z_s[b][base + (1 + jj), odd * C:(odd + 1) * C].astype(_BF16)
            y = _dot(tied(inv_v[odd * C // 4:(odd + 1) * C // 4]), z)
            for n in range(ND):
                y_s[b][n, pl.ds(jj * C + odd, C // 2, stride=2), :] = y[:, n * L:(n + 1) * L]

    def stat(k, rows):
        s = stat_s[k][base + 1, rows]
        return jnp.tile(s + after_mark() if k % 2 == 0 else s, (1, ND))

    def q_rows(b, rows):
        return q_v[b * R + rows.start:b * R + rows.stop, :].astype(_F32)

    def norm1_mean(b, rows):
        stat_s[0][1, rows] = _row_mean(q_rows(b, rows), after_mark())
        wrote(stat_s[0], 't')

    def norm1_scale(b, rows):
        xc = q_rows(b, rows) - stat(0, rows)
        stat_s[1][1, rows] = jax.lax.rsqrt(_row_mean(xc * xc) + EPS)
        wrote(stat_s[1], 't')

    def residual(b, rows):
        x = q_rows(b, rows)
        y = jnp.concatenate([y_s[b][base + n, rows] for n in range(ND)], axis=1)
        h = (x - stat(0, rows)) * stat(1, rows) * (1.0 + mod(1)) + mod(0)
        x1 = x + mod(2) * (h * y)
        x1_s[b % 2, rows] = x1
        stat_s[2][1, rows] = _row_mean(x1)
        wrote(stat_s[2], 't')

    def norm2_scale(b, rows):
        xc = x1_s[base + b % 2, rows] - stat(2, rows)
        stat_s[3][1, rows] = jax.lax.rsqrt(_row_mean(xc * xc) + EPS)
        wrote(stat_s[3], 't')

    def norm2_apply(b, rows):
        xc = x1_s[base + b % 2, rows] - stat(2, rows)
        h2 = xc * stat(3, rows) * (1.0 + mod(4))
        h2_s[b % 2][1, rows] = h2
        wrote(h2_s[b % 2], 'h')

    def tied(words):
        if written:
            top = words[0:8, 0:L]
            for ref in written:
                top = top | pltpu.bitcast(ref[base, 0:8, 0:L], jnp.uint32)
            written.clear()
            if words.shape[1] > L:
                top = jnp.concatenate([top, words[0:8, L:]], axis=1)
            words = jnp.concatenate([top, words[8:]], axis=0)
        return pltpu.bitcast(words, _BF16)

    def weight(b, raw, packed, tile, rows):
        words = slice(rows.start // 2, rows.stop // 2)
        if b == 0:
            w = raw[rows, tile * L:(tile + 1) * L]
            packed[tile, words] = pltpu.bitcast(w, jnp.uint32)
            return w
        return tied(packed[base + tile, words])

    live = {}

    def ffn_gate(b, f):
        if f == 0:
            live["h2"] = (h2_s[b % 2][base + 1] + mod(3)).astype(_BF16)
        if b == 0 and f % WG == 0:
            wait(("w1", f // WG), ("w3", f // WG))
            if f == (Q1_AFTER + 1) * WG:
                wait(("q", 1))
        live["gate"] = _dot(live["h2"], weight(b, w1_v, w1_p, f, slice(0, D)))
        mark(live["gate"])

    def ffn_up(b, f):
        up = _dot(live["h2"], weight(b, w3_v, w3_p, f, slice(0, D)))
        mark(up)
        live["act", f] = (_silu(live.pop("gate")) * up).astype(_BF16)

    out_copies = []

    def write_out(b, n, o):
        rows = pl.ds(b * R, R)
        cols = slice(n * L, (n + 1) * L)
        out_v[rows, cols] = (x1_s[base + b % 2, :, cols] + mod(5)[:, cols] * o).astype(_BF16)

    def send_out(b):
        first = max([s + 1 for s in SEND_AT if s < b], default=0)
        rows = pl.ds(first * R, (b + 1 - first) * R)
        cp = pltpu.make_async_copy(out_v.at[rows, :], out_hbm.at[rows, :], out_sems.at[b])
        cp.start()
        out_copies.append(cp)

    def ffn_down(b, n, kk):
        if b == 0 and kk == 0 and n in dict(W2_GROUPS):
            wait(("w2", n))
        act = jnp.concatenate([live["act", kk * KT + j] for j in range(KT)], axis=1)
        o = _dot(act, weight(b, w2_v, w2_p, n, slice(kk * KT * L, (kk + 1) * KT * L)))
        mark(o)
        if kk > 0:
            o = live.pop(("out", n)) + o
        if kk + 1 < NF // KT or b == 0:
            live["out", n] = o
        else:
            write_out(b, n, o)

    def ffn_steps(b):
        steps = []
        for f in range(NF):
            steps += [lambda f=f: ffn_gate(b, f), lambda f=f: ffn_up(b, f)]
        steps += [lambda n=n, kk=kk: ffn_down(b, n, kk)
                  for n in range(ND) for kk in range(NF // KT)]
        return steps

    def short_conv_steps(b):
        return ([(lambda r0=r0: widen_k(r0), 2 * RW * ND // 8)
                 for r0 in range(b * R, (b + 1) * R, RW)]
                + [(lambda i=i, p=p: short_conv(i, p), 9 * RP * ND // 8)
                   for i in range(b * CPB, (b + 1) * CPB) for p in range(C // RP)])

    def mac_steps(b):
        cost = sum(j + 1 for j in range(b * CPB, (b + 1) * CPB)) * 16
        return [(lambda g=g, n=n: mac(b, g, n), cost)
                for g in range(C // 16) for n in range(ND)]

    def norm_passes(b, rn=RN):
        return [[(lambda p=p, fn=fn: fn(b, slice(p * rn, (p + 1) * rn)), ops * rn * ND // 8)
                 for p in range(R // rn)]
                for fn, ops in ((norm1_mean, 2), (norm1_scale, 5), (residual, 9),
                                (norm2_scale, 4), (norm2_apply, 5))]

    def transform_steps(b):
        return [(lambda i=i, fn=fn: fn(i), 0)
                for fn in (ssm_transform, kv_transform) for i in range(b * CPB, (b + 1) * CPB)]

    def pipeline_step(b):
        main = ffn_steps(b)
        sizes = [ND] * (2 * NF) + [KT] * (len(main) - 2 * NF)
        slots = [[] for _ in main]
        if b == 1:
            for n in range(ND):
                slots[n].append((lambda n=n: write_out(0, n, live.pop(("out", n))), 3 * R // 8))
        if b in CONV_AT:
            for step, at in zip(transform_steps(CONV_AT[b]), XFORM_AT):
                slots[at].append(step)
        if b + 1 < NB:
            for jj in range(CPB):
                slots[INV0 + jj].append((lambda jj=jj: inverse_transform(b + 1, jj), 0))
            late = 2 * WG * (Q1_AFTER + 1) if b == 0 else 0
            for steps, (first, stop) in zip(norm_passes(b + 1), NORM_AT):
                _spread(slots, steps, late + first, late + stop)
        if b + 1 in CONV_AT:
            if b == 1:
                slots[SC0].append((lambda: wait(("k", CONV_AT[2]), ("v", CONV_AT[2])), 0))
            _spread(slots, short_conv_steps(CONV_AT[b + 1]), SC0, SC1)
        macs = [step for blk, lo, hi in MAC_AT.get(b, ()) for step in mac_steps(blk)[lo:hi]]
        if macs:
            fresh = MAC_AT[b][0][0] == CONV_AT.get(b)
            _fill(slots, sizes, macs, XFORM_AT[-1] + MAC_LAG if fresh else 0)
        for at in CUTS if b > 0 else ():
            slots[at].append((fence, 0))
        for step, side in zip(main, slots):
            step()
            for extra, _ in side:
                extra()
        if b in SEND_AT:
            send_out(b)

    def run(steps):
        for step, _ in steps:
            step()

    wait("fwd", "shift", "d", "c", "inv")
    norm0 = norm_passes(0, R)
    for r in range(NPRO + 2):
        if r < NPRO:
            wait(("k", r), ("v", r), ("sk", r))
        elif r == NPRO:
            wait(("q", 0))
            run(norm0[0] + norm0[1])
        else:
            wait(("wm", 1), ("wm", 0), ("wm", 2))
            for j in (1, 0, 2):
                compute_mod(j)
            run(norm0[2] + norm0[3])
        if 1 <= r <= NPRO:
            run(transform_steps(r - 1)[CPB:])
        if r < NPRO:
            run(transform_steps(r)[:CPB] + short_conv_steps(r))
        if r == 3:
            for jj in range(CPB):
                inverse_transform(0, jj)
        if 2 <= r < MPRO + 2:
            run(mac_steps(r - 2))
        written.clear()
    wait(("wm", 4))
    compute_mod(4)
    run(norm0[4])
    wait(("wm", 3))
    compute_mod(3)
    for b in range(NB):
        needs = [("q", b + 1)] if 1 <= b < NB - 1 else []
        if b in CONV_AT:
            needs += [("sk", CONV_AT[b])]
        if b + 1 in CONV_AT and b > 1:
            needs += [("k", CONV_AT[b + 1]), ("v", CONV_AT[b + 1])]
        if needs:
            wait(*needs)
        if b == NB - 1:
            fence()
        if b == 1:
            wait(("wm", 5))
            compute_mod(5)
        pipeline_step(b)
    for cp in out_copies:
        cp.wait()


@jax.jit
def pallas_adaLN_cond__ssm_conv_h3__glu_gated_swiglu__prompt_kernel(
    A_q: jax.Array,
    A_k: jax.Array,
    A_v: jax.Array,
    A_shift_k: jax.Array,
    A_ssm_k: jax.Array,
    A_ssm_D: jax.Array,
    B_x: jax.Array,
    B_w1: jax.Array,
    B_w3: jax.Array,
    B_w2: jax.Array,
    c: jax.Array,
    w_mod: jax.Array,
):
    del B_x
    B, S, D = A_q.shape
    FH = B_w1.shape[1]
    KS = A_shift_k.shape[1]
    assert B == 1 and S % R == 0 and FH % (KT * L) == 0 and D % L == 0 and KS <= HALO + 1
    NB, CPB = S // R, R // C
    NF, ND = FH // L, D // L
    n_in = 6 + 4 * NB + 6 + 2 * (NF // WG) + len(W2_GROUPS)

    hbm = pl.BlockSpec(memory_space=pl.ANY)
    out = pl.pallas_call(
        _kernel,
        out_shape=jax.ShapeDtypeStruct((S, D), A_q.dtype),
        in_specs=[hbm] * 14,
        out_specs=hbm,
        scratch_shapes=[
            pltpu.VMEM((S, D), _BF16),
            pltpu.VMEM((S, D), _BF16),
            pltpu.VMEM((S, D), _BF16),
            pltpu.VMEM((KS, D), _BF16),
            pltpu.VMEM((D, S), _BF16),
            pltpu.VMEM((D,), _BF16),
            pltpu.VMEM((D, FH), _BF16),
            pltpu.VMEM((D, FH), _BF16),
            pltpu.VMEM((FH, D), _BF16),
            pltpu.VMEM((1, D), _BF16),
            pltpu.VMEM((6, D, D), _BF16),
            pltpu.VMEM(_FWD.shape, jnp.uint32),
            pltpu.VMEM(_INV.shape, jnp.uint32),
            pltpu.SMEM((1,), jnp.int32),
            pltpu.VMEM((ND, HALO + S, L), _F32),
            [pltpu.VMEM((CPB + 1, C, D), _F32)] * NB,
            [pltpu.VMEM((CPB, 2 * C, D), _F32)] * NB,
            [pltpu.VMEM((CPB, 2 * C, D), _F32)] * NB,
            [pltpu.VMEM((1, 2 * C, D), _F32)] * 2,
            [pltpu.VMEM((CPB + 1, 2 * C, D), _F32)] * NB,
            [pltpu.VMEM((ND, R, L), _F32)] * NB,
            pltpu.VMEM((8, 6 * D), _F32),
            [pltpu.VMEM((2, R, L), _F32)] * 4,
            [pltpu.VMEM((2, 8, L), _F32)] * 8,
            pltpu.VMEM((2, R, D), _F32),
            [pltpu.VMEM((2, R, D), _F32)] * 2,
            pltpu.VMEM((NF, D // 2, L), jnp.uint32),
            pltpu.VMEM((NF, D // 2, L), jnp.uint32),
            pltpu.VMEM((ND, FH // 2, L), jnp.uint32),
            pltpu.VMEM((S, D), _BF16),
            pltpu.SemaphoreType.DMA((n_in,)),
            pltpu.SemaphoreType.DMA((NB,)),
        ],
        compiler_params=pltpu.CompilerParams(vmem_limit_bytes=120 * 1024 * 1024),
    )(
        A_q.reshape(S, D), A_k.reshape(S, D), A_v.reshape(S, D),
        A_shift_k.T, A_ssm_k, A_ssm_D,
        B_w1, B_w3, B_w2, c, w_mod,
        _FWD, _INV, np.zeros((1,), np.int32),
    )
    return out.reshape(B, S, D)
```

```python
import numpy as np

import jax
import jax.numpy as jnp
import jax.experimental.pallas as pl
import jax.experimental.pallas.tpu as pltpu

C = 128
R = 256
L = 128
HALO = 8
RW = 128
RP = 32
RN = 32
MAC_LAG = 3
MARK_LAG = 3
TIE = 'zcth'
INV0 = 0
SC0, SC1 = 14, 24
NORM_AT = ((0, 3), (2, 5), (5, 9), (8, 11), (11, 14))
XFORM_AT = (3, 5, 11, 12)
NPRO = 4
MPRO = 3
CONV_AT = {2: 4, 3: 5, 4: 6, 5: 7}
MAC_AT = {1: [(3, 0, 40)], 2: [(4, 0, 40)], 3: [(5, 0, 40)],
          4: [(6, 0, 40)], 5: [(7, 0, 40)]}
SEND_AT = (1, 2, 3, 4, 5, 6, 7)
W13_GROUPS = ((0, 2), (2, 6), (6, 12))
KT = 4
EPS = 1e-5

_F32 = jnp.float32
_BF16 = jnp.bfloat16
_NT = (((1,), (1,)), ((), ()))


def _packed_bf16(x):
    bits = np.ascontiguousarray(x, np.float32).view(np.uint32)
    bits = (bits + 0x7FFF + ((bits >> 16) & 1)) >> 16
    return bits[0::2] | (bits[1::2] << 16)


def _dft_matrices():
    even = np.arange(0, C, 2)
    f = np.stack([even.reshape(-1, 8), C - 1 - even.reshape(-1, 8)], axis=1).reshape(-1)
    step = 2.0 * np.pi / (2 * C)
    ang = step * (f[:, None] + 0.5) * np.arange(C)[None, :]
    fwd = np.concatenate([np.cos(ang), -np.sin(ang)], axis=0)
    n = np.concatenate([even, even + 1])
    ang = step * n[:, None] * (even[None, :] + 0.5)
    inv = np.concatenate([np.cos(ang), -np.sin(ang)], axis=1) / C
    return _packed_bf16(fwd), _packed_bf16(inv)


_FWD, _INV = _dft_matrices()


def _dot(a, b):
    return jnp.dot(a, b, preferred_element_type=_F32)


def _row_mean(x, zero=None):
    acc = x[:, 0:L] if zero is None else x[:, 0:L] + zero
    for n in range(1, x.shape[1] // L):
        acc = acc + x[:, n * L:(n + 1) * L]
    m = jnp.sum(acc, axis=-1, keepdims=True) * (1.0 / x.shape[1])
    return jnp.broadcast_to(m, (x.shape[0], L))


def _silu(x):
    hx = 0.5 * x
    return hx * jnp.tanh(hx) + hx


def _spread(slots, steps, first, last):
    for k, step in enumerate(steps):
        slots[first + (k * (last - first)) // len(steps)].append(step)


def _fill(slots, sizes, steps, first):
    held = [sum(cost for _, cost in slot) for slot in slots]
    rate = (sum(held[first:]) + sum(cost for _, cost in steps)) / sum(sizes[first:])
    budget, k = 0.0, 0
    for s in range(first, len(slots)):
        budget += rate * sizes[s] - held[s]
        while k < len(steps) and (budget >= 0.5 * steps[k][1] or s == len(slots) - 1):
            slots[s].append(steps[k])
            budget -= steps[k][1]
            k += 1


def _kernel(q_hbm, k_hbm, v_hbm, shift_hbm, sk_hbm, d_hbm, w1_hbm, w3_hbm, w2_hbm,
            c_hbm, wm_hbm, fwd_hbm, inv_hbm, base_hbm, out_hbm,
            q_v, k_v, v_v, shift_v, sk_v, d_v, w1_v, w3_v, w2_v, c_v, wm_v, fwd_v, inv_v, base_sm,
            k_s, kv_s, u_s, kf_s, carry_s, z_s, y_s, mod_s, stat_s, mark_s, x1_s, h2_s, out_v,
            in_sems, out_sems):
    S, D = q_hbm.shape
    FH = w1_hbm.shape[1]
    NB = S // R
    NC = S // C
    CPB = R // C
    NF = FH // L
    ND = D // L

    copies = {}

    def start(name, src, dst):
        cp = pltpu.make_async_copy(src, dst, in_sems.at[len(copies)])
        cp.start()
        copies[name] = cp

    def start_ssm(b):
        cols = pl.ds(b * R, R)
        start(("sk", b), sk_hbm.at[:, cols], sk_v.at[:, cols])

    def start_kv(b):
        rows = pl.ds(b * R, R)
        start(("k", b), k_hbm.at[rows, :], k_v.at[rows, :])
        start(("v", b), v_hbm.at[rows, :], v_v.at[rows, :])

    def start_q(b):
        rows = pl.ds(b * R, R)
        start(("q", b), q_hbm.at[rows, :], q_v.at[rows, :])

    start("base", base_hbm, base_sm)
    start("fwd", fwd_hbm, fwd_v)
    start("shift", shift_hbm, shift_v)
    start("d", d_hbm, d_v)
    start("c", c_hbm, c_v)
    start("inv", inv_hbm, inv_v)
    def start_mod(j):
        start(("wm", j), wm_hbm.at[:, pl.ds(j * D, D)], wm_v.at[j])

    for b in range(NPRO):
        start_kv(b)
        start_ssm(b)
    start_q(0)
    start_q(1)
    for j in (1, 0, 2, 4, 3):
        start_mod(j)
    for f in range(NF):
        start(("w1", f), w1_hbm.at[:, pl.ds(f * L, L)], w1_v.at[f])
        start(("w3", f), w3_hbm.at[:, pl.ds(f * L, L)], w3_v.at[f])
        if f + 1 == W13_GROUPS[0][1]:
            start_q(2)
    for n in range(ND):
        start(("w2", n), w2_hbm.at[:, pl.ds(n * L, L)], w2_v.at[n])
    start_mod(5)
    for b in range(1, NB - 1):
        if b > 1:
            start_q(b + 1)
        if b in CONV_AT:
            start_ssm(CONV_AT[b])
        if b + 1 in CONV_AT:
            start_kv(CONV_AT[b + 1])

    copies["base"].wait()
    base = base_sm[0]

    def fence():
        @pl.loop(0, base)
        def _(i):
            mark_s[0][1] = jnp.zeros((8, L), _F32)

    def wait(*names):
        for name in names:
            copies[name].wait()
        fence()

    for ref in (*z_s, *kv_s):
        ref[0, 0:8, 0:L] = jnp.zeros((8, L), _F32)
    for ref in stat_s:
        ref[0, 0:8] = jnp.zeros((8, L), _F32)
    for ref in h2_s:
        ref[0, 0:8, 0:L] = jnp.zeros((8, L), _F32)
    k_s[:, 0:HALO] = jnp.zeros((ND, HALO, L), _F32)

    written = []

    def wrote(ref, slot):
        if slot in TIE and not any(ref is r for r in written):
            written.append(ref)

    emitted = [0]

    def mark(result):
        mark_s[emitted[0] % len(mark_s)][1] = result[0:8, 0:L]
        emitted[0] += 1

    def after_mark(lag=MARK_LAG):
        return mark_s[(emitted[0] - 1 - lag) % len(mark_s)][base, 0:1]

    for ref in mark_s:
        ref[0] = jnp.zeros((8, L), _F32)

    def mod(j):
        return mod_s[0:1, j * D:(j + 1) * D]

    def compute_mod(j):
        sc = _silu(c_v[...].astype(_F32)).astype(_BF16)
        sc = jnp.broadcast_to(sc, (16, D))
        mod_s[:, j * D:(j + 1) * D] = _dot(sc, wm_v[j])[0:8]

    def ssm_transform(m):
        spec = jax.lax.dot_general(tied(fwd_v[...]), sk_v[:, m * C:(m + 1) * C], _NT,
                                   preferred_element_type=_F32)
        if m == 0:
            kf_s[0][0, 0:C] = spec[0:C] + d_v[...].astype(_F32).reshape(1, D)
            kf_s[0][0, C:2 * C] = spec[C:2 * C]
        else:
            kf_s[m // CPB][m % CPB] = spec

    def widen_k(r0):
        kk = k_v[r0:r0 + RW, :].astype(_F32) + jnp.tile(after_mark(), (1, ND))
        for n in range(ND):
            k_s[n, HALO + r0:HALO + r0 + RW] = kk[:, n * L:(n + 1) * L]

    def short_conv(i, p):
        r0 = i * C + p * RP
        w = shift_v[...].astype(_F32)
        ks = None
        for j in range(w.shape[0]):
            kj = jnp.concatenate([k_s[base + n, HALO + r0 - j:HALO + r0 - j + RP]
                                  for n in range(ND)], axis=1)
            ks = kj * w[j:j + 1] if ks is None else ks + kj * w[j:j + 1]
        kv_s[i // CPB][1 + i % CPB, p * RP:(p + 1) * RP] = ks * v_v[r0:r0 + RP, :].astype(_F32)
        wrote(kv_s[i // CPB], 'c')

    def kv_transform(i):
        kv = kv_s[i // CPB][base + (1 + i % CPB)].astype(_BF16)
        u_s[i // CPB][i % CPB] = _dot(tied(fwd_v[...]), kv)

    def mac(b, g, n):
        chunks = range(b * CPB, (b + 1) * CPB)
        re = pl.ds(16 * g, 16)
        im = pl.ds(C + 16 * g, 16)
        ln = slice(n * L, (n + 1) * L)

        def tile(refs, i):
            return refs[i // CPB][base + i % CPB, re, ln], refs[i // CPB][base + i % CPB, im, ln]

        acc = {}
        kf = {}
        for i in range(chunks[-1] + 1):
            ur, ui = tile(u_s, i)
            for j in chunks:
                if j < i:
                    continue
                if j - i not in kf:
                    kf[j - i] = tile(kf_s, j - i)
                kr, ki = kf[j - i]
                pr, pi = kr * ur - ki * ui, kr * ui + ki * ur
                acc[j] = (acc[j][0] + pr, acc[j][1] + pi) if j in acc else (pr, pi)
        if b > 0:
            carry = carry_s[(b - 1) % 2]
            acc[chunks[0] - 1] = (carry[base, re, ln], carry[base, im, ln])
        if b + 1 < NB:
            carry_s[b % 2][0, re, ln], carry_s[b % 2][0, im, ln] = acc[chunks[-1]]
        for j in chunks:
            (ar, br), (ai, bi) = ((x[0:8], x[8:16]) for x in acc[j])
            if j > 0:
                pr, pi = acc[j - 1]
                ar, ai = ar - pi[0:8], ai + pr[0:8]
                br, bi = br + pi[8:16], bi - pr[8:16]
            for k, x in enumerate((ar + br, ai - bi, ar - br, ai + bi)):
                z_s[b][1 + j % CPB, pl.ds(k * (C // 2) + 8 * g, 8), ln] = x
        wrote(z_s[b], 'z')

    def inverse_transform(b, jj):
        for odd in range(2):
            z = z_s[b][base + (1 + jj), odd * C:(odd + 1) * C].astype(_BF16)
            y = _dot(tied(inv_v[odd * C // 4:(odd + 1) * C // 4]), z)
            for n in range(ND):
                y_s[b][n, pl.ds(jj * C + odd, C // 2, stride=2), :] = y[:, n * L:(n + 1) * L]

    def stat(k, b, rows):
        s = stat_s[k][base + (1 + b % 2), rows]
        return jnp.tile(s + after_mark() if k % 2 == 0 else s, (1, ND))

    def q_rows(b, rows):
        return q_v[b * R + rows.start:b * R + rows.stop, :].astype(_F32)

    def norm1_mean(b, rows):
        stat_s[0][1 + b % 2, rows] = _row_mean(q_rows(b, rows), after_mark())
        wrote(stat_s[0], 't')

    def norm1_scale(b, rows):
        xc = q_rows(b, rows) - stat(0, b, rows)
        stat_s[1][1 + b % 2, rows] = jax.lax.rsqrt(_row_mean(xc * xc) + EPS)
        wrote(stat_s[1], 't')

    def residual(b, rows):
        x = q_rows(b, rows)
        y = jnp.concatenate([y_s[b][base + n, rows] for n in range(ND)], axis=1)
        h = (x - stat(0, b, rows)) * stat(1, b, rows) * (1.0 + mod(1)) + mod(0)
        x1 = x + mod(2) * (h * y)
        x1_s[b % 3, rows] = x1
        stat_s[2][1 + b % 2, rows] = _row_mean(x1)
        wrote(stat_s[2], 't')

    def norm2_scale(b, rows):
        xc = x1_s[base + b % 3, rows] - stat(2, b, rows)
        stat_s[3][1 + b % 2, rows] = jax.lax.rsqrt(_row_mean(xc * xc) + EPS)
        wrote(stat_s[3], 't')

    def norm2_apply(b, rows):
        xc = x1_s[base + b % 3, rows] - stat(2, b, rows)
        h2 = xc * stat(3, b, rows) * (1.0 + mod(4))
        h2_s[b % 2][1, rows] = h2
        wrote(h2_s[b % 2], 'h')

    def tied(words):
        if written:
            top = words[0:8, 0:L]
            for ref in written:
                top = top | pltpu.bitcast(ref[base, 0:8, 0:L], jnp.uint32)
            written.clear()
            if words.shape[1] > L:
                top = jnp.concatenate([top, words[0:8, L:]], axis=1)
            words = jnp.concatenate([top, words[8:]], axis=0)
        return pltpu.bitcast(words, _BF16)

    def weight(ref, tile, rows):
        return tied(ref.bitcast(jnp.uint32)[tile, rows.start // 2:rows.stop // 2])

    live = {}

    def ffn_gate(blocks, f):
        first = blocks[0] == 0
        if f == 0:
            h2 = jnp.concatenate([h2_s[b % 2][base + 1] for b in blocks], axis=0)
            live["h2"] = (h2 + mod(3)).astype(_BF16)
        if first and f in dict(W13_GROUPS):
            wait(*[(w, j) for j in range(f, dict(W13_GROUPS)[f]) for w in ("w1", "w3")],
                 *([("q", 2)] if f == W13_GROUPS[1][0] else []))
        live["gate"] = _dot(live["h2"], weight(w1_v, f, slice(0, D)))
        mark(live["gate"])

    def ffn_up(blocks, f):
        up = _dot(live["h2"], weight(w3_v, f, slice(0, D)))
        mark(up)
        live["act", f] = (_silu(live.pop("gate")) * up).astype(_BF16)

    def ffn_down(blocks, n, kk):
        first = blocks[0] == 0
        if first and n == 0 and kk == 0:
            wait(*[("w2", j) for j in range(ND)], ("wm", 5), ("k", CONV_AT[2]), ("v", CONV_AT[2]))
            compute_mod(5)
        act = jnp.concatenate([live["act", kk * KT + j] for j in range(KT)], axis=1)
        o = _dot(act, weight(w2_v, n, slice(kk * KT * L, (kk + 1) * KT * L)))
        mark(o)
        if kk > 0:
            o = live.pop("out") + o
        if kk + 1 < NF // KT:
            live["out"] = o
            return
        cols = slice(n * L, (n + 1) * L)
        for j, b in enumerate(blocks):
            res = x1_s[base + b % 3, :, cols] + mod(5)[:, cols] * o[j * R:(j + 1) * R]
            out_v[b * R:(b + 1) * R, cols] = res.astype(_BF16)

    out_copies = []

    def send_out(b):
        first = max([s + 1 for s in SEND_AT if s < b], default=0)
        rows = pl.ds(first * R, (b + 1 - first) * R)
        cp = pltpu.make_async_copy(out_v.at[rows, :], out_hbm.at[rows, :], out_sems.at[b])
        cp.start()
        out_copies.append(cp)

    def ffn_steps(blocks):
        steps = []
        for f in range(NF):
            steps += [lambda f=f: ffn_gate(blocks, f), lambda f=f: ffn_up(blocks, f)]
        steps += [lambda n=n, kk=kk: ffn_down(blocks, n, kk)
                  for n in range(ND) for kk in range(NF // KT)]
        return steps

    def short_conv_steps(b):
        return ([(lambda r0=r0: widen_k(r0), 2 * RW * ND // 8)
                 for r0 in range(b * R, (b + 1) * R, RW)]
                + [(lambda i=i, p=p: short_conv(i, p), 9 * RP * ND // 8)
                   for i in range(b * CPB, (b + 1) * CPB) for p in range(C // RP)])

    def mac_steps(b):
        cost = sum(j + 1 for j in range(b * CPB, (b + 1) * CPB)) * 16
        return [(lambda g=g, n=n: mac(b, g, n), cost)
                for g in range(C // 16) for n in range(ND)]

    def norm_passes(b, rn=RN):
        return [[(lambda p=p, fn=fn: fn(b, slice(p * rn, (p + 1) * rn)), ops * rn * ND // 8)
                 for p in range(R // rn)]
                for fn, ops in ((norm1_mean, 2), (norm1_scale, 5), (residual, 9),
                                (norm2_scale, 4), (norm2_apply, 5))]

    def transform_steps(b):
        return [(lambda i=i, fn=fn: fn(i), 0)
                for fn in (ssm_transform, kv_transform) for i in range(b * CPB, (b + 1) * CPB)]

    def pipeline_step(*blocks):
        b = blocks[-1]
        main = ffn_steps(blocks)
        sizes = [ND] * (2 * NF) + [KT] * (len(main) - 2 * NF)
        slots = [[] for _ in main]
        if b in CONV_AT:
            for step, at in zip(transform_steps(CONV_AT[b]), XFORM_AT):
                slots[at].append(step)
        if b + 1 < NB:
            for jj in range(CPB):
                slots[INV0 + jj].append((lambda jj=jj: inverse_transform(b + 1, jj), 0))
            late = 2 * W13_GROUPS[1][0] if b == 1 else 0
            for steps, (first, stop) in zip(norm_passes(b + 1), NORM_AT):
                _spread(slots, steps, late + first, late + stop)
        if b + 1 in CONV_AT:
            first, stop = (2 * NF, len(main)) if b == 1 else (SC0, SC1)
            _spread(slots, short_conv_steps(CONV_AT[b + 1]), first, stop)
        macs = [step for blk, lo, hi in MAC_AT.get(b, ()) for step in mac_steps(blk)[lo:hi]]
        if macs:
            fresh = MAC_AT[b][0][0] == CONV_AT.get(b)
            _fill(slots, sizes, macs, XFORM_AT[-1] + MAC_LAG if fresh else 0)
        for step, side in zip(main, slots):
            step()
            for extra, _ in side:
                extra()
        if b in SEND_AT:
            send_out(b)

    def run(steps):
        for step, _ in steps:
            step()

    wait("fwd", "shift", "d", "c", "inv")
    def norms(first, stop):
        for k in range(first, stop):
            for b in range(2):
                run(norm_passes(b, R)[k])

    for r in range(NPRO + 2):
        if r < NPRO:
            wait(("k", r), ("v", r), ("sk", r))
        elif r == NPRO:
            wait(("q", 0), ("q", 1))
            norms(0, 2)
        else:
            wait(("wm", 1), ("wm", 0), ("wm", 2))
            for j in (1, 0, 2):
                compute_mod(j)
            norms(2, 4)
        if 1 <= r <= NPRO:
            run(transform_steps(r - 1)[CPB:])
        if r < NPRO:
            run(transform_steps(r)[:CPB] + short_conv_steps(r))
        if 3 <= r < 5:
            for jj in range(CPB):
                inverse_transform(r - 3, jj)
        if 2 <= r < MPRO + 2:
            run(mac_steps(r - 2))
        written.clear()
    wait(("wm", 4))
    compute_mod(4)
    norms(4, 5)
    wait(("wm", 3))
    compute_mod(3)
    pipeline_step(0, 1)
    for b in range(2, NB):
        needs = [("q", b + 1)] if b + 1 < NB else []
        if b in CONV_AT:
            needs += [("sk", CONV_AT[b])]
        if b + 1 in CONV_AT:
            needs += [("k", CONV_AT[b + 1]), ("v", CONV_AT[b + 1])]
        wait(*needs)
        pipeline_step(b)
    for cp in out_copies:
        cp.wait()


@jax.jit
def pallas_adaLN_cond__ssm_conv_h3__glu_gated_swiglu__prompt_kernel(
    A_q: jax.Array,
    A_k: jax.Array,
    A_v: jax.Array,
    A_shift_k: jax.Array,
    A_ssm_k: jax.Array,
    A_ssm_D: jax.Array,
    B_x: jax.Array,
    B_w1: jax.Array,
    B_w3: jax.Array,
    B_w2: jax.Array,
    c: jax.Array,
    w_mod: jax.Array,
):
    del B_x
    B, S, D = A_q.shape
    FH = B_w1.shape[1]
    KS = A_shift_k.shape[1]
    assert B == 1 and S % R == 0 and FH % (KT * L) == 0 and D % L == 0 and KS <= HALO + 1
    NB, CPB = S // R, R // C
    NF, ND = FH // L, D // L
    n_in = 6 + 4 * NB + 6 + 2 * NF + ND

    hbm = pl.BlockSpec(memory_space=pl.ANY)
    out = pl.pallas_call(
        _kernel,
        out_shape=jax.ShapeDtypeStruct((S, D), A_q.dtype),
        in_specs=[hbm] * 14,
        out_specs=hbm,
        scratch_shapes=[
            pltpu.VMEM((S, D), _BF16),
            pltpu.VMEM((S, D), _BF16),
            pltpu.VMEM((S, D), _BF16),
            pltpu.VMEM((KS, D), _BF16),
            pltpu.VMEM((D, S), _BF16),
            pltpu.VMEM((D,), _BF16),
            pltpu.VMEM((NF, D, L), _BF16),
            pltpu.VMEM((NF, D, L), _BF16),
            pltpu.VMEM((ND, FH, L), _BF16),
            pltpu.VMEM((1, D), _BF16),
            pltpu.VMEM((6, D, D), _BF16),
            pltpu.VMEM(_FWD.shape, jnp.uint32),
            pltpu.VMEM(_INV.shape, jnp.uint32),
            pltpu.SMEM((1,), jnp.int32),
            pltpu.VMEM((ND, HALO + S, L), _F32),
            [pltpu.VMEM((CPB + 1, C, D), _F32)] * NB,
            [pltpu.VMEM((CPB, 2 * C, D), _F32)] * NB,
            [pltpu.VMEM((CPB, 2 * C, D), _F32)] * NB,
            [pltpu.VMEM((1, 2 * C, D), _F32)] * 2,
            [pltpu.VMEM((CPB + 1, 2 * C, D), _F32)] * NB,
            [pltpu.VMEM((ND, R, L), _F32)] * NB,
            pltpu.VMEM((8, 6 * D), _F32),
            [pltpu.VMEM((3, R, L), _F32)] * 4,
            [pltpu.VMEM((2, 8, L), _F32)] * 8,
            pltpu.VMEM((3, R, D), _F32),
            [pltpu.VMEM((2, R, D), _F32)] * 2,
            pltpu.VMEM((S, D), _BF16),
            pltpu.SemaphoreType.DMA((n_in,)),
            pltpu.SemaphoreType.DMA((NB,)),
        ],
        compiler_params=pltpu.CompilerParams(vmem_limit_bytes=120 * 1024 * 1024),
    )(
        A_q.reshape(S, D), A_k.reshape(S, D), A_v.reshape(S, D),
        A_shift_k.T, A_ssm_k, A_ssm_D,
        B_w1, B_w3, B_w2, c, w_mod,
        _FWD, _INV, np.zeros((1,), np.int32),
    )
    return out.reshape(B, S, D)
```

```python
import numpy as np

import jax
import jax.numpy as jnp
import jax.experimental.pallas as pl
import jax.experimental.pallas.tpu as pltpu

C = 128
R = 256
L = 128
HALO = 8
RW = 128
RP = 32
RN = 32
MAC_LAG = 3
MARK_LAG = 3
TIE = 'zcth'
INV0 = 0
SC0, SC1 = 14, 24
NORM_AT = ((0, 3), (2, 5), (5, 9), (8, 11), (11, 14))
XFORM_AT = (3, 5, 11, 12)
NPRO = 4
PRO_MAC = {2: (0,), 3: (1,), 4: (2,)}
CONV_AT = {2: 4, 3: 5, 4: 6, 5: 7}
MAC_AT = {1: 3, 2: 4, 3: 5, 4: 6, 5: 7}
SC1ST = 26
W13_GROUPS = ((0, 2), (2, 6), (6, 12))
KT = 4
EPS = 1e-5

_F32 = jnp.float32
_BF16 = jnp.bfloat16
_NT = (((1,), (1,)), ((), ()))


def _packed_bf16(x):
    bits = np.ascontiguousarray(x, np.float32).view(np.uint32)
    bits = (bits + 0x7FFF + ((bits >> 16) & 1)) >> 16
    return bits[0::2] | (bits[1::2] << 16)


def _dft_matrices():
    even = np.arange(0, C, 2)
    f = np.stack([even.reshape(-1, 8), C - 1 - even.reshape(-1, 8)], axis=1).reshape(-1)
    step = 2.0 * np.pi / (2 * C)
    ang = step * (f[:, None] + 0.5) * np.arange(C)[None, :]
    fwd = np.concatenate([np.cos(ang), -np.sin(ang)], axis=0)
    n = np.concatenate([even, even + 1])
    ang = step * n[:, None] * (even[None, :] + 0.5)
    inv = np.concatenate([np.cos(ang), -np.sin(ang)], axis=1) / C
    return _packed_bf16(fwd), _packed_bf16(inv)


_FWD, _INV = _dft_matrices()


def _dot(a, b):
    return jnp.dot(a, b, preferred_element_type=_F32)


def _row_mean(x, zero=None):
    acc = x[:, 0:L] if zero is None else x[:, 0:L] + zero
    for n in range(1, x.shape[1] // L):
        acc = acc + x[:, n * L:(n + 1) * L]
    m = jnp.sum(acc, axis=-1, keepdims=True) * (1.0 / x.shape[1])
    return jnp.broadcast_to(m, (x.shape[0], L))


def _silu(x):
    hx = 0.5 * x
    return hx * jnp.tanh(hx) + hx


def _spread(slots, steps, first, last):
    for k, step in enumerate(steps):
        slots[first + (k * (last - first)) // len(steps)].append(step)


def _fill(slots, sizes, steps, first):
    held = [sum(cost for _, cost in slot) for slot in slots]
    rate = (sum(held[first:]) + sum(cost for _, cost in steps)) / sum(sizes[first:])
    budget, k = 0.0, 0
    for s in range(first, len(slots)):
        budget += rate * sizes[s] - held[s]
        while k < len(steps) and (budget >= 0.5 * steps[k][1] or s == len(slots) - 1):
            slots[s].append(steps[k])
            budget -= steps[k][1]
            k += 1


def _kernel(q_hbm, k_hbm, v_hbm, shift_hbm, sk_hbm, d_hbm, w1_hbm, w3_hbm, w2_hbm,
            c_hbm, wm_hbm, fwd_hbm, inv_hbm, base_hbm, out_hbm,
            q_v, k_v, v_v, shift_v, sk_v, d_v, w1_v, w3_v, w2_v, c_v, wm_v, fwd_v, inv_v, base_sm,
            k_s, kv_s, u_s, kf_s, carry_s, z_s, y_s, mod_s, stat_s, mark_s, x1_s, h2_s, out_v,
            in_sems, out_sems):
    S, D = q_hbm.shape
    FH = w1_hbm.shape[1]
    NB = S // R
    NC = S // C
    CPB = R // C
    NF = FH // L
    ND = D // L

    copies = {}

    def start(name, src, dst):
        cp = pltpu.make_async_copy(src, dst, in_sems.at[len(copies)])
        cp.start()
        copies[name] = cp

    def start_ssm(b):
        cols = pl.ds(b * R, R)
        start(("sk", b), sk_hbm.at[:, cols], sk_v.at[:, cols])

    def start_kv(b):
        rows = pl.ds(b * R, R)
        start(("k", b), k_hbm.at[rows, :], k_v.at[rows, :])
        start(("v", b), v_hbm.at[rows, :], v_v.at[rows, :])

    def start_q(b):
        rows = pl.ds(b * R, R)
        start(("q", b), q_hbm.at[rows, :], q_v.at[rows, :])

    start("base", base_hbm, base_sm)
    start("fwd", fwd_hbm, fwd_v)
    start("shift", shift_hbm, shift_v)
    start("d", d_hbm, d_v)
    def start_mod(j, count):
        cols = pl.ds(j * D, count * D)
        start(("wm", j), wm_hbm.at[:, cols], wm_v.at[:, cols])

    for b in range(NPRO):
        start_kv(b)
        start_ssm(b)
    start_q(0)
    start_q(1)
    start("c", c_hbm, c_v)
    start("inv", inv_hbm, inv_v)
    start_mod(0, 3)
    start_mod(3, 2)
    for f in range(NF):
        start(("w1", f), w1_hbm.at[:, pl.ds(f * L, L)], w1_v.at[f])
        start(("w3", f), w3_hbm.at[:, pl.ds(f * L, L)], w3_v.at[f])
        if f + 1 == W13_GROUPS[0][1]:
            start_q(2)
    for n in range(ND):
        start(("w2", n), w2_hbm.at[:, pl.ds(n * L, L)], w2_v.at[n])
    start_mod(5, 1)
    for b in range(1, NB - 1):
        if b > 1:
            start_q(b + 1)
        if b in CONV_AT:
            start_ssm(CONV_AT[b])
        if b + 1 in CONV_AT:
            start_kv(CONV_AT[b + 1])

    copies["base"].wait()
    base = base_sm[0]

    def fence():
        @pl.loop(0, base + 1)
        def _(i):
            mark_s[0][1] = jnp.zeros((8, L), _F32)

    def wait(*names):
        for name in names:
            copies[name].wait()
        fence()

    for ref in (*z_s, *kv_s):
        ref[0, 0:8, 0:L] = jnp.zeros((8, L), _F32)
    for ref in stat_s:
        ref[0, 0:8] = jnp.zeros((8, L), _F32)
    for ref in h2_s:
        ref[0, 0:8, 0:L] = jnp.zeros((8, L), _F32)
    k_s[:, 0:HALO] = jnp.zeros((ND, HALO, L), _F32)

    written = []

    def wrote(ref, slot):
        if slot in TIE and not any(ref is r for r in written):
            written.append(ref)

    emitted = [0]

    def mark(result):
        mark_s[emitted[0] % len(mark_s)][1] = result[0:8, 0:L]
        emitted[0] += 1

    def after_mark(lag=MARK_LAG):
        return mark_s[(emitted[0] - 1 - lag) % len(mark_s)][base, 0:1]

    for ref in mark_s:
        ref[0] = jnp.zeros((8, L), _F32)

    def mod(j):
        return mod_s[0:1, j * D:(j + 1) * D]

    def compute_mod(j):
        sc = _silu(c_v[...].astype(_F32)).astype(_BF16)
        sc = jnp.broadcast_to(sc, (16, D))
        mod_s[:, j * D:(j + 1) * D] = _dot(sc, wm_v[:, j * D:(j + 1) * D])[0:8]

    def ssm_transform(m):
        spec = jax.lax.dot_general(tied(fwd_v[...]), sk_v[:, m * C:(m + 1) * C], _NT,
                                   preferred_element_type=_F32)
        if m == 0:
            kf_s[0][0, 0:C] = spec[0:C] + d_v[...].astype(_F32).reshape(1, D)
            kf_s[0][0, C:2 * C] = spec[C:2 * C]
        else:
            kf_s[m // CPB][m % CPB] = spec

    def widen_k(r0):
        kk = k_v[r0:r0 + RW, :].astype(_F32) + jnp.tile(after_mark(), (1, ND))
        for n in range(ND):
            k_s[n, HALO + r0:HALO + r0 + RW] = kk[:, n * L:(n + 1) * L]

    def short_conv(i, p):
        r0 = i * C + p * RP
        w = shift_v[...].astype(_F32)
        ks = None
        for j in range(w.shape[0]):
            kj = jnp.concatenate([k_s[base + n, HALO + r0 - j:HALO + r0 - j + RP]
                                  for n in range(ND)], axis=1)
            ks = kj * w[j:j + 1] if ks is None else ks + kj * w[j:j + 1]
        kv_s[i // CPB][1 + i % CPB, p * RP:(p + 1) * RP] = ks * v_v[r0:r0 + RP, :].astype(_F32)
        wrote(kv_s[i // CPB], 'c')

    def kv_transform(i):
        kv = kv_s[i // CPB][base + (1 + i % CPB)].astype(_BF16)
        u_s[i // CPB][i % CPB] = _dot(tied(fwd_v[...]), kv)

    def mac(b, g, n):
        chunks = range(b * CPB, (b + 1) * CPB)
        re = pl.ds(16 * g, 16)
        im = pl.ds(C + 16 * g, 16)
        ln = slice(n * L, (n + 1) * L)

        def tile(refs, i):
            return refs[i // CPB][base + i % CPB, re, ln], refs[i // CPB][base + i % CPB, im, ln]

        acc = {}
        kf = {}
        for i in range(chunks[-1] + 1):
            ur, ui = tile(u_s, i)
            for j in chunks:
                if j < i:
                    continue
                if j - i not in kf:
                    kf[j - i] = tile(kf_s, j - i)
                kr, ki = kf[j - i]
                pr, pi = kr * ur - ki * ui, kr * ui + ki * ur
                acc[j] = (acc[j][0] + pr, acc[j][1] + pi) if j in acc else (pr, pi)
        if b > 0:
            carry = carry_s[(b - 1) % 2]
            acc[chunks[0] - 1] = (carry[base, re, ln], carry[base, im, ln])
        if b + 1 < NB:
            carry_s[b % 2][0, re, ln], carry_s[b % 2][0, im, ln] = acc[chunks[-1]]
        for j in chunks:
            (ar, br), (ai, bi) = ((x[0:8], x[8:16]) for x in acc[j])
            if j > 0:
                pr, pi = acc[j - 1]
                ar, ai = ar - pi[0:8], ai + pr[0:8]
                br, bi = br + pi[8:16], bi - pr[8:16]
            for k, x in enumerate((ar + br, ai - bi, ar - br, ai + bi)):
                z_s[b][1 + j % CPB, pl.ds(k * (C // 2) + 8 * g, 8), ln] = x
        wrote(z_s[b], 'z')

    def inverse_transform(b, jj):
        for odd in range(2):
            z = z_s[b][base + (1 + jj), odd * C:(odd + 1) * C].astype(_BF16)
            y = _dot(tied(inv_v[odd * C // 4:(odd + 1) * C // 4]), z)
            for n in range(ND):
                y_s[b][n, pl.ds(jj * C + odd, C // 2, stride=2), :] = y[:, n * L:(n + 1) * L]

    def stat(k, b, rows):
        s = stat_s[k][base + (1 + b % 2), rows]
        return jnp.tile(s + after_mark() if k % 2 == 0 else s, (1, ND))

    def q_rows(b, rows):
        return q_v[b * R + rows.start:b * R + rows.stop, :].astype(_F32)

    def norm1_mean(b, rows):
        stat_s[0][1 + b % 2, rows] = _row_mean(q_rows(b, rows), after_mark())
        wrote(stat_s[0], 't')

    def norm1_scale(b, rows):
        xc = q_rows(b, rows) - stat(0, b, rows)
        stat_s[1][1 + b % 2, rows] = jax.lax.rsqrt(_row_mean(xc * xc) + EPS)
        wrote(stat_s[1], 't')

    def residual(b, rows):
        x = q_rows(b, rows)
        y = jnp.concatenate([y_s[b][base + n, rows] for n in range(ND)], axis=1)
        h = (x - stat(0, b, rows)) * stat(1, b, rows) * (1.0 + mod(1)) + mod(0)
        x1 = x + mod(2) * (h * y)
        x1_s[b % 3, rows] = x1
        stat_s[2][1 + b % 2, rows] = _row_mean(x1)
        wrote(stat_s[2], 't')

    def norm2_scale(b, rows):
        xc = x1_s[base + b % 3, rows] - stat(2, b, rows)
        stat_s[3][1 + b % 2, rows] = jax.lax.rsqrt(_row_mean(xc * xc) + EPS)
        wrote(stat_s[3], 't')

    def norm2_apply(b, rows):
        xc = x1_s[base + b % 3, rows] - stat(2, b, rows)
        h2 = xc * stat(3, b, rows) * (1.0 + mod(4))
        h2_s[b % 2][1, rows] = h2
        wrote(h2_s[b % 2], 'h')

    def tied(words):
        if written:
            top = words[0:8, 0:L]
            for ref in written:
                top = top | pltpu.bitcast(ref[base, 0:8, 0:L], jnp.uint32)
            written.clear()
            if words.shape[1] > L:
                top = jnp.concatenate([top, words[0:8, L:]], axis=1)
            words = jnp.concatenate([top, words[8:]], axis=0)
        return pltpu.bitcast(words, _BF16)

    def weight(ref, tile, rows):
        return tied(ref.bitcast(jnp.uint32)[tile, rows.start // 2:rows.stop // 2])

    live = {}

    def ffn_gate(blocks, f):
        first = blocks[0] == 0
        if f == 0:
            h2 = jnp.concatenate([h2_s[b % 2][base + 1] for b in blocks], axis=0)
            live["h2"] = (h2 + mod(3)).astype(_BF16)
        if first and f in dict(W13_GROUPS):
            wait(*[(w, j) for j in range(f, dict(W13_GROUPS)[f]) for w in ("w1", "w3")],
                 *([("q", 2)] if f == W13_GROUPS[1][0] else []))
        live["gate"] = _dot(live["h2"], weight(w1_v, f, slice(0, D)))
        mark(live["gate"])

    def ffn_up(blocks, f):
        up = _dot(live["h2"], weight(w3_v, f, slice(0, D)))
        mark(up)
        live["act", f] = (_silu(live.pop("gate")) * up).astype(_BF16)

    def ffn_down(blocks, n, kk):
        first = blocks[0] == 0
        if first and n == 0 and kk == 0:
            wait(*[("w2", j) for j in range(ND)], ("wm", 5))
            compute_mod(5)
        act = jnp.concatenate([live["act", kk * KT + j] for j in range(KT)], axis=1)
        o = _dot(act, weight(w2_v, n, slice(kk * KT * L, (kk + 1) * KT * L)))
        mark(o)
        if kk > 0:
            o = live.pop("out") + o
        if kk + 1 < NF // KT:
            live["out"] = o
            return
        cols = slice(n * L, (n + 1) * L)
        for j, b in enumerate(blocks):
            res = x1_s[base + b % 3, :, cols] + mod(5)[:, cols] * o[j * R:(j + 1) * R]
            out_v[b * R:(b + 1) * R, cols] = res.astype(_BF16)
        if blocks[-1] + 1 == NB and n + 2 >= ND:
            send(pl.ds((NB - 1) * R, R), pl.ds(0, (ND - 1) * L) if n + 2 == ND else pl.ds(n * L, L))

    out_copies = []

    def send(rows, cols):
        cp = pltpu.make_async_copy(out_v.at[rows, cols], out_hbm.at[rows, cols],
                                   out_sems.at[len(out_copies)])
        cp.start()
        out_copies.append(cp)

    def ffn_steps(blocks):
        steps = []
        for f in range(NF):
            steps += [lambda f=f: ffn_gate(blocks, f), lambda f=f: ffn_up(blocks, f)]
        steps += [lambda n=n, kk=kk: ffn_down(blocks, n, kk)
                  for n in range(ND) for kk in range(NF // KT)]
        return steps

    def short_conv_steps(b):
        return ([(lambda r0=r0: widen_k(r0), 2 * RW * ND // 8)
                 for r0 in range(b * R, (b + 1) * R, RW)]
                + [(lambda i=i, p=p: short_conv(i, p), 9 * RP * ND // 8)
                   for i in range(b * CPB, (b + 1) * CPB) for p in range(C // RP)])

    def mac_steps(b):
        cost = sum(j + 1 for j in range(b * CPB, (b + 1) * CPB)) * 16
        return [(lambda g=g, n=n: mac(b, g, n), cost)
                for g in range(C // 16) for n in range(ND)]

    def norm_passes(b, rn=RN):
        return [[(lambda p=p, fn=fn: fn(b, slice(p * rn, (p + 1) * rn)), ops * rn * ND // 8)
                 for p in range(R // rn)]
                for fn, ops in ((norm1_mean, 2), (norm1_scale, 5), (residual, 9),
                                (norm2_scale, 4), (norm2_apply, 5))]

    def transform_steps(b):
        return [(lambda i=i, fn=fn: fn(i), 0)
                for fn in (ssm_transform, kv_transform) for i in range(b * CPB, (b + 1) * CPB)]

    def pipeline_step(*blocks):
        b = blocks[-1]
        main = ffn_steps(blocks)
        sizes = [ND] * (2 * NF) + [KT] * (len(main) - 2 * NF)
        slots = [[] for _ in main]
        if b in CONV_AT:
            for step, at in zip(transform_steps(CONV_AT[b]), XFORM_AT):
                slots[at].append(step)
        if b + 1 < NB:
            for jj in range(CPB):
                slots[INV0 + jj].append((lambda jj=jj: inverse_transform(b + 1, jj), 0))
            late = 2 * W13_GROUPS[1][0] if b == 1 else 0
            for steps, (first, stop) in zip(norm_passes(b + 1), NORM_AT):
                _spread(slots, steps, late + first, late + stop)
        if b + 1 in CONV_AT:
            first, stop = (SC1ST, len(main)) if b == 1 else (SC0, SC1)
            if b == 1:
                for name in ("k", "v"):
                    slots[first].append((copies[name, CONV_AT[2]].wait, 0))
            _spread(slots, short_conv_steps(CONV_AT[b + 1]), first, stop)
        if b in MAC_AT:
            first = XFORM_AT[-1] + MAC_LAG if MAC_AT[b] == CONV_AT.get(b) else 0
            _fill(slots, sizes, mac_steps(MAC_AT[b]), first)
        for step, side in zip(main, slots):
            step()
            for extra, _ in side:
                extra()
        if b + 1 < NB:
            send(pl.ds(blocks[0] * R, len(blocks) * R), pl.ds(0, D))

    def run(steps):
        for step, _ in steps:
            step()

    wait("fwd", "shift", "d")
    def norms(first, stop):
        for k in range(first, stop):
            for b in range(2):
                run(norm_passes(b, R)[k])

    for r in range(NPRO + 2):
        if r < NPRO:
            wait(("k", r), ("v", r), ("sk", r))
        elif r == NPRO:
            wait(("q", 0), ("q", 1), "c", "inv")
            norms(0, 2)
        else:
            wait(("wm", 0))
            for j in (1, 0, 2):
                compute_mod(j)
            norms(2, 4)
        if 1 <= r <= NPRO:
            run(transform_steps(r - 1)[CPB:])
        if r < NPRO:
            run(transform_steps(r)[:CPB] + short_conv_steps(r))
        for b in PRO_MAC.get(r, ()):
            run(mac_steps(b))
        if r == NPRO:
            for b in range(2):
                for jj in range(CPB):
                    inverse_transform(b, jj)
        written.clear()
    wait(("wm", 3))
    compute_mod(4)
    compute_mod(3)
    norms(4, 5)
    pipeline_step(0, 1)
    for b in range(2, NB):
        needs = [("q", b + 1)] if b + 1 < NB else []
        if b in CONV_AT:
            needs += [("sk", CONV_AT[b])]
        if b + 1 in CONV_AT:
            needs += [("k", CONV_AT[b + 1]), ("v", CONV_AT[b + 1])]
        wait(*needs)
        pipeline_step(b)
    for cp in out_copies:
        cp.wait()


@jax.jit
def pallas_adaLN_cond__ssm_conv_h3__glu_gated_swiglu__prompt_kernel(
    A_q: jax.Array,
    A_k: jax.Array,
    A_v: jax.Array,
    A_shift_k: jax.Array,
    A_ssm_k: jax.Array,
    A_ssm_D: jax.Array,
    B_x: jax.Array,
    B_w1: jax.Array,
    B_w3: jax.Array,
    B_w2: jax.Array,
    c: jax.Array,
    w_mod: jax.Array,
):
    del B_x
    B, S, D = A_q.shape
    FH = B_w1.shape[1]
    KS = A_shift_k.shape[1]
    assert B == 1 and S % R == 0 and FH % (KT * L) == 0 and D % L == 0 and KS <= HALO + 1
    NB, CPB = S // R, R // C
    NF, ND = FH // L, D // L
    n_in = 6 + 4 * NB + 3 + 2 * NF + ND

    hbm = pl.BlockSpec(memory_space=pl.ANY)
    out = pl.pallas_call(
        _kernel,
        out_shape=jax.ShapeDtypeStruct((S, D), A_q.dtype),
        in_specs=[hbm] * 14,
        out_specs=hbm,
        scratch_shapes=[
            pltpu.VMEM((S, D), _BF16),
            pltpu.VMEM((S, D), _BF16),
            pltpu.VMEM((S, D), _BF16),
            pltpu.VMEM((KS, D), _BF16),
            pltpu.VMEM((D, S), _BF16),
            pltpu.VMEM((D,), _BF16),
            pltpu.VMEM((NF, D, L), _BF16),
            pltpu.VMEM((NF, D, L), _BF16),
            pltpu.VMEM((ND, FH, L), _BF16),
            pltpu.VMEM((1, D), _BF16),
            pltpu.VMEM((D, 6 * D), _BF16),
            pltpu.VMEM(_FWD.shape, jnp.uint32),
            pltpu.VMEM(_INV.shape, jnp.uint32),
            pltpu.SMEM((1,), jnp.int32),
            pltpu.VMEM((ND, HALO + S, L), _F32),
            [pltpu.VMEM((CPB + 1, C, D), _F32)] * NB,
            [pltpu.VMEM((CPB, 2 * C, D), _F32)] * NB,
            [pltpu.VMEM((CPB, 2 * C, D), _F32)] * NB,
            [pltpu.VMEM((1, 2 * C, D), _F32)] * 2,
            [pltpu.VMEM((CPB + 1, 2 * C, D), _F32)] * NB,
            [pltpu.VMEM((ND, R, L), _F32)] * NB,
            pltpu.VMEM((8, 6 * D), _F32),
            [pltpu.VMEM((3, R, L), _F32)] * 4,
            [pltpu.VMEM((2, 8, L), _F32)] * 8,
            pltpu.VMEM((3, R, D), _F32),
            [pltpu.VMEM((2, R, D), _F32)] * 2,
            pltpu.VMEM((S, D), _BF16),
            pltpu.SemaphoreType.DMA((n_in,)),
            pltpu.SemaphoreType.DMA((NB,)),
        ],
        compiler_params=pltpu.CompilerParams(vmem_limit_bytes=120 * 1024 * 1024),
    )(
        A_q.reshape(S, D), A_k.reshape(S, D), A_v.reshape(S, D),
        A_shift_k.T, A_ssm_k, A_ssm_D,
        B_w1, B_w3, B_w2, c, w_mod,
        _FWD, _INV, np.zeros((1,), np.int32),
    )
    return out.reshape(B, S, D)
```

```python
import numpy as np

import jax
import jax.numpy as jnp
import jax.experimental.pallas as pl
import jax.experimental.pallas.tpu as pltpu

C = 128
R = 256
L = 128
HALO = 8
RW = 128
RP = 32
RN = 32
MAC_LAG = 3
MARK_LAG = 3
TIE = 'zc'
INV0 = 0
SC0, SC1 = 14, 24
NORM_AT = ((0, 3), (2, 5), (5, 9), (8, 11), (11, 14))
XFORM_AT = (3, 5, 11, 12)
NPRO = 4
PRO_MAC = {2: (0,), 3: (1,), 4: (2,)}
CONV_AT = {2: 4, 3: 5, 4: 6, 5: 7}
MAC_AT = {1: 3, 2: 4, 3: 5, 4: 6, 5: 7}
SC_FIRST = (25, 39)
MAC_FIRST = (4, 39)
NORM_FIRST = ((4, 8), (7, 12), (12, 17), (16, 20), (19, 24))
NORM_WIDE = ((0, 8), (6, 14), (14, 22), (21, 29), (28, 36))
W13_GROUPS = ((0, 2), (2, 6), (6, 12))
KT = 4
EPS = 1e-5

_F32 = jnp.float32
_BF16 = jnp.bfloat16
_NT = (((1,), (1,)), ((), ()))


def _packed_bf16(x):
    bits = np.ascontiguousarray(x, np.float32).view(np.uint32)
    bits = (bits + 0x7FFF + ((bits >> 16) & 1)) >> 16
    return bits[0::2] | (bits[1::2] << 16)


def _dft_matrices():
    even = np.arange(0, C, 2)
    f = np.stack([even.reshape(-1, 8), C - 1 - even.reshape(-1, 8)], axis=1).reshape(-1)
    step = 2.0 * np.pi / (2 * C)
    ang = step * (f[:, None] + 0.5) * np.arange(C)[None, :]
    fwd = np.concatenate([np.cos(ang), -np.sin(ang)], axis=0)
    n = np.concatenate([even, even + 1])
    ang = step * n[:, None] * (even[None, :] + 0.5)
    inv = np.concatenate([np.cos(ang), -np.sin(ang)], axis=1) / C
    return _packed_bf16(fwd), _packed_bf16(inv)


_FWD, _INV = _dft_matrices()


def _dot(a, b):
    return jnp.dot(a, b, preferred_element_type=_F32)


def _row_mean(x, zero=None):
    acc = x[:, 0:L] if zero is None else x[:, 0:L] + zero
    for n in range(1, x.shape[1] // L):
        acc = acc + x[:, n * L:(n + 1) * L]
    m = jnp.sum(acc, axis=-1, keepdims=True) * (1.0 / x.shape[1])
    return jnp.broadcast_to(m, (x.shape[0], L))


def _silu(x):
    hx = 0.5 * x
    return hx * jnp.tanh(hx) + hx


def _spread(slots, steps, first, last):
    for k, step in enumerate(steps):
        slots[first + (k * (last - first)) // len(steps)].append(step)


def _fill(slots, sizes, steps, first):
    held = [sum(cost for _, cost in slot) for slot in slots]
    rate = (sum(held[first:]) + sum(cost for _, cost in steps)) / sum(sizes[first:])
    budget, k = 0.0, 0
    for s in range(first, len(slots)):
        budget += rate * sizes[s] - held[s]
        while k < len(steps) and (budget >= 0.5 * steps[k][1] or s == len(slots) - 1):
            slots[s].append(steps[k])
            budget -= steps[k][1]
            k += 1


def _kernel(q_hbm, k_hbm, v_hbm, shift_hbm, sk_hbm, d_hbm, w1_hbm, w3_hbm, w2_hbm,
            c_hbm, wm_hbm, fwd_hbm, inv_hbm, base_hbm, out_hbm,
            q_v, k_v, v_v, shift_v, sk_v, d_v, w1_v, w3_v, w2_v, c_v, wm_v, fwd_v, inv_v, base_sm,
            k_s, kv_s, u_s, kf_s, carry_s, z_s, y_s, mod_s, stat_s, mark_s, x1_s, h2_s, out_v,
            in_sems, out_sems):
    S, D = q_hbm.shape
    FH = w1_hbm.shape[1]
    NB = S // R
    NC = S // C
    CPB = R // C
    NF = FH // L
    ND = D // L

    copies = {}

    def start(name, src, dst):
        cp = pltpu.make_async_copy(src, dst, in_sems.at[len(copies)])
        cp.start()
        copies[name] = cp

    def start_ssm(b):
        cols = pl.ds(b * R, R)
        start(("sk", b), sk_hbm.at[:, cols], sk_v.at[:, cols])

    def start_kv(b):
        rows = pl.ds(b * R, R)
        start(("k", b), k_hbm.at[rows, :], k_v.at[rows, :])
        start(("v", b), v_hbm.at[rows, :], v_v.at[rows, :])

    def start_q(b):
        rows = pl.ds(b * R, R)
        start(("q", b), q_hbm.at[rows, :], q_v.at[rows, :])

    start("base", base_hbm, base_sm)
    start("fwd", fwd_hbm, fwd_v)
    start("shift", shift_hbm, shift_v)
    start("d", d_hbm, d_v)
    def start_mod(j, count):
        cols = pl.ds(j * D, count * D)
        start(("wm", j), wm_hbm.at[:, cols], wm_v.at[:, cols])

    for b in range(NPRO):
        start_kv(b)
        start_ssm(b)
    start_q(0)
    start_q(1)
    start("c", c_hbm, c_v)
    start("inv", inv_hbm, inv_v)
    start_mod(0, 3)
    start_mod(3, 2)
    for f in range(NF):
        start(("w1", f), w1_hbm.at[:, pl.ds(f * L, L)], w1_v.at[f])
        start(("w3", f), w3_hbm.at[:, pl.ds(f * L, L)], w3_v.at[f])
        if f + 1 == W13_GROUPS[0][1]:
            start_q(2)
    start_kv(CONV_AT[2])
    for n in range(ND):
        start(("w2", n), w2_hbm.at[:, pl.ds(n * L, L)], w2_v.at[n])
    start_mod(5, 1)
    for b in range(1, NB - 1):
        if b > 1:
            start_q(b + 1)
        if b in CONV_AT:
            start_ssm(CONV_AT[b])
        if b > 1 and b + 1 in CONV_AT:
            start_kv(CONV_AT[b + 1])

    copies["base"].wait()
    base = base_sm[0]

    def fence():
        @pl.loop(0, base + 1)
        def _(i):
            mark_s[0][1] = jnp.zeros((8, L), _F32)

    def wait(*names):
        for name in names:
            copies[name].wait()
        fence()

    for ref in (*z_s, *kv_s):
        ref[0, 0:8, 0:L] = jnp.zeros((8, L), _F32)
    for ref in stat_s:
        ref[0, 0:8] = jnp.zeros((8, L), _F32)
    for ref in h2_s:
        ref[0, 0:8, 0:L] = jnp.zeros((8, L), _F32)
    k_s[:, 0:HALO] = jnp.zeros((ND, HALO, L), _F32)

    written = []

    def wrote(ref, slot):
        if slot in TIE and not any(ref is r for r in written):
            written.append(ref)

    emitted = [0]

    def mark(result):
        mark_s[emitted[0] % len(mark_s)][1] = result[0:8, 0:L]
        emitted[0] += 1

    def after_mark(lag=MARK_LAG):
        return mark_s[(emitted[0] - 1 - lag) % len(mark_s)][base, 0:1]

    for ref in mark_s:
        ref[0] = jnp.zeros((8, L), _F32)

    def mod(j):
        return mod_s[0:1, j * D:(j + 1) * D]

    def compute_mod(j):
        sc = _silu(c_v[...].astype(_F32)).astype(_BF16)
        sc = jnp.broadcast_to(sc, (16, D))
        mod_s[:, j * D:(j + 1) * D] = _dot(sc, wm_v[:, j * D:(j + 1) * D])[0:8]

    def ssm_transform(m):
        spec = jax.lax.dot_general(tied(fwd_v[...]), sk_v[:, m * C:(m + 1) * C], _NT,
                                   preferred_element_type=_F32)
        if m == 0:
            kf_s[0][0, 0:C] = spec[0:C] + d_v[...].astype(_F32).reshape(1, D)
            kf_s[0][0, C:2 * C] = spec[C:2 * C]
        else:
            kf_s[m // CPB][m % CPB] = spec

    def widen_k(r0):
        kk = k_v[r0:r0 + RW, :].astype(_F32) + jnp.tile(after_mark(), (1, ND))
        for n in range(ND):
            k_s[n, HALO + r0:HALO + r0 + RW] = kk[:, n * L:(n + 1) * L]

    def short_conv(i, p):
        r0 = i * C + p * RP
        w = shift_v[...].astype(_F32)
        ks = None
        for j in range(w.shape[0]):
            kj = jnp.concatenate([k_s[base + n, HALO + r0 - j:HALO + r0 - j + RP]
                                  for n in range(ND)], axis=1)
            ks = kj * w[j:j + 1] if ks is None else ks + kj * w[j:j + 1]
        kv_s[i // CPB][1 + i % CPB, p * RP:(p + 1) * RP] = ks * v_v[r0:r0 + RP, :].astype(_F32)
        wrote(kv_s[i // CPB], 'c')

    def kv_transform(i):
        kv = kv_s[i // CPB][base + (1 + i % CPB)].astype(_BF16)
        u_s[i // CPB][i % CPB] = _dot(tied(fwd_v[...]), kv)

    def mac(b, g, n):
        chunks = range(b * CPB, (b + 1) * CPB)
        re = pl.ds(16 * g, 16)
        im = pl.ds(C + 16 * g, 16)
        ln = slice(n * L, (n + 1) * L)

        def tile(refs, i):
            return refs[i // CPB][base + i % CPB, re, ln], refs[i // CPB][base + i % CPB, im, ln]

        acc = {}
        kf = {}
        for i in range(chunks[-1] + 1):
            ur, ui = tile(u_s, i)
            for j in chunks:
                if j < i:
                    continue
                if j - i not in kf:
                    kf[j - i] = tile(kf_s, j - i)
                kr, ki = kf[j - i]
                pr, pi = kr * ur - ki * ui, kr * ui + ki * ur
                acc[j] = (acc[j][0] + pr, acc[j][1] + pi) if j in acc else (pr, pi)
        if b > 0:
            carry = carry_s[(b - 1) % 2]
            acc[chunks[0] - 1] = (carry[base, re, ln], carry[base, im, ln])
        if b + 1 < NB:
            carry_s[b % 2][0, re, ln], carry_s[b % 2][0, im, ln] = acc[chunks[-1]]
        for j in chunks:
            (ar, br), (ai, bi) = ((x[0:8], x[8:16]) for x in acc[j])
            if j > 0:
                pr, pi = acc[j - 1]
                ar, ai = ar - pi[0:8], ai + pr[0:8]
                br, bi = br + pi[8:16], bi - pr[8:16]
            for k, x in enumerate((ar + br, ai - bi, ar - br, ai + bi)):
                z_s[b][1 + j % CPB, pl.ds(k * (C // 2) + 8 * g, 8), ln] = x
        wrote(z_s[b], 'z')

    def inverse_transform(b, jj):
        for odd in range(2):
            z = z_s[b][base + (1 + jj), odd * C:(odd + 1) * C].astype(_BF16)
            y = _dot(tied(inv_v[odd * C // 4:(odd + 1) * C // 4]), z)
            for n in range(ND):
                y_s[b][n, pl.ds(jj * C + odd, C // 2, stride=2), :] = y[:, n * L:(n + 1) * L]

    def stat(k, b, rows):
        s = stat_s[k][base + (1 + b % 2), rows]
        return jnp.tile(s + after_mark() if k % 2 == 0 else s, (1, ND))

    def q_rows(b, rows):
        return q_v[b * R + rows.start:b * R + rows.stop, :].astype(_F32)

    def norm1_mean(b, rows):
        stat_s[0][1 + b % 2, rows] = _row_mean(q_rows(b, rows), after_mark())
        wrote(stat_s[0], 't')

    def norm1_scale(b, rows):
        xc = q_rows(b, rows) - stat(0, b, rows)
        stat_s[1][1 + b % 2, rows] = jax.lax.rsqrt(_row_mean(xc * xc) + EPS)
        wrote(stat_s[1], 't')

    def residual(b, rows):
        x = q_rows(b, rows)
        y = jnp.concatenate([y_s[b][base + n, rows] for n in range(ND)], axis=1)
        h = (x - stat(0, b, rows)) * stat(1, b, rows) * (1.0 + mod(1)) + mod(0)
        x1 = x + mod(2) * (h * y)
        x1_s[b % 3, rows] = x1
        stat_s[2][1 + b % 2, rows] = _row_mean(x1)
        wrote(stat_s[2], 't')

    def norm2_scale(b, rows):
        xc = x1_s[base + b % 3, rows] - stat(2, b, rows)
        stat_s[3][1 + b % 2, rows] = jax.lax.rsqrt(_row_mean(xc * xc) + EPS)
        wrote(stat_s[3], 't')

    def norm2_apply(b, rows):
        xc = x1_s[base + b % 3, rows] - stat(2, b, rows)
        h2 = xc * stat(3, b, rows) * (1.0 + mod(4))
        h2_s[b % 2][1, rows] = h2
        wrote(h2_s[b % 2], 'h')

    def tied(words):
        if written:
            top = words[0:8, 0:L]
            for ref in written:
                top = top | pltpu.bitcast(ref[base, 0:8, 0:L], jnp.uint32)
            written.clear()
            if words.shape[1] > L:
                top = jnp.concatenate([top, words[0:8, L:]], axis=1)
            words = jnp.concatenate([top, words[8:]], axis=0)
        return pltpu.bitcast(words, _BF16)

    def weight(ref, tile, rows):
        return tied(ref.bitcast(jnp.uint32)[tile, rows.start // 2:rows.stop // 2])

    live = {}

    def ffn_gate(blocks, f):
        first = blocks[0] == 0
        if f == 0:
            h2 = jnp.concatenate([h2_s[b % 2][base + 1] for b in blocks], axis=0)
            live["h2"] = (h2 + mod(3)).astype(_BF16)
        if first and f in dict(W13_GROUPS):
            wait(*[(w, j) for j in range(f, dict(W13_GROUPS)[f]) for w in ("w1", "w3")],
                 *([("q", 2)] if f == W13_GROUPS[1][0] else []))
        live["gate"] = _dot(live["h2"], weight(w1_v, f, slice(0, D)))
        mark(live["gate"])

    def ffn_up(blocks, f):
        up = _dot(live["h2"], weight(w3_v, f, slice(0, D)))
        mark(up)
        live["act", f] = (_silu(live.pop("gate")) * up).astype(_BF16)

    def ffn_down(blocks, n, kk):
        first = blocks[0] == 0
        if first and n == 0 and kk == 0:
            wait(*[("w2", j) for j in range(ND)], ("wm", 5))
            compute_mod(5)
        act = jnp.concatenate([live["act", kk * KT + j] for j in range(KT)], axis=1)
        o = _dot(act, weight(w2_v, n, slice(kk * KT * L, (kk + 1) * KT * L)))
        mark(o)
        if kk > 0:
            o = live.pop("out") + o
        if kk + 1 < NF // KT:
            live["out"] = o
            return
        cols = slice(n * L, (n + 1) * L)
        for j, b in enumerate(blocks):
            res = x1_s[base + b % 3, :, cols] + mod(5)[:, cols] * o[j * R:(j + 1) * R]
            out_v[b * R:(b + 1) * R, cols] = res.astype(_BF16)
        if blocks[-1] + 1 == NB and n + 2 >= ND:
            send(pl.ds((NB - 1) * R, R), pl.ds(0, (ND - 1) * L) if n + 2 == ND else pl.ds(n * L, L))

    out_copies = []

    def send(rows, cols):
        cp = pltpu.make_async_copy(out_v.at[rows, cols], out_hbm.at[rows, cols],
                                   out_sems.at[len(out_copies)])
        cp.start()
        out_copies.append(cp)

    def ffn_steps(blocks):
        steps = []
        for f in range(NF):
            steps += [lambda f=f: ffn_gate(blocks, f), lambda f=f: ffn_up(blocks, f)]
        steps += [lambda n=n, kk=kk: ffn_down(blocks, n, kk)
                  for n in range(ND) for kk in range(NF // KT)]
        return steps

    def short_conv_steps(b):
        return ([(lambda r0=r0: widen_k(r0), 2 * RW * ND // 8)
                 for r0 in range(b * R, (b + 1) * R, RW)]
                + [(lambda i=i, p=p: short_conv(i, p), 9 * RP * ND // 8)
                   for i in range(b * CPB, (b + 1) * CPB) for p in range(C // RP)])

    def mac_steps(b):
        cost = sum(j + 1 for j in range(b * CPB, (b + 1) * CPB)) * 16
        return [(lambda g=g, n=n: mac(b, g, n), cost)
                for g in range(C // 16) for n in range(ND)]

    def norm_passes(b, rn=RN):
        return [[(lambda p=p, fn=fn: fn(b, slice(p * rn, (p + 1) * rn)), ops * rn * ND // 8)
                 for p in range(R // rn)]
                for fn, ops in ((norm1_mean, 2), (norm1_scale, 5), (residual, 9),
                                (norm2_scale, 4), (norm2_apply, 5))]

    def transform_steps(b):
        return [(lambda i=i, fn=fn: fn(i), 0)
                for fn in (ssm_transform, kv_transform) for i in range(b * CPB, (b + 1) * CPB)]

    def pipeline_step(*blocks):
        b = blocks[-1]
        main = ffn_steps(blocks)
        sizes = [ND] * (2 * NF) + [KT] * (len(main) - 2 * NF)
        slots = [[] for _ in main]
        if b in CONV_AT:
            for step, at in zip(transform_steps(CONV_AT[b]), XFORM_AT):
                slots[at].append(step)
        if b + 1 < NB:
            for jj in range(CPB):
                slots[INV0 + jj].append((lambda jj=jj: inverse_transform(b + 1, jj), 0))
            norm_at = NORM_FIRST if b == 1 else NORM_AT if b in MAC_AT else NORM_WIDE
            for steps, (first, stop) in zip(norm_passes(b + 1), norm_at):
                _spread(slots, steps, first, stop)
        if b + 1 in CONV_AT:
            first, stop = SC_FIRST if b == 1 else (SC0, SC1)
            if b == 1:
                for name in ("k", "v"):
                    slots[first].append((copies[name, CONV_AT[2]].wait, 0))
            _spread(slots, short_conv_steps(CONV_AT[b + 1]), first, stop)
        if b in MAC_AT:
            first, stop = MAC_FIRST if b == 1 else (XFORM_AT[-1] + MAC_LAG, len(slots))
            _fill(slots[:stop], sizes[:stop], mac_steps(MAC_AT[b]), first)
        for step, side in zip(main, slots):
            step()
            for extra, _ in side:
                extra()
        if b + 1 < NB:
            send(pl.ds(blocks[0] * R, len(blocks) * R), pl.ds(0, D))

    def run(steps):
        for step, _ in steps:
            step()

    wait("fwd", "shift", "d")
    def norms(first, stop):
        for k in range(first, stop):
            for b in range(2):
                run(norm_passes(b, R)[k])

    for r in range(NPRO + 2):
        if r < NPRO:
            wait(("k", r), ("v", r), ("sk", r))
        elif r == NPRO:
            wait(("q", 0), ("q", 1), "c", "inv")
            norms(0, 2)
        else:
            wait(("wm", 0))
            for j in (1, 0, 2):
                compute_mod(j)
            norms(2, 4)
        if 1 <= r <= NPRO:
            run(transform_steps(r - 1)[CPB:])
        if r < NPRO:
            run(transform_steps(r)[:CPB] + short_conv_steps(r))
        for b in PRO_MAC.get(r, ()):
            run(mac_steps(b))
        if r == NPRO:
            for b in range(2):
                for jj in range(CPB):
                    inverse_transform(b, jj)
        written.clear()
    wait(("wm", 3))
    compute_mod(4)
    compute_mod(3)
    norms(4, 5)
    pipeline_step(0, 1)
    for b in range(2, NB):
        needs = [("q", b + 1)] if b + 1 < NB else []
        if b in CONV_AT:
            needs += [("sk", CONV_AT[b])]
        if b + 1 in CONV_AT:
            needs += [("k", CONV_AT[b + 1]), ("v", CONV_AT[b + 1])]
        wait(*needs)
        pipeline_step(b)
    for cp in out_copies:
        cp.wait()


@jax.jit
def pallas_adaLN_cond__ssm_conv_h3__glu_gated_swiglu__prompt_kernel(
    A_q: jax.Array,
    A_k: jax.Array,
    A_v: jax.Array,
    A_shift_k: jax.Array,
    A_ssm_k: jax.Array,
    A_ssm_D: jax.Array,
    B_x: jax.Array,
    B_w1: jax.Array,
    B_w3: jax.Array,
    B_w2: jax.Array,
    c: jax.Array,
    w_mod: jax.Array,
):
    del B_x
    B, S, D = A_q.shape
    FH = B_w1.shape[1]
    KS = A_shift_k.shape[1]
    assert B == 1 and S % R == 0 and FH % (KT * L) == 0 and D % L == 0 and KS <= HALO + 1
    NB, CPB = S // R, R // C
    NF, ND = FH // L, D // L
    n_in = 6 + 4 * NB + 3 + 2 * NF + ND

    hbm = pl.BlockSpec(memory_space=pl.ANY)
    out = pl.pallas_call(
        _kernel,
        out_shape=jax.ShapeDtypeStruct((S, D), A_q.dtype),
        in_specs=[hbm] * 14,
        out_specs=hbm,
        scratch_shapes=[
            pltpu.VMEM((S, D), _BF16),
            pltpu.VMEM((S, D), _BF16),
            pltpu.VMEM((S, D), _BF16),
            pltpu.VMEM((KS, D), _BF16),
            pltpu.VMEM((D, S), _BF16),
            pltpu.VMEM((D,), _BF16),
            pltpu.VMEM((NF, D, L), _BF16),
            pltpu.VMEM((NF, D, L), _BF16),
            pltpu.VMEM((ND, FH, L), _BF16),
            pltpu.VMEM((1, D), _BF16),
            pltpu.VMEM((D, 6 * D), _BF16),
            pltpu.VMEM(_FWD.shape, jnp.uint32),
            pltpu.VMEM(_INV.shape, jnp.uint32),
            pltpu.SMEM((1,), jnp.int32),
            pltpu.VMEM((ND, HALO + S, L), _F32),
            [pltpu.VMEM((CPB + 1, C, D), _F32)] * NB,
            [pltpu.VMEM((CPB, 2 * C, D), _F32)] * NB,
            [pltpu.VMEM((CPB, 2 * C, D), _F32)] * NB,
            [pltpu.VMEM((1, 2 * C, D), _F32)] * 2,
            [pltpu.VMEM((CPB + 1, 2 * C, D), _F32)] * NB,
            [pltpu.VMEM((ND, R, L), _F32)] * NB,
            pltpu.VMEM((8, 6 * D), _F32),
            [pltpu.VMEM((3, R, L), _F32)] * 4,
            [pltpu.VMEM((2, 8, L), _F32)] * 8,
            pltpu.VMEM((3, R, D), _F32),
            [pltpu.VMEM((2, R, D), _F32)] * 2,
            pltpu.VMEM((S, D), _BF16),
            pltpu.SemaphoreType.DMA((n_in,)),
            pltpu.SemaphoreType.DMA((NB,)),
        ],
        compiler_params=pltpu.CompilerParams(vmem_limit_bytes=120 * 1024 * 1024),
    )(
        A_q.reshape(S, D), A_k.reshape(S, D), A_v.reshape(S, D),
        A_shift_k.T, A_ssm_k, A_ssm_D,
        B_w1, B_w3, B_w2, c, w_mod,
        _FWD, _INV, np.zeros((1,), np.int32),
    )
    return out.reshape(B, S, D)
```

```python
import numpy as np

import jax
import jax.numpy as jnp
import jax.experimental.pallas as pl
import jax.experimental.pallas.tpu as pltpu

C = 128
R = 256
L = 128
HALO = 8
RW = 128
RP = 32
RN = 32
MAC_LAG = 3
MARK_LAG = 3
TIE = 'zc'
INV0 = 0
SC0, SC1 = 14, 24
NORM_AT = ((0, 3), (2, 5), (5, 9), (8, 11), (11, 14))
XFORM_AT = (3, 5, 11, 12)
NPRO = 4
PRO_MAC = {2: (0,), 3: (1,), 4: (2,)}
CONV_AT = {2: 4, 3: 5, 4: 6, 5: 7}
MAC_AT = {1: 3, 2: 4, 3: 5, 4: 6, 5: 7}
SC_FIRST = (25, 39)
MAC_FIRST = (4, 39)
NORM_FIRST = ((4, 8), (7, 12), (12, 17), (16, 20), (19, 24))
NORM_WIDE = ((0, 8), (6, 14), (14, 22), (21, 29), (28, 36))
W13_GROUPS = ((0, 2), (2, 6), (6, 12))
KT = 4
EPS = 1e-5

_F32 = jnp.float32
_BF16 = jnp.bfloat16
_NT = (((1,), (1,)), ((), ()))


def _packed_bf16(x):
    bits = np.ascontiguousarray(x, np.float32).view(np.uint32)
    bits = (bits + 0x7FFF + ((bits >> 16) & 1)) >> 16
    return bits[0::2] | (bits[1::2] << 16)


def _dft_matrices():
    even = np.arange(0, C, 2)
    f = np.stack([even.reshape(-1, 8), C - 1 - even.reshape(-1, 8)], axis=1).reshape(-1)
    step = 2.0 * np.pi / (2 * C)
    ang = step * (f[:, None] + 0.5) * np.arange(C)[None, :]
    fwd = np.concatenate([np.cos(ang), -np.sin(ang)], axis=0)
    n = np.concatenate([even, even + 1])
    ang = step * n[:, None] * (even[None, :] + 0.5)
    inv = np.concatenate([np.cos(ang), -np.sin(ang)], axis=1) / C
    return _packed_bf16(fwd), _packed_bf16(inv)


_FWD, _INV = _dft_matrices()


def _dot(a, b):
    return jnp.dot(a, b, preferred_element_type=_F32)


def _row_mean(x, zero=None):
    acc = x[:, 0:L] if zero is None else x[:, 0:L] + zero
    for n in range(1, x.shape[1] // L):
        acc = acc + x[:, n * L:(n + 1) * L]
    m = jnp.sum(acc, axis=-1, keepdims=True) * (1.0 / x.shape[1])
    return jnp.broadcast_to(m, (x.shape[0], L))


def _silu(x):
    hx = 0.5 * x
    return hx * jnp.tanh(hx) + hx


def _spread(slots, steps, first, last):
    for k, step in enumerate(steps):
        slots[first + (k * (last - first)) // len(steps)].append(step)


def _fill(slots, sizes, steps, first):
    held = [sum(cost for _, cost in slot) for slot in slots]
    rate = (sum(held[first:]) + sum(cost for _, cost in steps)) / sum(sizes[first:])
    budget, k = 0.0, 0
    for s in range(first, len(slots)):
        budget += rate * sizes[s] - held[s]
        while k < len(steps) and (budget >= 0.5 * steps[k][1] or s == len(slots) - 1):
            slots[s].append(steps[k])
            budget -= steps[k][1]
            k += 1


def _kernel(q_hbm, k_hbm, v_hbm, shift_hbm, sk_hbm, d_hbm, w1_hbm, w3_hbm, w2_hbm,
            c_hbm, wm_hbm, fwd_hbm, inv_hbm, base_hbm, out_hbm,
            q_v, k_v, v_v, shift_v, sk_v, d_v, w1_v, w3_v, w2_v, c_v, wm_v, fwd_v, inv_v, base_sm,
            k_s, kv_s, u_s, kf_s, carry_s, z_s, y_s, mod_s, stat_s, mark_s, x1_s, h2_s, out_v,
            in_sems, out_sems):
    S, D = q_hbm.shape
    FH = w1_hbm.shape[1]
    NB = S // R
    NC = S // C
    CPB = R // C
    NF = FH // L
    ND = D // L

    copies = {}

    def start(name, src, dst):
        cp = pltpu.make_async_copy(src, dst, in_sems.at[len(copies)])
        cp.start()
        copies[name] = cp

    def start_ssm(b):
        cols = pl.ds(b * R, R)
        start(("sk", b), sk_hbm.at[:, cols], sk_v.at[:, cols])

    def start_kv(b):
        rows = pl.ds(b * R, R)
        start(("k", b), k_hbm.at[rows, :], k_v.at[rows, :])
        start(("v", b), v_hbm.at[rows, :], v_v.at[rows, :])

    def start_q(b):
        rows = pl.ds(b * R, R)
        start(("q", b), q_hbm.at[rows, :], q_v.at[rows, :])

    start("base", base_hbm, base_sm)
    start("fwd", fwd_hbm, fwd_v)
    start("shift", shift_hbm, shift_v)
    start("d", d_hbm, d_v)
    def start_mod(j, count):
        cols = pl.ds(j * D, count * D)
        start(("wm", j), wm_hbm.at[:, cols], wm_v.at[:, cols])

    for b in range(NPRO):
        start_kv(b)
        start_ssm(b)
    start_q(0)
    start_q(1)
    start("c", c_hbm, c_v)
    start("inv", inv_hbm, inv_v)
    start_mod(0, 3)
    start_mod(4, 1)
    start_mod(3, 1)
    for f in range(NF):
        start(("w1", f), w1_hbm.at[:, pl.ds(f * L, L)], w1_v.at[f])
        start(("w3", f), w3_hbm.at[:, pl.ds(f * L, L)], w3_v.at[f])
        if f + 1 == W13_GROUPS[0][1]:
            start_q(2)
    start_kv(CONV_AT[2])
    for n in range(ND):
        start(("w2", n), w2_hbm.at[:, pl.ds(n * L, L)], w2_v.at[n])
    start_mod(5, 1)
    for b in range(1, NB - 1):
        if b > 1:
            start_q(b + 1)
        if b in CONV_AT:
            start_ssm(CONV_AT[b])
        if b > 1 and b + 1 in CONV_AT:
            start_kv(CONV_AT[b + 1])

    copies["base"].wait()
    base = base_sm[0]

    def fence():
        @pl.loop(0, base + 1)
        def _(i):
            mark_s[0][1] = jnp.zeros((8, L), _F32)

    def wait(*names):
        for name in names:
            copies[name].wait()
        fence()

    for ref in (*z_s, *kv_s):
        ref[0, 0:8, 0:L] = jnp.zeros((8, L), _F32)
    for ref in stat_s:
        ref[0, 0:8] = jnp.zeros((8, L), _F32)
    for ref in h2_s:
        ref[0, 0:8, 0:L] = jnp.zeros((8, L), _F32)
    k_s[:, 0:HALO] = jnp.zeros((ND, HALO, L), _F32)

    written = []

    def wrote(ref, slot):
        if slot in TIE and not any(ref is r for r in written):
            written.append(ref)

    emitted = [0]

    def mark(result):
        mark_s[emitted[0] % len(mark_s)][1] = result[0:8, 0:L]
        emitted[0] += 1

    def after_mark(lag=MARK_LAG):
        return mark_s[(emitted[0] - 1 - lag) % len(mark_s)][base, 0:1]

    for ref in mark_s:
        ref[0] = jnp.zeros((8, L), _F32)

    def mod(j):
        return mod_s[0:1, j * D:(j + 1) * D]

    def compute_mod(j):
        sc = _silu(c_v[...].astype(_F32)).astype(_BF16)
        sc = jnp.broadcast_to(sc, (16, D))
        mod_s[:, j * D:(j + 1) * D] = _dot(sc, wm_v[:, j * D:(j + 1) * D])[0:8]

    def ssm_transform(m):
        spec = jax.lax.dot_general(tied(fwd_v[...]), sk_v[:, m * C:(m + 1) * C], _NT,
                                   preferred_element_type=_F32)
        if m == 0:
            kf_s[0][0, 0:C] = spec[0:C] + d_v[...].astype(_F32).reshape(1, D)
            kf_s[0][0, C:2 * C] = spec[C:2 * C]
        else:
            kf_s[m // CPB][m % CPB] = spec

    def widen_k(r0):
        kk = k_v[r0:r0 + RW, :].astype(_F32) + jnp.tile(after_mark(), (1, ND))
        for n in range(ND):
            k_s[n, HALO + r0:HALO + r0 + RW] = kk[:, n * L:(n + 1) * L]

    def short_conv(i, p):
        r0 = i * C + p * RP
        w = shift_v[...].astype(_F32)
        ks = None
        for j in range(w.shape[0]):
            kj = jnp.concatenate([k_s[base + n, HALO + r0 - j:HALO + r0 - j + RP]
                                  for n in range(ND)], axis=1)
            ks = kj * w[j:j + 1] if ks is None else ks + kj * w[j:j + 1]
        kv_s[i // CPB][1 + i % CPB, p * RP:(p + 1) * RP] = ks * v_v[r0:r0 + RP, :].astype(_F32)
        wrote(kv_s[i // CPB], 'c')

    def kv_transform(i):
        kv = kv_s[i // CPB][base + (1 + i % CPB)].astype(_BF16)
        u_s[i // CPB][i % CPB] = _dot(tied(fwd_v[...]), kv)

    def mac(b, g, n):
        chunks = range(b * CPB, (b + 1) * CPB)
        re = pl.ds(16 * g, 16)
        im = pl.ds(C + 16 * g, 16)
        ln = slice(n * L, (n + 1) * L)

        def tile(refs, i):
            return refs[i // CPB][base + i % CPB, re, ln], refs[i // CPB][base + i % CPB, im, ln]

        acc = {}
        kf = {}
        for i in range(chunks[-1] + 1):
            ur, ui = tile(u_s, i)
            for j in chunks:
                if j < i:
                    continue
                if j - i not in kf:
                    kf[j - i] = tile(kf_s, j - i)
                kr, ki = kf[j - i]
                pr, pi = kr * ur - ki * ui, kr * ui + ki * ur
                acc[j] = (acc[j][0] + pr, acc[j][1] + pi) if j in acc else (pr, pi)
        if b > 0:
            carry = carry_s[(b - 1) % 2]
            acc[chunks[0] - 1] = (carry[base, re, ln], carry[base, im, ln])
        if b + 1 < NB:
            carry_s[b % 2][0, re, ln], carry_s[b % 2][0, im, ln] = acc[chunks[-1]]
        for j in chunks:
            (ar, br), (ai, bi) = ((x[0:8], x[8:16]) for x in acc[j])
            if j > 0:
                pr, pi = acc[j - 1]
                ar, ai = ar - pi[0:8], ai + pr[0:8]
                br, bi = br + pi[8:16], bi - pr[8:16]
            for k, x in enumerate((ar + br, ai - bi, ar - br, ai + bi)):
                z_s[b][1 + j % CPB, pl.ds(k * (C // 2) + 8 * g, 8), ln] = x
        wrote(z_s[b], 'z')

    def inverse_transform(b, jj):
        for odd in range(2):
            z = z_s[b][base + (1 + jj), odd * C:(odd + 1) * C].astype(_BF16)
            y = _dot(tied(inv_v[odd * C // 4:(odd + 1) * C // 4]), z)
            for n in range(ND):
                y_s[b][n, pl.ds(jj * C + odd, C // 2, stride=2), :] = y[:, n * L:(n + 1) * L]

    def stat(k, b, rows):
        s = stat_s[k][base + (1 + b % 2), rows]
        return jnp.tile(s + after_mark() if k % 2 == 0 else s, (1, ND))

    def q_rows(b, rows):
        return q_v[b * R + rows.start:b * R + rows.stop, :].astype(_F32)

    def norm1_mean(b, rows):
        stat_s[0][1 + b % 2, rows] = _row_mean(q_rows(b, rows), after_mark())
        wrote(stat_s[0], 't')

    def norm1_scale(b, rows):
        xc = q_rows(b, rows) - stat(0, b, rows)
        stat_s[1][1 + b % 2, rows] = jax.lax.rsqrt(_row_mean(xc * xc) + EPS)
        wrote(stat_s[1], 't')

    def residual(b, rows):
        x = q_rows(b, rows)
        y = jnp.concatenate([y_s[b][base + n, rows] for n in range(ND)], axis=1)
        h = (x - stat(0, b, rows)) * stat(1, b, rows) * (mod(2) * (1.0 + mod(1))) + mod(2) * mod(0)
        x1 = x + h * y
        x1_s[b % 3, rows] = x1
        stat_s[2][1 + b % 2, rows] = _row_mean(x1)
        wrote(stat_s[2], 't')

    def norm2_scale(b, rows):
        xc = x1_s[base + b % 3, rows] - stat(2, b, rows)
        stat_s[3][1 + b % 2, rows] = jax.lax.rsqrt(_row_mean(xc * xc) + EPS)
        wrote(stat_s[3], 't')

    def norm2_apply(b, rows):
        xc = x1_s[base + b % 3, rows] - stat(2, b, rows)
        h2 = xc * stat(3, b, rows) * (1.0 + mod(4))
        h2_s[b % 2][1, rows] = h2
        wrote(h2_s[b % 2], 'h')

    def tied(words):
        if written:
            top = words[0:8, 0:L]
            for ref in written:
                top = top | pltpu.bitcast(ref[base, 0:8, 0:L], jnp.uint32)
            written.clear()
            if words.shape[1] > L:
                top = jnp.concatenate([top, words[0:8, L:]], axis=1)
            words = jnp.concatenate([top, words[8:]], axis=0)
        return pltpu.bitcast(words, _BF16)

    def weight(ref, tile, rows):
        return tied(ref.bitcast(jnp.uint32)[tile, rows.start // 2:rows.stop // 2])

    live = {}

    def ffn_gate(blocks, f):
        first = blocks[0] == 0
        if f == 0:
            h2 = jnp.concatenate([h2_s[b % 2][base + 1] for b in blocks], axis=0)
            live["h2"] = (h2 + mod(3)).astype(_BF16)
        if first and f in dict(W13_GROUPS):
            wait(*[(w, j) for j in range(f, dict(W13_GROUPS)[f]) for w in ("w1", "w3")],
                 *([("q", 2)] if f == W13_GROUPS[1][0] else []))
        live["gate"] = _dot(live["h2"], weight(w1_v, f, slice(0, D)))
        mark(live["gate"])

    def ffn_up(blocks, f):
        up = _dot(live["h2"], weight(w3_v, f, slice(0, D)))
        mark(up)
        live["act", f] = (_silu(live.pop("gate")) * up).astype(_BF16)

    def ffn_down(blocks, n, kk):
        first = blocks[0] == 0
        if first and n == 0 and kk == 0:
            wait(*[("w2", j) for j in range(ND)], ("wm", 5))
            compute_mod(5)
        act = jnp.concatenate([live["act", kk * KT + j] for j in range(KT)], axis=1)
        o = _dot(act, weight(w2_v, n, slice(kk * KT * L, (kk + 1) * KT * L)))
        mark(o)
        if kk > 0:
            o = live.pop("out") + o
        if kk + 1 < NF // KT:
            live["out"] = o
            return
        cols = slice(n * L, (n + 1) * L)
        for j, b in enumerate(blocks):
            res = x1_s[base + b % 3, :, cols] + mod(5)[:, cols] * o[j * R:(j + 1) * R]
            out_v[b * R:(b + 1) * R, cols] = res.astype(_BF16)
        if blocks[-1] + 1 == NB and n + 2 >= ND:
            send(pl.ds((NB - 1) * R, R), pl.ds(0, (ND - 1) * L) if n + 2 == ND else pl.ds(n * L, L))

    out_copies = []

    def send(rows, cols):
        cp = pltpu.make_async_copy(out_v.at[rows, cols], out_hbm.at[rows, cols],
                                   out_sems.at[len(out_copies)])
        cp.start()
        out_copies.append(cp)

    def ffn_steps(blocks):
        steps = []
        for f in range(NF):
            steps += [lambda f=f: ffn_gate(blocks, f), lambda f=f: ffn_up(blocks, f)]
        steps += [lambda n=n, kk=kk: ffn_down(blocks, n, kk)
                  for n in range(ND) for kk in range(NF // KT)]
        return steps

    def short_conv_steps(b):
        return ([(lambda r0=r0: widen_k(r0), 2 * RW * ND // 8)
                 for r0 in range(b * R, (b + 1) * R, RW)]
                + [(lambda i=i, p=p: short_conv(i, p), 9 * RP * ND // 8)
                   for i in range(b * CPB, (b + 1) * CPB) for p in range(C // RP)])

    def mac_steps(b):
        cost = sum(j + 1 for j in range(b * CPB, (b + 1) * CPB)) * 16
        return [(lambda g=g, n=n: mac(b, g, n), cost)
                for g in range(C // 16) for n in range(ND)]

    def norm_passes(b, rn=RN):
        return [[(lambda p=p, fn=fn: fn(b, slice(p * rn, (p + 1) * rn)), ops * rn * ND // 8)
                 for p in range(R // rn)]
                for fn, ops in ((norm1_mean, 2), (norm1_scale, 5), (residual, 9),
                                (norm2_scale, 4), (norm2_apply, 5))]

    def transform_steps(b):
        return [(lambda i=i, fn=fn: fn(i), 0)
                for fn in (ssm_transform, kv_transform) for i in range(b * CPB, (b + 1) * CPB)]

    def pipeline_step(*blocks):
        b = blocks[-1]
        main = ffn_steps(blocks)
        sizes = [ND] * (2 * NF) + [KT] * (len(main) - 2 * NF)
        slots = [[] for _ in main]
        if b in CONV_AT:
            for step, at in zip(transform_steps(CONV_AT[b]), XFORM_AT):
                slots[at].append(step)
        if b + 1 < NB:
            for jj in range(CPB):
                slots[INV0 + jj].append((lambda jj=jj: inverse_transform(b + 1, jj), 0))
            norm_at = NORM_FIRST if b == 1 else NORM_AT if b in MAC_AT else NORM_WIDE
            for steps, (first, stop) in zip(norm_passes(b + 1), norm_at):
                _spread(slots, steps, first, stop)
        if b + 1 in CONV_AT:
            first, stop = SC_FIRST if b == 1 else (SC0, SC1)
            if b == 1:
                for name in ("k", "v"):
                    slots[first].append((copies[name, CONV_AT[2]].wait, 0))
            _spread(slots, short_conv_steps(CONV_AT[b + 1]), first, stop)
        if b in MAC_AT:
            first, stop = MAC_FIRST if b == 1 else (XFORM_AT[-1] + MAC_LAG, len(slots))
            _fill(slots[:stop], sizes[:stop], mac_steps(MAC_AT[b]), first)
        for step, side in zip(main, slots):
            step()
            for extra, _ in side:
                extra()
        if b + 1 < NB:
            send(pl.ds(blocks[0] * R, len(blocks) * R), pl.ds(0, D))

    def run(steps):
        for step, _ in steps:
            step()

    wait("fwd", "shift", "d")
    def norms(first, stop):
        for k in range(first, stop):
            for b in range(2):
                run(norm_passes(b, R)[k])

    for r in range(NPRO + 2):
        if r < NPRO:
            wait(("k", r), ("v", r), ("sk", r))
        elif r == NPRO:
            wait(("q", 0), ("q", 1), "c", "inv")
            norms(0, 2)
        else:
            wait(("wm", 0))
            for j in (1, 0, 2):
                compute_mod(j)
            norms(2, 4)
        if 1 <= r <= NPRO:
            run(transform_steps(r - 1)[CPB:])
        if r < NPRO:
            run(transform_steps(r)[:CPB] + short_conv_steps(r))
        for b in PRO_MAC.get(r, ()):
            run(mac_steps(b))
        if r == NPRO:
            for b in range(2):
                for jj in range(CPB):
                    inverse_transform(b, jj)
        written.clear()
    wait(("wm", 4))
    compute_mod(4)
    norms(4, 5)
    wait(("wm", 3))
    compute_mod(3)
    pipeline_step(0, 1)
    for b in range(2, NB):
        needs = [("q", b + 1)] if b + 1 < NB else []
        if b in CONV_AT:
            needs += [("sk", CONV_AT[b])]
        if b + 1 in CONV_AT:
            needs += [("k", CONV_AT[b + 1]), ("v", CONV_AT[b + 1])]
        wait(*needs)
        pipeline_step(b)
    for cp in out_copies:
        cp.wait()


@jax.jit
def pallas_adaLN_cond__ssm_conv_h3__glu_gated_swiglu__prompt_kernel(
    A_q: jax.Array,
    A_k: jax.Array,
    A_v: jax.Array,
    A_shift_k: jax.Array,
    A_ssm_k: jax.Array,
    A_ssm_D: jax.Array,
    B_x: jax.Array,
    B_w1: jax.Array,
    B_w3: jax.Array,
    B_w2: jax.Array,
    c: jax.Array,
    w_mod: jax.Array,
):
    del B_x
    B, S, D = A_q.shape
    FH = B_w1.shape[1]
    KS = A_shift_k.shape[1]
    assert B == 1 and S % R == 0 and FH % (KT * L) == 0 and D % L == 0 and KS <= HALO + 1
    NB, CPB = S // R, R // C
    NF, ND = FH // L, D // L
    n_in = 6 + 4 * NB + 4 + 2 * NF + ND

    hbm = pl.BlockSpec(memory_space=pl.ANY)
    out = pl.pallas_call(
        _kernel,
        out_shape=jax.ShapeDtypeStruct((S, D), A_q.dtype),
        in_specs=[hbm] * 14,
        out_specs=hbm,
        scratch_shapes=[
            pltpu.VMEM((S, D), _BF16),
            pltpu.VMEM((S, D), _BF16),
            pltpu.VMEM((S, D), _BF16),
            pltpu.VMEM((KS, D), _BF16),
            pltpu.VMEM((D, S), _BF16),
            pltpu.VMEM((D,), _BF16),
            pltpu.VMEM((NF, D, L), _BF16),
            pltpu.VMEM((NF, D, L), _BF16),
            pltpu.VMEM((ND, FH, L), _BF16),
            pltpu.VMEM((1, D), _BF16),
            pltpu.VMEM((D, 6 * D), _BF16),
            pltpu.VMEM(_FWD.shape, jnp.uint32),
            pltpu.VMEM(_INV.shape, jnp.uint32),
            pltpu.SMEM((1,), jnp.int32),
            pltpu.VMEM((ND, HALO + S, L), _F32),
            [pltpu.VMEM((CPB + 1, C, D), _F32)] * NB,
            [pltpu.VMEM((CPB, 2 * C, D), _F32)] * NB,
            [pltpu.VMEM((CPB, 2 * C, D), _F32)] * NB,
            [pltpu.VMEM((1, 2 * C, D), _F32)] * 2,
            [pltpu.VMEM((CPB + 1, 2 * C, D), _F32)] * NB,
            [pltpu.VMEM((ND, R, L), _F32)] * NB,
            pltpu.VMEM((8, 6 * D), _F32),
            [pltpu.VMEM((3, R, L), _F32)] * 4,
            [pltpu.VMEM((2, 8, L), _F32)] * 8,
            pltpu.VMEM((3, R, D), _F32),
            [pltpu.VMEM((2, R, D), _F32)] * 2,
            pltpu.VMEM((S, D), _BF16),
            pltpu.SemaphoreType.DMA((n_in,)),
            pltpu.SemaphoreType.DMA((NB,)),
        ],
        compiler_params=pltpu.CompilerParams(vmem_limit_bytes=120 * 1024 * 1024),
    )(
        A_q.reshape(S, D), A_k.reshape(S, D), A_v.reshape(S, D),
        A_shift_k.T, A_ssm_k, A_ssm_D,
        B_w1, B_w3, B_w2, c, w_mod,
        _FWD, _INV, np.zeros((1,), np.int32),
    )
    return out.reshape(B, S, D)
```

```python
import numpy as np

import jax
import jax.numpy as jnp
import jax.experimental.pallas as pl
import jax.experimental.pallas.tpu as pltpu

C = 128
R = 256
L = 128
HALO = 8
RW = 128
RP = 32
RN = 32
MAC_LAG = 3
MARK_LAG = 5
TIE = 'zc'
INV0 = 0
SC0, SC1 = 14, 24
NORM_AT = ((0, 3), (2, 5), (5, 9), (8, 11), (11, 14))
XFORM_AT = (3, 5, 11, 12)
NPRO = 4
PRO_MAC = {2: (0,), 3: (1,), 4: (2,)}
CONV_AT = {2: 4, 3: 5, 4: 6, 5: 7}
MAC_AT = {1: 3, 2: 4, 3: 5, 4: 6, 5: 7}
SC_FIRST = (25, 39)
MAC_FIRST = (4, 39)
NORM_FIRST = ((4, 8), (7, 12), (12, 17), (16, 20), (19, 24))
NORM_WIDE = ((0, 8), (6, 14), (14, 22), (21, 29), (28, 36))
W13_GROUPS = ((0, 2), (2, 6), (6, 12))
KT = 4
EPS = 1e-5

_F32 = jnp.float32
_BF16 = jnp.bfloat16
_NT = (((1,), (1,)), ((), ()))


def _packed_bf16(x):
    bits = np.ascontiguousarray(x, np.float32).view(np.uint32)
    bits = (bits + 0x7FFF + ((bits >> 16) & 1)) >> 16
    return bits[0::2] | (bits[1::2] << 16)


def _dft_matrices():
    even = np.arange(0, C, 2)
    f = np.stack([even.reshape(-1, 8), C - 1 - even.reshape(-1, 8)], axis=1).reshape(-1)
    step = 2.0 * np.pi / (2 * C)
    ang = step * (f[:, None] + 0.5) * np.arange(C)[None, :]
    fwd = np.concatenate([np.cos(ang), -np.sin(ang)], axis=0)
    n = np.concatenate([even, even + 1])
    ang = step * n[:, None] * (even[None, :] + 0.5)
    inv = np.concatenate([np.cos(ang), -np.sin(ang)], axis=1) / C
    return _packed_bf16(fwd), _packed_bf16(inv)


_FWD, _INV = _dft_matrices()


def _dot(a, b):
    return jnp.dot(a, b, preferred_element_type=_F32)


def _row_mean(x, zero=None):
    acc = x[:, 0:L] if zero is None else x[:, 0:L] + zero
    for n in range(1, x.shape[1] // L):
        acc = acc + x[:, n * L:(n + 1) * L]
    m = jnp.sum(acc, axis=-1, keepdims=True) * (1.0 / x.shape[1])
    return jnp.broadcast_to(m, (x.shape[0], L))


def _silu(x):
    hx = 0.5 * x
    return hx * jnp.tanh(hx) + hx


def _spread(slots, steps, first, last):
    for k, step in enumerate(steps):
        slots[first + (k * (last - first)) // len(steps)].append(step)


def _fill(slots, sizes, steps, first):
    held = [sum(cost for _, cost in slot) for slot in slots]
    rate = (sum(held[first:]) + sum(cost for _, cost in steps)) / sum(sizes[first:])
    budget, k = 0.0, 0
    for s in range(first, len(slots)):
        budget += rate * sizes[s] - held[s]
        while k < len(steps) and (budget >= 0.5 * steps[k][1] or s == len(slots) - 1):
            slots[s].append(steps[k])
            budget -= steps[k][1]
            k += 1


def _kernel(q_hbm, k_hbm, v_hbm, shift_hbm, sk_hbm, d_hbm, w1_hbm, w3_hbm, w2_hbm,
            c_hbm, wm_hbm, fwd_hbm, inv_hbm, base_hbm, out_hbm,
            q_v, k_v, v_v, shift_v, sk_v, d_v, w1_v, w3_v, w2_v, c_v, wm_v, fwd_v, inv_v, base_sm,
            taps_s, k_s, kv_s, u_s, kf_s, carry_s, z_s, y_s, mod_s, stat_s, mark_s, x1_s, h2_s, out_v,
            in_sems, out_sems):
    S, D = q_hbm.shape
    FH = w1_hbm.shape[1]
    NB = S // R
    NC = S // C
    CPB = R // C
    NF = FH // L
    ND = D // L

    copies = {}

    def start(name, src, dst):
        cp = pltpu.make_async_copy(src, dst, in_sems.at[len(copies)])
        cp.start()
        copies[name] = cp

    def start_ssm(b):
        cols = pl.ds(b * R, R)
        start(("sk", b), sk_hbm.at[:, cols], sk_v.at[:, cols])

    def start_kv(b):
        rows = pl.ds(b * R, R)
        start(("k", b), k_hbm.at[rows, :], k_v.at[rows, :])
        start(("v", b), v_hbm.at[rows, :], v_v.at[rows, :])

    def start_q(b):
        rows = pl.ds(b * R, R)
        start(("q", b), q_hbm.at[rows, :], q_v.at[rows, :])

    start("base", base_hbm, base_sm)
    start("fwd", fwd_hbm, fwd_v)
    start("shift", shift_hbm, shift_v)
    start("d", d_hbm, d_v)
    def start_mod(j, count):
        cols = pl.ds(j * D, count * D)
        start(("wm", j), wm_hbm.at[:, cols], wm_v.at[:, cols])

    for b in range(NPRO):
        start_kv(b)
        start_ssm(b)
    start_q(0)
    start_q(1)
    start("c", c_hbm, c_v)
    start("inv", inv_hbm, inv_v)
    start_mod(0, 3)
    start_mod(4, 1)
    start_mod(3, 1)
    for f in range(NF):
        start(("w1", f), w1_hbm.at[:, pl.ds(f * L, L)], w1_v.at[f])
        start(("w3", f), w3_hbm.at[:, pl.ds(f * L, L)], w3_v.at[f])
        if f + 1 == W13_GROUPS[0][1]:
            start_q(2)
    start_kv(CONV_AT[2])
    for n in range(ND):
        start(("w2", n), w2_hbm.at[:, pl.ds(n * L, L)], w2_v.at[n])
    start_mod(5, 1)
    for b in range(1, NB - 1):
        if b > 1:
            start_q(b + 1)
        if b in CONV_AT:
            start_ssm(CONV_AT[b])
        if b > 1 and b + 1 in CONV_AT:
            start_kv(CONV_AT[b + 1])

    copies["base"].wait()
    base = base_sm[0]

    def fence():
        @pl.loop(0, base + 1)
        def _(i):
            mark_s[0][1] = jnp.zeros((8, L), _F32)

    def wait(*names):
        for name in names:
            copies[name].wait()
        fence()

    for ref in (*z_s, *kv_s):
        ref[0, 0:8, 0:L] = jnp.zeros((8, L), _F32)
    for ref in stat_s:
        ref[0, 0:8] = jnp.zeros((8, L), _F32)
    for ref in h2_s:
        ref[0, 0:8, 0:L] = jnp.zeros((8, L), _F32)
    k_s[:, 0:HALO] = jnp.zeros((ND, HALO, L), _F32)

    written = []

    def wrote(ref, slot):
        if slot in TIE and not any(ref is r for r in written):
            written.append(ref)

    emitted = [0]

    def mark(result):
        mark_s[emitted[0] % len(mark_s)][1] = result[0:8, 0:L]
        emitted[0] += 1

    def after_mark(lag=MARK_LAG):
        return mark_s[(emitted[0] - 1 - lag) % len(mark_s)][base, 0:1]

    for ref in mark_s:
        ref[0] = jnp.zeros((8, L), _F32)

    def mod(j):
        return mod_s[0:1, j * D:(j + 1) * D]

    def compute_mod(j):
        sc = _silu(c_v[...].astype(_F32)).astype(_BF16)
        sc = jnp.broadcast_to(sc, (16, D))
        mod_s[:, j * D:(j + 1) * D] = _dot(sc, wm_v[:, j * D:(j + 1) * D])[0:8]

    def ssm_transform(m):
        spec = jax.lax.dot_general(tied(fwd_v[...]), sk_v[:, m * C:(m + 1) * C], _NT,
                                   preferred_element_type=_F32)
        if m == 0:
            kf_s[0][0, 0:C] = spec[0:C] + d_v[...].astype(_F32).reshape(1, D)
            kf_s[0][0, C:2 * C] = spec[C:2 * C]
        else:
            kf_s[m // CPB][m % CPB] = spec

    def widen_k(r0):
        kk = k_v[r0:r0 + RW, :].astype(_F32) + jnp.tile(after_mark(), (1, ND))
        for n in range(ND):
            k_s[n, HALO + r0:HALO + r0 + RW] = kk[:, n * L:(n + 1) * L]

    def short_conv(i, p):
        r0 = i * C + p * RP
        ks = None
        for j in range(shift_v.shape[0]):
            kj = jnp.concatenate([k_s[base + n, HALO + r0 - j:HALO + r0 - j + RP]
                                  for n in range(ND)], axis=1)
            term = kj * jnp.tile(taps_s[base + j], (RP // 8, 1))
            ks = term if ks is None else ks + term
        kv_s[i // CPB][1 + i % CPB, p * RP:(p + 1) * RP] = ks * v_v[r0:r0 + RP, :].astype(_F32)
        wrote(kv_s[i // CPB], 'c')

    def kv_transform(i):
        kv = kv_s[i // CPB][base + (1 + i % CPB)].astype(_BF16)
        u_s[i // CPB][i % CPB] = _dot(tied(fwd_v[...]), kv)

    def mac(b, g, n):
        chunks = range(b * CPB, (b + 1) * CPB)
        re = pl.ds(16 * g, 16)
        im = pl.ds(C + 16 * g, 16)
        ln = slice(n * L, (n + 1) * L)

        def tile(refs, i):
            return refs[i // CPB][base + i % CPB, re, ln], refs[i // CPB][base + i % CPB, im, ln]

        acc = {}
        kf = {}
        for i in range(chunks[-1] + 1):
            ur, ui = tile(u_s, i)
            for j in chunks:
                if j < i:
                    continue
                if j - i not in kf:
                    kf[j - i] = tile(kf_s, j - i)
                kr, ki = kf[j - i]
                pr, pi = kr * ur - ki * ui, kr * ui + ki * ur
                acc[j] = (acc[j][0] + pr, acc[j][1] + pi) if j in acc else (pr, pi)
        if b > 0:
            carry = carry_s[(b - 1) % 2]
            acc[chunks[0] - 1] = (carry[base, re, ln], carry[base, im, ln])
        if b + 1 < NB:
            carry_s[b % 2][0, re, ln], carry_s[b % 2][0, im, ln] = acc[chunks[-1]]
        for j in chunks:
            (ar, br), (ai, bi) = ((x[0:8], x[8:16]) for x in acc[j])
            if j > 0:
                pr, pi = acc[j - 1]
                ar, ai = ar - pi[0:8], ai + pr[0:8]
                br, bi = br + pi[8:16], bi - pr[8:16]
            for k, x in enumerate((ar + br, ai - bi, ar - br, ai + bi)):
                z_s[b][1 + j % CPB, pl.ds(k * (C // 2) + 8 * g, 8), ln] = x
        wrote(z_s[b], 'z')

    def inverse_transform(b, jj):
        for odd in range(2):
            z = z_s[b][base + (1 + jj), odd * C:(odd + 1) * C].astype(_BF16)
            y = _dot(tied(inv_v[odd * C // 4:(odd + 1) * C // 4]), z)
            for n in range(ND):
                y_s[b][n, pl.ds(jj * C + odd, C // 2, stride=2), :] = y[:, n * L:(n + 1) * L]

    def stat(k, b, rows):
        s = stat_s[k][base + (1 + b % 2), rows]
        return jnp.tile(s + after_mark() if k % 2 == 0 else s, (1, ND))

    def q_rows(b, rows):
        return q_v[b * R + rows.start:b * R + rows.stop, :].astype(_F32)

    def norm1_mean(b, rows):
        stat_s[0][1 + b % 2, rows] = _row_mean(q_rows(b, rows), after_mark())
        wrote(stat_s[0], 't')

    def norm1_scale(b, rows):
        xc = q_rows(b, rows) - stat(0, b, rows)
        stat_s[1][1 + b % 2, rows] = jax.lax.rsqrt(_row_mean(xc * xc) + EPS)
        wrote(stat_s[1], 't')

    def residual(b, rows):
        x = q_rows(b, rows)
        y = jnp.concatenate([y_s[b][base + n, rows] for n in range(ND)], axis=1)
        h = (x - stat(0, b, rows)) * stat(1, b, rows) * (mod(2) * (1.0 + mod(1))) + mod(2) * mod(0)
        x1 = x + h * y
        x1_s[b % 3, rows] = x1
        stat_s[2][1 + b % 2, rows] = _row_mean(x1)
        wrote(stat_s[2], 't')

    def norm2_scale(b, rows):
        xc = x1_s[base + b % 3, rows] - stat(2, b, rows)
        stat_s[3][1 + b % 2, rows] = jax.lax.rsqrt(_row_mean(xc * xc) + EPS)
        wrote(stat_s[3], 't')

    def norm2_apply(b, rows):
        xc = x1_s[base + b % 3, rows] - stat(2, b, rows)
        h2 = xc * stat(3, b, rows) * (1.0 + mod(4))
        h2_s[b % 2][1, rows] = h2
        wrote(h2_s[b % 2], 'h')

    def tied(words):
        if written:
            top = words[0:8, 0:L]
            for ref in written:
                top = top | pltpu.bitcast(ref[base, 0:8, 0:L], jnp.uint32)
            written.clear()
            if words.shape[1] > L:
                top = jnp.concatenate([top, words[0:8, L:]], axis=1)
            words = jnp.concatenate([top, words[8:]], axis=0)
        return pltpu.bitcast(words, _BF16)

    def weight(ref, tile, rows):
        return tied(ref.bitcast(jnp.uint32)[tile, rows.start // 2:rows.stop // 2])

    live = {}

    def ffn_gate(blocks, f):
        first = blocks[0] == 0
        if f == 0:
            h2 = jnp.concatenate([h2_s[b % 2][base + 1] for b in blocks], axis=0)
            live["h2"] = (h2 + mod(3)).astype(_BF16)
        if first and f in dict(W13_GROUPS):
            wait(*[(w, j) for j in range(f, dict(W13_GROUPS)[f]) for w in ("w1", "w3")],
                 *([("q", 2)] if f == W13_GROUPS[1][0] else []))
        live["gate"] = _dot(live["h2"], weight(w1_v, f, slice(0, D)))
        mark(live["gate"])

    def ffn_up(blocks, f):
        up = _dot(live["h2"], weight(w3_v, f, slice(0, D)))
        mark(up)
        live["act", f] = (_silu(live.pop("gate")) * up).astype(_BF16)

    def ffn_down(blocks, n, kk):
        first = blocks[0] == 0
        if first and n == 0 and kk == 0:
            wait(*[("w2", j) for j in range(ND)], ("wm", 5))
            compute_mod(5)
        act = jnp.concatenate([live["act", kk * KT + j] for j in range(KT)], axis=1)
        o = _dot(act, weight(w2_v, n, slice(kk * KT * L, (kk + 1) * KT * L)))
        mark(o)
        if kk > 0:
            o = live.pop("out") + o
        if kk + 1 < NF // KT:
            live["out"] = o
            return
        cols = slice(n * L, (n + 1) * L)
        for j, b in enumerate(blocks):
            res = x1_s[base + b % 3, :, cols] + mod(5)[:, cols] * o[j * R:(j + 1) * R]
            out_v[b * R:(b + 1) * R, cols] = res.astype(_BF16)
        if blocks[-1] + 1 == NB and n + 2 >= ND:
            send(pl.ds((NB - 1) * R, R), pl.ds(0, (ND - 1) * L) if n + 2 == ND else pl.ds(n * L, L))

    out_copies = []

    def send(rows, cols):
        cp = pltpu.make_async_copy(out_v.at[rows, cols], out_hbm.at[rows, cols],
                                   out_sems.at[len(out_copies)])
        cp.start()
        out_copies.append(cp)

    def ffn_steps(blocks):
        steps = []
        for f in range(NF):
            steps += [lambda f=f: ffn_gate(blocks, f), lambda f=f: ffn_up(blocks, f)]
        steps += [lambda n=n, kk=kk: ffn_down(blocks, n, kk)
                  for n in range(ND) for kk in range(NF // KT)]
        return steps

    def short_conv_steps(b):
        return ([(lambda r0=r0: widen_k(r0), 2 * RW * ND // 8)
                 for r0 in range(b * R, (b + 1) * R, RW)]
                + [(lambda i=i, p=p: short_conv(i, p), 9 * RP * ND // 8)
                   for i in range(b * CPB, (b + 1) * CPB) for p in range(C // RP)])

    def mac_steps(b):
        cost = sum(j + 1 for j in range(b * CPB, (b + 1) * CPB)) * 16
        return [(lambda g=g, n=n: mac(b, g, n), cost)
                for g in range(C // 16) for n in range(ND)]

    def norm_passes(b, rn=RN):
        return [[(lambda p=p, fn=fn: fn(b, slice(p * rn, (p + 1) * rn)), ops * rn * ND // 8)
                 for p in range(R // rn)]
                for fn, ops in ((norm1_mean, 2), (norm1_scale, 5), (residual, 9),
                                (norm2_scale, 4), (norm2_apply, 5))]

    def transform_steps(b):
        return [(lambda i=i, fn=fn: fn(i), 0)
                for fn in (ssm_transform, kv_transform) for i in range(b * CPB, (b + 1) * CPB)]

    def pipeline_step(*blocks):
        b = blocks[-1]
        main = ffn_steps(blocks)
        sizes = [ND] * (2 * NF) + [KT] * (len(main) - 2 * NF)
        slots = [[] for _ in main]
        if b in CONV_AT:
            for step, at in zip(transform_steps(CONV_AT[b]), XFORM_AT):
                slots[at].append(step)
        if b + 1 < NB:
            for jj in range(CPB):
                slots[INV0 + jj].append((lambda jj=jj: inverse_transform(b + 1, jj), 0))
            norm_at = NORM_FIRST if b == 1 else NORM_AT if b in MAC_AT else NORM_WIDE
            for steps, (first, stop) in zip(norm_passes(b + 1), norm_at):
                _spread(slots, steps, first, stop)
        if b + 1 in CONV_AT:
            first, stop = SC_FIRST if b == 1 else (SC0, SC1)
            if b == 1:
                for name in ("k", "v"):
                    slots[first].append((copies[name, CONV_AT[2]].wait, 0))
            _spread(slots, short_conv_steps(CONV_AT[b + 1]), first, stop)
        if b in MAC_AT:
            first, stop = MAC_FIRST if b == 1 else (XFORM_AT[-1] + MAC_LAG, len(slots))
            _fill(slots[:stop], sizes[:stop], mac_steps(MAC_AT[b]), first)
        for step, side in zip(main, slots):
            step()
            for extra, _ in side:
                extra()
        if b + 1 < NB:
            send(pl.ds(blocks[0] * R, len(blocks) * R), pl.ds(0, D))

    def run(steps):
        for step, _ in steps:
            step()

    wait("fwd", "shift", "d")
    taps = shift_v[...].astype(_F32)
    for j in range(taps.shape[0]):
        taps_s[j] = jnp.broadcast_to(taps[j:j + 1], (8, D))
    def norms(first, stop):
        for k in range(first, stop):
            for b in range(2):
                run(norm_passes(b, R)[k])

    for r in range(NPRO + 2):
        if r < NPRO:
            wait(("k", r), ("v", r), ("sk", r))
        elif r == NPRO:
            wait(("q", 0), ("q", 1), "c", "inv")
            norms(0, 2)
        else:
            wait(("wm", 0))
            for j in (1, 0, 2):
                compute_mod(j)
            norms(2, 4)
        if 1 <= r <= NPRO:
            run(transform_steps(r - 1)[CPB:])
        if r < NPRO:
            run(transform_steps(r)[:CPB] + short_conv_steps(r))
        for b in PRO_MAC.get(r, ()):
            run(mac_steps(b))
        if r == NPRO:
            for b in range(2):
                for jj in range(CPB):
                    inverse_transform(b, jj)
        written.clear()
    wait(("wm", 4))
    compute_mod(4)
    norms(4, 5)
    wait(("wm", 3))
    compute_mod(3)
    pipeline_step(0, 1)
    for b in range(2, NB):
        needs = [("q", b + 1)] if b + 1 < NB else []
        if b in CONV_AT:
            needs += [("sk", CONV_AT[b])]
        if b + 1 in CONV_AT:
            needs += [("k", CONV_AT[b + 1]), ("v", CONV_AT[b + 1])]
        wait(*needs)
        pipeline_step(b)
    for cp in out_copies:
        cp.wait()


@jax.jit
def pallas_adaLN_cond__ssm_conv_h3__glu_gated_swiglu__prompt_kernel(
    A_q: jax.Array,
    A_k: jax.Array,
    A_v: jax.Array,
    A_shift_k: jax.Array,
    A_ssm_k: jax.Array,
    A_ssm_D: jax.Array,
    B_x: jax.Array,
    B_w1: jax.Array,
    B_w3: jax.Array,
    B_w2: jax.Array,
    c: jax.Array,
    w_mod: jax.Array,
):
    del B_x
    B, S, D = A_q.shape
    FH = B_w1.shape[1]
    KS = A_shift_k.shape[1]
    assert B == 1 and S % R == 0 and FH % (KT * L) == 0 and D % L == 0 and KS <= HALO + 1
    NB, CPB = S // R, R // C
    NF, ND = FH // L, D // L
    n_in = 6 + 4 * NB + 4 + 2 * NF + ND

    hbm = pl.BlockSpec(memory_space=pl.ANY)
    out = pl.pallas_call(
        _kernel,
        out_shape=jax.ShapeDtypeStruct((S, D), A_q.dtype),
        in_specs=[hbm] * 14,
        out_specs=hbm,
        scratch_shapes=[
            pltpu.VMEM((S, D), _BF16),
            pltpu.VMEM((S, D), _BF16),
            pltpu.VMEM((S, D), _BF16),
            pltpu.VMEM((KS, D), _BF16),
            pltpu.VMEM((D, S), _BF16),
            pltpu.VMEM((D,), _BF16),
            pltpu.VMEM((NF, D, L), _BF16),
            pltpu.VMEM((NF, D, L), _BF16),
            pltpu.VMEM((ND, FH, L), _BF16),
            pltpu.VMEM((1, D), _BF16),
            pltpu.VMEM((D, 6 * D), _BF16),
            pltpu.VMEM(_FWD.shape, jnp.uint32),
            pltpu.VMEM(_INV.shape, jnp.uint32),
            pltpu.SMEM((1,), jnp.int32),
            pltpu.VMEM((KS, 8, D), _F32),
            pltpu.VMEM((ND, HALO + S, L), _F32),
            [pltpu.VMEM((CPB + 1, C, D), _F32)] * NB,
            [pltpu.VMEM((CPB, 2 * C, D), _F32)] * NB,
            [pltpu.VMEM((CPB, 2 * C, D), _F32)] * NB,
            [pltpu.VMEM((1, 2 * C, D), _F32)] * 2,
            [pltpu.VMEM((CPB + 1, 2 * C, D), _F32)] * NB,
            [pltpu.VMEM((ND, R, L), _F32)] * NB,
            pltpu.VMEM((8, 6 * D), _F32),
            [pltpu.VMEM((3, R, L), _F32)] * 4,
            [pltpu.VMEM((2, 8, L), _F32)] * 8,
            pltpu.VMEM((3, R, D), _F32),
            [pltpu.VMEM((2, R, D), _F32)] * 2,
            pltpu.VMEM((S, D), _BF16),
            pltpu.SemaphoreType.DMA((n_in,)),
            pltpu.SemaphoreType.DMA((NB,)),
        ],
        compiler_params=pltpu.CompilerParams(vmem_limit_bytes=120 * 1024 * 1024),
    )(
        A_q.reshape(S, D), A_k.reshape(S, D), A_v.reshape(S, D),
        A_shift_k.T, A_ssm_k, A_ssm_D,
        B_w1, B_w3, B_w2, c, w_mod,
        _FWD, _INV, np.zeros((1,), np.int32),
    )
    return out.reshape(B, S, D)
```

```python
import numpy as np

import jax
import jax.numpy as jnp
import jax.experimental.pallas as pl
import jax.experimental.pallas.tpu as pltpu

C = 128
R = 256
L = 128
HALO = 16
RW = 128
RP = 32
RN = 32
MAC_LAG = 3
MARK_LAG = 5
TIE = 'zc'
INV0 = 0
SC0, SC1 = 14, 24
NORM_AT = ((0, 3), (2, 5), (5, 9), (8, 11), (11, 14))
XFORM_AT = (3, 5, 11, 12)
NPRO = 4
PRO_MAC = {2: (0,), 3: (1,), 4: (2,)}
CONV_AT = {2: 4, 3: 5, 4: 6, 5: 7}
MAC_AT = {1: 3, 2: 4, 3: 5, 4: 6, 5: 7}
SC_FIRST = (25, 39)
MAC_FIRST = (4, 39)
NORM_FIRST = ((4, 8), (7, 12), (12, 17), (16, 20), (19, 24))
NORM_WIDE = ((0, 8), (6, 14), (14, 22), (21, 29), (28, 36))
W13_GROUPS = ((0, 2), (2, 6), (6, 12))
KT = 4
EPS = 1e-5

_F32 = jnp.float32
_BF16 = jnp.bfloat16
_NT = (((1,), (1,)), ((), ()))


def _packed_bf16(x):
    bits = np.ascontiguousarray(x, np.float32).view(np.uint32)
    bits = (bits + 0x7FFF + ((bits >> 16) & 1)) >> 16
    return bits[0::2] | (bits[1::2] << 16)


def _dft_matrices():
    even = np.arange(0, C, 2)
    f = np.stack([even.reshape(-1, 8), C - 1 - even.reshape(-1, 8)], axis=1).reshape(-1)
    step = 2.0 * np.pi / (2 * C)
    ang = step * (f[:, None] + 0.5) * np.arange(C)[None, :]
    fwd = np.concatenate([np.cos(ang), -np.sin(ang)], axis=0)
    n = np.concatenate([even, even + 1])
    ang = step * n[:, None] * (even[None, :] + 0.5)
    inv = np.concatenate([np.cos(ang), -np.sin(ang)], axis=1) / C
    return _packed_bf16(fwd), _packed_bf16(inv)


_FWD, _INV = _dft_matrices()


def _dot(a, b):
    return jnp.dot(a, b, preferred_element_type=_F32)


def _row_mean(x, zero=None):
    acc = x[:, 0:L] if zero is None else x[:, 0:L] + zero
    for n in range(1, x.shape[1] // L):
        acc = acc + x[:, n * L:(n + 1) * L]
    m = jnp.sum(acc, axis=-1, keepdims=True) * (1.0 / x.shape[1])
    return jnp.broadcast_to(m, (x.shape[0], L))


def _silu(x):
    hx = 0.5 * x
    return hx * jnp.tanh(hx) + hx


def _spread(slots, steps, first, last):
    for k, step in enumerate(steps):
        slots[first + (k * (last - first)) // len(steps)].append(step)


def _fill(slots, sizes, steps, first):
    held = [sum(cost for _, cost in slot) for slot in slots]
    rate = (sum(held[first:]) + sum(cost for _, cost in steps)) / sum(sizes[first:])
    budget, k = 0.0, 0
    for s in range(first, len(slots)):
        budget += rate * sizes[s] - held[s]
        while k < len(steps) and (budget >= 0.5 * steps[k][1] or s == len(slots) - 1):
            slots[s].append(steps[k])
            budget -= steps[k][1]
            k += 1


def _kernel(q_hbm, k_hbm, v_hbm, shift_hbm, sk_hbm, d_hbm, w1_hbm, w3_hbm, w2_hbm,
            c_hbm, wm_hbm, fwd_hbm, inv_hbm, base_hbm, out_hbm,
            q_v, k_v, v_v, shift_v, sk_v, d_v, w1_v, w3_v, w2_v, c_v, wm_v, fwd_v, inv_v, base_sm,
            taps_s, k_s, kv_s, u_s, kf_s, carry_s, z_s, y_s, mod_s, stat_s, mark_s, x1_s, h2_s, out_v,
            in_sems, out_sems):
    S, D = q_hbm.shape
    FH = w1_hbm.shape[1]
    NB = S // R
    NC = S // C
    CPB = R // C
    NF = FH // L
    ND = D // L

    copies = {}

    def start(name, src, dst):
        cp = pltpu.make_async_copy(src, dst, in_sems.at[len(copies)])
        cp.start()
        copies[name] = cp

    def start_ssm(b):
        cols = pl.ds(b * R, R)
        start(("sk", b), sk_hbm.at[:, cols], sk_v.at[:, cols])

    def start_kv(b):
        rows = pl.ds(b * R, R)
        start(("k", b), k_hbm.at[rows, :], k_v.at[rows, :])
        start(("v", b), v_hbm.at[rows, :], v_v.at[rows, :])

    def start_q(b):
        rows = pl.ds(b * R, R)
        start(("q", b), q_hbm.at[rows, :], q_v.at[rows, :])

    start("base", base_hbm, base_sm)
    start("fwd", fwd_hbm, fwd_v)
    start("shift", shift_hbm, shift_v)
    start("d", d_hbm, d_v)
    def start_mod(j, count):
        cols = pl.ds(j * D, count * D)
        start(("wm", j), wm_hbm.at[:, cols], wm_v.at[:, cols])

    for b in range(NPRO):
        start_kv(b)
        start_ssm(b)
    start_q(0)
    start_q(1)
    start("c", c_hbm, c_v)
    start("inv", inv_hbm, inv_v)
    start_mod(0, 3)
    start_mod(4, 1)
    start_mod(3, 1)
    for f in range(NF):
        start(("w1", f), w1_hbm.at[:, pl.ds(f * L, L)], w1_v.at[f])
        start(("w3", f), w3_hbm.at[:, pl.ds(f * L, L)], w3_v.at[f])
        if f + 1 == W13_GROUPS[0][1]:
            start_q(2)
    start_kv(CONV_AT[2])
    for n in range(ND):
        start(("w2", n), w2_hbm.at[:, pl.ds(n * L, L)], w2_v.at[n])
    start_mod(5, 1)
    for b in range(1, NB - 1):
        if b > 1:
            start_q(b + 1)
        if b in CONV_AT:
            start_ssm(CONV_AT[b])
        if b > 1 and b + 1 in CONV_AT:
            start_kv(CONV_AT[b + 1])

    copies["base"].wait()
    base = base_sm[0]

    def fence():
        @pl.loop(0, base + 1)
        def _(i):
            mark_s[0][1] = jnp.zeros((8, L), _F32)

    def wait(*names):
        for name in names:
            copies[name].wait()
        fence()

    for ref in (*z_s, *kv_s):
        ref[0, 0:8, 0:L] = jnp.zeros((8, L), _F32)
    for ref in stat_s:
        ref[0, 0:8] = jnp.zeros((8, L), _F32)
    for ref in h2_s:
        ref[0, 0:8, 0:L] = jnp.zeros((8, L), _F32)
    k_s[:, 0:HALO] = jnp.zeros((ND, HALO, L), _F32)

    written = []

    def wrote(ref, slot):
        if slot in TIE and not any(ref is r for r in written):
            written.append(ref)

    emitted = [0]

    def mark(result):
        mark_s[emitted[0] % len(mark_s)][1] = result[0:8, 0:L]
        emitted[0] += 1

    def after_mark(lag=MARK_LAG):
        return mark_s[(emitted[0] - 1 - lag) % len(mark_s)][base, 0:1]

    for ref in mark_s:
        ref[0] = jnp.zeros((8, L), _F32)

    def mod(j):
        return mod_s[0:1, j * D:(j + 1) * D]

    def compute_mod(j):
        sc = _silu(c_v[...].astype(_F32)).astype(_BF16)
        sc = jnp.broadcast_to(sc, (16, D))
        mod_s[:, j * D:(j + 1) * D] = _dot(sc, wm_v[:, j * D:(j + 1) * D])[0:8]

    def ssm_transform(m):
        spec = jax.lax.dot_general(tied(fwd_v[...]), sk_v[:, m * C:(m + 1) * C], _NT,
                                   preferred_element_type=_F32)
        if m == 0:
            kf_s[0][0, 0:C] = spec[0:C] + d_v[...].astype(_F32).reshape(1, D)
            kf_s[0][0, C:2 * C] = spec[C:2 * C]
        else:
            kf_s[m // CPB][m % CPB] = spec

    def widen_k(r0):
        kk = k_v[r0:r0 + RW, :].astype(_F32) + jnp.tile(after_mark(), (1, ND))
        for n in range(ND):
            k_s[n, HALO + r0:HALO + r0 + RW] = kk[:, n * L:(n + 1) * L]

    def short_conv(i, p):
        r0 = i * C + p * RP
        sums = [None, None]
        for j in range(shift_v.shape[0]):
            first = HALO + r0 - 8 - 2 * (j // 2)
            kj = jnp.concatenate([k_s[base + n, first:first + RP + 8] for n in range(ND)], axis=1)
            if j % 2 == 0:
                kj = kj[8:]
            term = kj * jnp.tile(taps_s[base + j], (kj.shape[0] // 8, 1))
            sums[j % 2] = term if j < 2 else sums[j % 2] + term
        ks = sums[0] if sums[1] is None else sums[0] + pltpu.roll(sums[1], 1, 0)[8:]
        kv_s[i // CPB][1 + i % CPB, p * RP:(p + 1) * RP] = ks * v_v[r0:r0 + RP, :].astype(_F32)
        wrote(kv_s[i // CPB], 'c')

    def kv_transform(i):
        kv = kv_s[i // CPB][base + (1 + i % CPB)].astype(_BF16)
        u_s[i // CPB][i % CPB] = _dot(tied(fwd_v[...]), kv)

    def mac(b, g, n):
        chunks = range(b * CPB, (b + 1) * CPB)
        re = pl.ds(16 * g, 16)
        im = pl.ds(C + 16 * g, 16)
        ln = slice(n * L, (n + 1) * L)

        def tile(refs, i):
            return refs[i // CPB][base + i % CPB, re, ln], refs[i // CPB][base + i % CPB, im, ln]

        acc = {}
        kf = {}
        for i in range(chunks[-1] + 1):
            ur, ui = tile(u_s, i)
            for j in chunks:
                if j < i:
                    continue
                if j - i not in kf:
                    kf[j - i] = tile(kf_s, j - i)
                kr, ki = kf[j - i]
                pr, pi = kr * ur - ki * ui, kr * ui + ki * ur
                acc[j] = (acc[j][0] + pr, acc[j][1] + pi) if j in acc else (pr, pi)
        if b > 0:
            carry = carry_s[(b - 1) % 2]
            acc[chunks[0] - 1] = (carry[base, re, ln], carry[base, im, ln])
        if b + 1 < NB:
            carry_s[b % 2][0, re, ln], carry_s[b % 2][0, im, ln] = acc[chunks[-1]]
        for j in chunks:
            (ar, br), (ai, bi) = ((x[0:8], x[8:16]) for x in acc[j])
            if j > 0:
                pr, pi = acc[j - 1]
                ar, ai = ar - pi[0:8], ai + pr[0:8]
                br, bi = br + pi[8:16], bi - pr[8:16]
            for k, x in enumerate((ar + br, ai - bi, ar - br, ai + bi)):
                z_s[b][1 + j % CPB, pl.ds(k * (C // 2) + 8 * g, 8), ln] = x
        wrote(z_s[b], 'z')

    def inverse_transform(b, jj):
        for odd in range(2):
            z = z_s[b][base + (1 + jj), odd * C:(odd + 1) * C].astype(_BF16)
            y = _dot(tied(inv_v[odd * C // 4:(odd + 1) * C // 4]), z)
            for n in range(ND):
                y_s[b][n, pl.ds(jj * C + odd, C // 2, stride=2), :] = y[:, n * L:(n + 1) * L]

    def stat(k, b, rows):
        s = stat_s[k][base + (1 + b % 2), rows]
        return jnp.tile(s + after_mark() if k % 2 == 0 else s, (1, ND))

    def q_rows(b, rows):
        return q_v[b * R + rows.start:b * R + rows.stop, :].astype(_F32)

    def norm1_mean(b, rows):
        stat_s[0][1 + b % 2, rows] = _row_mean(q_rows(b, rows), after_mark())
        wrote(stat_s[0], 't')

    def norm1_scale(b, rows):
        xc = q_rows(b, rows) - stat(0, b, rows)
        stat_s[1][1 + b % 2, rows] = jax.lax.rsqrt(_row_mean(xc * xc) + EPS)
        wrote(stat_s[1], 't')

    def residual(b, rows):
        x = q_rows(b, rows)
        y = jnp.concatenate([y_s[b][base + n, rows] for n in range(ND)], axis=1)
        h = (x - stat(0, b, rows)) * stat(1, b, rows) * (mod(2) * (1.0 + mod(1))) + mod(2) * mod(0)
        x1 = x + h * y
        x1_s[b % 3, rows] = x1
        stat_s[2][1 + b % 2, rows] = _row_mean(x1)
        wrote(stat_s[2], 't')

    def norm2_scale(b, rows):
        xc = x1_s[base + b % 3, rows] - stat(2, b, rows)
        stat_s[3][1 + b % 2, rows] = jax.lax.rsqrt(_row_mean(xc * xc) + EPS)
        wrote(stat_s[3], 't')

    def norm2_apply(b, rows):
        xc = x1_s[base + b % 3, rows] - stat(2, b, rows)
        h2 = xc * stat(3, b, rows) * (1.0 + mod(4))
        h2_s[b % 2][1, rows] = h2
        wrote(h2_s[b % 2], 'h')

    def tied(words):
        if written:
            top = words[0:8, 0:L]
            for ref in written:
                top = top | pltpu.bitcast(ref[base, 0:8, 0:L], jnp.uint32)
            written.clear()
            if words.shape[1] > L:
                top = jnp.concatenate([top, words[0:8, L:]], axis=1)
            words = jnp.concatenate([top, words[8:]], axis=0)
        return pltpu.bitcast(words, _BF16)

    def weight(ref, tile, rows):
        return tied(ref.bitcast(jnp.uint32)[tile, rows.start // 2:rows.stop // 2])

    live = {}

    def ffn_gate(blocks, f):
        first = blocks[0] == 0
        if f == 0:
            h2 = jnp.concatenate([h2_s[b % 2][base + 1] for b in blocks], axis=0)
            live["h2"] = (h2 + mod(3)).astype(_BF16)
        if first and f in dict(W13_GROUPS):
            wait(*[(w, j) for j in range(f, dict(W13_GROUPS)[f]) for w in ("w1", "w3")],
                 *([("q", 2)] if f == W13_GROUPS[1][0] else []))
        live["gate"] = _dot(live["h2"], weight(w1_v, f, slice(0, D)))
        mark(live["gate"])

    def ffn_up(blocks, f):
        up = _dot(live["h2"], weight(w3_v, f, slice(0, D)))
        mark(up)
        live["act", f] = (_silu(live.pop("gate")) * up).astype(_BF16)

    def ffn_down(blocks, n, kk):
        first = blocks[0] == 0
        if first and n == 0 and kk == 0:
            wait(*[("w2", j) for j in range(ND)], ("wm", 5))
            compute_mod(5)
        act = jnp.concatenate([live["act", kk * KT + j] for j in range(KT)], axis=1)
        o = _dot(act, weight(w2_v, n, slice(kk * KT * L, (kk + 1) * KT * L)))
        mark(o)
        if kk > 0:
            o = live.pop("out") + o
        if kk + 1 < NF // KT:
            live["out"] = o
            return
        cols = slice(n * L, (n + 1) * L)
        for j, b in enumerate(blocks):
            res = x1_s[base + b % 3, :, cols] + mod(5)[:, cols] * o[j * R:(j + 1) * R]
            out_v[b * R:(b + 1) * R, cols] = res.astype(_BF16)
        if blocks[-1] + 1 == NB and n + 2 >= ND:
            send(pl.ds((NB - 1) * R, R), pl.ds(0, (ND - 1) * L) if n + 2 == ND else pl.ds(n * L, L))

    out_copies = []

    def send(rows, cols):
        cp = pltpu.make_async_copy(out_v.at[rows, cols], out_hbm.at[rows, cols],
                                   out_sems.at[len(out_copies)])
        cp.start()
        out_copies.append(cp)

    def ffn_steps(blocks):
        steps = []
        for f in range(NF):
            steps += [lambda f=f: ffn_gate(blocks, f), lambda f=f: ffn_up(blocks, f)]
        steps += [lambda n=n, kk=kk: ffn_down(blocks, n, kk)
                  for n in range(ND) for kk in range(NF // KT)]
        return steps

    def short_conv_steps(b):
        return ([(lambda r0=r0: widen_k(r0), 2 * RW * ND // 8)
                 for r0 in range(b * R, (b + 1) * R, RW)]
                + [(lambda i=i, p=p: short_conv(i, p), 9 * RP * ND // 8)
                   for i in range(b * CPB, (b + 1) * CPB) for p in range(C // RP)])

    def mac_steps(b):
        cost = sum(j + 1 for j in range(b * CPB, (b + 1) * CPB)) * 16
        return [(lambda g=g, n=n: mac(b, g, n), cost)
                for g in range(C // 16) for n in range(ND)]

    def norm_passes(b, rn=RN):
        return [[(lambda p=p, fn=fn: fn(b, slice(p * rn, (p + 1) * rn)), ops * rn * ND // 8)
                 for p in range(R // rn)]
                for fn, ops in ((norm1_mean, 2), (norm1_scale, 5), (residual, 9),
                                (norm2_scale, 4), (norm2_apply, 5))]

    def transform_steps(b):
        return [(lambda i=i, fn=fn: fn(i), 0)
                for fn in (ssm_transform, kv_transform) for i in range(b * CPB, (b + 1) * CPB)]

    def pipeline_step(*blocks):
        b = blocks[-1]
        main = ffn_steps(blocks)
        sizes = [ND] * (2 * NF) + [KT] * (len(main) - 2 * NF)
        slots = [[] for _ in main]
        if b in CONV_AT:
            for step, at in zip(transform_steps(CONV_AT[b]), XFORM_AT):
                slots[at].append(step)
        if b + 1 < NB:
            for jj in range(CPB):
                slots[INV0 + jj].append((lambda jj=jj: inverse_transform(b + 1, jj), 0))
            norm_at = NORM_FIRST if b == 1 else NORM_AT if b in MAC_AT else NORM_WIDE
            for steps, (first, stop) in zip(norm_passes(b + 1), norm_at):
                _spread(slots, steps, first, stop)
        if b + 1 in CONV_AT:
            first, stop = SC_FIRST if b == 1 else (SC0, SC1)
            if b == 1:
                for name in ("k", "v"):
                    slots[first].append((copies[name, CONV_AT[2]].wait, 0))
            _spread(slots, short_conv_steps(CONV_AT[b + 1]), first, stop)
        if b in MAC_AT:
            first, stop = MAC_FIRST if b == 1 else (XFORM_AT[-1] + MAC_LAG, len(slots))
            _fill(slots[:stop], sizes[:stop], mac_steps(MAC_AT[b]), first)
        for step, side in zip(main, slots):
            step()
            for extra, _ in side:
                extra()
        if b + 1 < NB:
            send(pl.ds(blocks[0] * R, len(blocks) * R), pl.ds(0, D))

    def run(steps):
        for step, _ in steps:
            step()

    wait("fwd", "shift", "d")
    taps = shift_v[...].astype(_F32)
    for j in range(taps.shape[0]):
        taps_s[j] = jnp.broadcast_to(taps[j:j + 1], (8, D))
    def norms(first, stop):
        for k in range(first, stop):
            for b in range(2):
                run(norm_passes(b, R)[k])

    for r in range(NPRO + 2):
        if r < NPRO:
            wait(("k", r), ("v", r), ("sk", r))
        elif r == NPRO:
            wait(("q", 0), ("q", 1), "c", "inv")
            norms(0, 2)
        else:
            wait(("wm", 0))
            for j in (1, 0, 2):
                compute_mod(j)
            norms(2, 4)
        if 1 <= r <= NPRO:
            run(transform_steps(r - 1)[CPB:])
        if r < NPRO:
            run(transform_steps(r)[:CPB] + short_conv_steps(r))
        for b in PRO_MAC.get(r, ()):
            run(mac_steps(b))
        if r == NPRO:
            for b in range(2):
                for jj in range(CPB):
                    inverse_transform(b, jj)
        written.clear()
    wait(("wm", 4))
    compute_mod(4)
    norms(4, 5)
    wait(("wm", 3))
    compute_mod(3)
    pipeline_step(0, 1)
    for b in range(2, NB):
        needs = [("q", b + 1)] if b + 1 < NB else []
        if b in CONV_AT:
            needs += [("sk", CONV_AT[b])]
        if b + 1 in CONV_AT:
            needs += [("k", CONV_AT[b + 1]), ("v", CONV_AT[b + 1])]
        wait(*needs)
        pipeline_step(b)
    for cp in out_copies:
        cp.wait()


@jax.jit
def pallas_adaLN_cond__ssm_conv_h3__glu_gated_swiglu__prompt_kernel(
    A_q: jax.Array,
    A_k: jax.Array,
    A_v: jax.Array,
    A_shift_k: jax.Array,
    A_ssm_k: jax.Array,
    A_ssm_D: jax.Array,
    B_x: jax.Array,
    B_w1: jax.Array,
    B_w3: jax.Array,
    B_w2: jax.Array,
    c: jax.Array,
    w_mod: jax.Array,
):
    del B_x
    B, S, D = A_q.shape
    FH = B_w1.shape[1]
    KS = A_shift_k.shape[1]
    assert B == 1 and S % R == 0 and FH % (KT * L) == 0 and D % L == 0 and KS <= HALO - 6
    NB, CPB = S // R, R // C
    NF, ND = FH // L, D // L
    n_in = 6 + 4 * NB + 4 + 2 * NF + ND

    hbm = pl.BlockSpec(memory_space=pl.ANY)
    out = pl.pallas_call(
        _kernel,
        out_shape=jax.ShapeDtypeStruct((S, D), A_q.dtype),
        in_specs=[hbm] * 14,
        out_specs=hbm,
        scratch_shapes=[
            pltpu.VMEM((S, D), _BF16),
            pltpu.VMEM((S, D), _BF16),
            pltpu.VMEM((S, D), _BF16),
            pltpu.VMEM((KS, D), _BF16),
            pltpu.VMEM((D, S), _BF16),
            pltpu.VMEM((D,), _BF16),
            pltpu.VMEM((NF, D, L), _BF16),
            pltpu.VMEM((NF, D, L), _BF16),
            pltpu.VMEM((ND, FH, L), _BF16),
            pltpu.VMEM((1, D), _BF16),
            pltpu.VMEM((D, 6 * D), _BF16),
            pltpu.VMEM(_FWD.shape, jnp.uint32),
            pltpu.VMEM(_INV.shape, jnp.uint32),
            pltpu.SMEM((1,), jnp.int32),
            pltpu.VMEM((KS, 8, D), _F32),
            pltpu.VMEM((ND, HALO + S, L), _F32),
            [pltpu.VMEM((CPB + 1, C, D), _F32)] * NB,
            [pltpu.VMEM((CPB, 2 * C, D), _F32)] * NB,
            [pltpu.VMEM((CPB, 2 * C, D), _F32)] * NB,
            [pltpu.VMEM((1, 2 * C, D), _F32)] * 2,
            [pltpu.VMEM((CPB + 1, 2 * C, D), _F32)] * NB,
            [pltpu.VMEM((ND, R, L), _F32)] * NB,
            pltpu.VMEM((8, 6 * D), _F32),
            [pltpu.VMEM((3, R, L), _F32)] * 4,
            [pltpu.VMEM((2, 8, L), _F32)] * 8,
            pltpu.VMEM((3, R, D), _F32),
            [pltpu.VMEM((2, R, D), _F32)] * 2,
            pltpu.VMEM((S, D), _BF16),
            pltpu.SemaphoreType.DMA((n_in,)),
            pltpu.SemaphoreType.DMA((NB,)),
        ],
        compiler_params=pltpu.CompilerParams(vmem_limit_bytes=120 * 1024 * 1024),
    )(
        A_q.reshape(S, D), A_k.reshape(S, D), A_v.reshape(S, D),
        A_shift_k.T, A_ssm_k, A_ssm_D,
        B_w1, B_w3, B_w2, c, w_mod,
        _FWD, _INV, np.zeros((1,), np.int32),
    )
    return out.reshape(B, S, D)
```

```python
import numpy as np

import jax
import jax.numpy as jnp
import jax.experimental.pallas as pl
import jax.experimental.pallas.tpu as pltpu

C = 128
R = 256
L = 128
HALO = 16
RW = 128
RP = 16
RN = 32
MAC_LAG = 3
MARK_LAG = 3
TIE = 'zc'
INV0 = 0
SC0, SC1 = 14, 24
NORM_AT = ((0, 3), (2, 5), (5, 9), (8, 11), (11, 14))
XFORM_AT = (3, 5, 11, 12)
NPRO = 4
PRO_MAC = {2: (0,), 3: (1,), 4: (2,)}
CONV_AT = {2: 4, 3: 5, 4: 6, 5: 7}
MAC_AT = {1: 3, 2: 4, 3: 5, 4: 6, 5: 7}
SC_FIRST = (25, 34)
MAC_FIRST = (0, 18)
NORM_FIRST = ((4, 8), (7, 12), (12, 17), (16, 20), (19, 24))
NORM_WIDE = ((0, 8), (6, 14), (14, 22), (21, 29), (28, 36))
W13_GROUPS = ((0, 1), (1, 3), (3, 7), (7, 12))
KT = 4
EPS = 1e-5

_F32 = jnp.float32
_BF16 = jnp.bfloat16
_NT = (((1,), (1,)), ((), ()))


def _packed_bf16(x):
    bits = np.ascontiguousarray(x, np.float32).view(np.uint32)
    bits = (bits + 0x7FFF + ((bits >> 16) & 1)) >> 16
    return bits[0::2] | (bits[1::2] << 16)


def _dft_matrices():
    even = np.arange(0, C, 2)
    f = np.stack([even.reshape(-1, 8), C - 1 - even.reshape(-1, 8)], axis=1).reshape(-1)
    step = 2.0 * np.pi / (2 * C)
    ang = step * (f[:, None] + 0.5) * np.arange(C)[None, :]
    fwd = np.concatenate([np.cos(ang), -np.sin(ang)], axis=0)
    n = np.concatenate([even, even + 1])
    ang = step * n[:, None] * (even[None, :] + 0.5)
    inv = np.concatenate([np.cos(ang), -np.sin(ang)], axis=1) / C
    return _packed_bf16(fwd), _packed_bf16(inv)


_FWD, _INV = _dft_matrices()


def _dot(a, b):
    return jnp.dot(a, b, preferred_element_type=_F32)


def _row_mean(x, zero=None):
    acc = x[:, 0:L] if zero is None else x[:, 0:L] + zero
    for n in range(1, x.shape[1] // L):
        acc = acc + x[:, n * L:(n + 1) * L]
    m = jnp.sum(acc, axis=-1, keepdims=True) * (1.0 / x.shape[1])
    return jnp.broadcast_to(m, (x.shape[0], L))


def _silu(x):
    hx = 0.5 * x
    return hx * jnp.tanh(hx) + hx


def _spread(slots, steps, first, last):
    for k, step in enumerate(steps):
        slots[first + (k * (last - first)) // len(steps)].append(step)


def _fill(slots, sizes, steps, first):
    held = [sum(cost for _, cost in slot) for slot in slots]
    rate = (sum(held[first:]) + sum(cost for _, cost in steps)) / sum(sizes[first:])
    budget, k = 0.0, 0
    for s in range(first, len(slots)):
        budget += rate * sizes[s] - held[s]
        while k < len(steps) and (budget >= 0.5 * steps[k][1] or s == len(slots) - 1):
            slots[s].append(steps[k])
            budget -= steps[k][1]
            k += 1


def _kernel(q_hbm, k_hbm, v_hbm, shift_hbm, sk_hbm, d_hbm, w1_hbm, w3_hbm, w2_hbm,
            c_hbm, wm_hbm, fwd_hbm, inv_hbm, base_hbm, out_hbm,
            q_v, k_v, v_v, shift_v, sk_v, d_v, w1_v, w3_v, w2_v, c_v, wm_v, fwd_v, inv_v, base_sm,
            taps_s, k_s, kv_s, u_s, kf_s, carry_s, z_s, y_s, mod_s, stat_s, mark_s, x1_s, h2_s, out_v,
            in_sems, out_sems):
    S, D = q_hbm.shape
    FH = w1_hbm.shape[1]
    NB = S // R
    NC = S // C
    CPB = R // C
    NF = FH // L
    ND = D // L

    copies = {}

    def start(name, src, dst):
        cp = pltpu.make_async_copy(src, dst, in_sems.at[len(copies)])
        cp.start()
        copies[name] = cp

    def start_ssm(b):
        cols = pl.ds(b * R, R)
        start(("sk", b), sk_hbm.at[:, cols], sk_v.at[:, cols])

    def start_kv(b):
        rows = pl.ds(b * R, R)
        start(("k", b), k_hbm.at[rows, :], k_v.at[rows, :])
        start(("v", b), v_hbm.at[rows, :], v_v.at[rows, :])

    def start_q(b):
        rows = pl.ds(b * R, R)
        start(("q", b), q_hbm.at[rows, :], q_v.at[rows, :])

    start("base", base_hbm, base_sm)
    start("fwd", fwd_hbm, fwd_v)
    start("shift", shift_hbm, shift_v)
    start("d", d_hbm, d_v)
    def start_mod(j, count):
        cols = pl.ds(j * D, count * D)
        start(("wm", j), wm_hbm.at[:, cols], wm_v.at[:, cols])

    for b in range(NPRO):
        start_kv(b)
        start_ssm(b)
    start_q(0)
    start_q(1)
    start("c", c_hbm, c_v)
    start("inv", inv_hbm, inv_v)
    start_mod(0, 3)
    start_mod(4, 1)
    start_mod(3, 1)
    for f in range(NF):
        start(("w1", f), w1_hbm.at[:, pl.ds(f * L, L)], w1_v.at[f])
        start(("w3", f), w3_hbm.at[:, pl.ds(f * L, L)], w3_v.at[f])
        if f + 1 == W13_GROUPS[0][1]:
            start_q(2)
    start_kv(CONV_AT[2])
    for n in range(ND):
        start(("w2", n), w2_hbm.at[:, pl.ds(n * L, L)], w2_v.at[n])
    start_mod(5, 1)
    for b in range(1, NB - 1):
        if b > 1:
            start_q(b + 1)
        if b in CONV_AT:
            start_ssm(CONV_AT[b])
        if b > 1 and b + 1 in CONV_AT:
            start_kv(CONV_AT[b + 1])

    copies["base"].wait()
    base = base_sm[0]

    def fence():
        @pl.loop(0, base + 1)
        def _(i):
            mark_s[0][1] = jnp.zeros((8, L), _F32)

    def wait(*names):
        for name in names:
            copies[name].wait()
        fence()

    for ref in (*z_s, *kv_s):
        ref[0, 0:8, 0:L] = jnp.zeros((8, L), _F32)
    for ref in stat_s:
        ref[0, 0:8] = jnp.zeros((8, L), _F32)
    for ref in h2_s:
        ref[0, 0:8, 0:L] = jnp.zeros((8, L), _F32)
    k_s[:, 0:HALO] = jnp.zeros((ND, HALO, L), _F32)

    written = []

    def wrote(ref, slot):
        if slot in TIE and not any(ref is r for r in written):
            written.append(ref)

    emitted = [0]

    def mark(result):
        mark_s[emitted[0] % len(mark_s)][1] = result[0:8, 0:L]
        emitted[0] += 1

    def after_mark(rows):
        return jnp.tile(mark_s[(emitted[0] - 1 - MARK_LAG) % len(mark_s)][base], (rows // 8, 1))

    for ref in mark_s:
        ref[0] = jnp.zeros((8, L), _F32)

    def mod(k, rows, cols=slice(0, D)):
        return jnp.tile(mod_s[k, :, cols], ((rows.stop - rows.start) // 8, 1))

    def project(j):
        sc = _silu(c_v[...].astype(_F32)).astype(_BF16)
        return _dot(jnp.broadcast_to(sc, (16, D)), wm_v[:, j * D:(j + 1) * D])[0:8]

    def ssm_transform(m):
        spec = jax.lax.dot_general(tied(fwd_v[...]), sk_v[:, m * C:(m + 1) * C], _NT,
                                   preferred_element_type=_F32)
        if m == 0:
            kf_s[0][0, 0:C] = spec[0:C] + d_v[...].astype(_F32).reshape(1, D)
            kf_s[0][0, C:2 * C] = spec[C:2 * C]
        else:
            kf_s[m // CPB][m % CPB] = spec

    def widen_k(r0):
        kk = k_v[r0:r0 + RW, :].astype(_F32) + jnp.tile(after_mark(RW), (1, ND))
        for n in range(ND):
            k_s[n, HALO + r0:HALO + r0 + RW] = kk[:, n * L:(n + 1) * L]

    def short_conv(i, p):
        r0 = i * C + p * RP
        sums = [None, None]
        for j in range(shift_v.shape[0]):
            first = HALO + r0 - 8 - 2 * (j // 2)
            kj = jnp.concatenate([k_s[base + n, first:first + RP + 8] for n in range(ND)], axis=1)
            if j % 2 == 0:
                kj = kj[8:]
            term = kj * jnp.tile(taps_s[base + j], (kj.shape[0] // 8, 1))
            sums[j % 2] = term if j < 2 else sums[j % 2] + term
        ks = sums[0] if sums[1] is None else sums[0] + pltpu.roll(sums[1], 1, 0)[8:]
        kv_s[i // CPB][1 + i % CPB, p * RP:(p + 1) * RP] = ks * v_v[r0:r0 + RP, :].astype(_F32)
        wrote(kv_s[i // CPB], 'c')

    def kv_transform(i):
        kv = kv_s[i // CPB][base + (1 + i % CPB)].astype(_BF16)
        u_s[i // CPB][i % CPB] = _dot(tied(fwd_v[...]), kv)

    def mac(b, g, n):
        chunks = range(b * CPB, (b + 1) * CPB)
        re = pl.ds(16 * g, 16)
        im = pl.ds(C + 16 * g, 16)
        ln = slice(n * L, (n + 1) * L)

        def tile(refs, i):
            return refs[i // CPB][base + i % CPB, re, ln], refs[i // CPB][base + i % CPB, im, ln]

        acc = {}
        kf = {}
        for i in range(chunks[-1] + 1):
            ur, ui = tile(u_s, i)
            for j in chunks:
                if j < i:
                    continue
                if j - i not in kf:
                    kf[j - i] = tile(kf_s, j - i)
                kr, ki = kf[j - i]
                pr, pi = kr * ur - ki * ui, kr * ui + ki * ur
                acc[j] = (acc[j][0] + pr, acc[j][1] + pi) if j in acc else (pr, pi)
        if b > 0:
            carry = carry_s[(b - 1) % 2]
            acc[chunks[0] - 1] = (carry[base, re, ln], carry[base, im, ln])
        if b + 1 < NB:
            carry_s[b % 2][0, re, ln], carry_s[b % 2][0, im, ln] = acc[chunks[-1]]
        for j in chunks:
            (ar, br), (ai, bi) = ((x[0:8], x[8:16]) for x in acc[j])
            if j > 0:
                pr, pi = acc[j - 1]
                ar, ai = ar - pi[0:8], ai + pr[0:8]
                br, bi = br + pi[8:16], bi - pr[8:16]
            for k, x in enumerate((ar + br, ai - bi, ar - br, ai + bi)):
                z_s[b][1 + j % CPB, pl.ds(k * (C // 2) + 8 * g, 8), ln] = x
        wrote(z_s[b], 'z')

    def inverse_transform(b, jj):
        for odd in range(2):
            z = z_s[b][base + (1 + jj), odd * C:(odd + 1) * C].astype(_BF16)
            y = _dot(tied(inv_v[odd * C // 4:(odd + 1) * C // 4]), z)
            for n in range(ND):
                y_s[b][n, pl.ds(jj * C + odd, C // 2, stride=2), :] = y[:, n * L:(n + 1) * L]

    def stat(k, b, rows):
        s = stat_s[k][base + (1 + b % 2), rows]
        return jnp.tile(s + after_mark(s.shape[0]) if k % 2 == 0 else s, (1, ND))

    def q_rows(b, rows):
        return q_v[b * R + rows.start:b * R + rows.stop, :].astype(_F32)

    def norm1_mean(b, rows):
        stat_s[0][1 + b % 2, rows] = _row_mean(q_rows(b, rows), after_mark(rows.stop - rows.start))
        wrote(stat_s[0], 't')

    def norm1_scale(b, rows):
        xc = q_rows(b, rows) - stat(0, b, rows)
        stat_s[1][1 + b % 2, rows] = jax.lax.rsqrt(_row_mean(xc * xc) + EPS)
        wrote(stat_s[1], 't')

    def residual(b, rows):
        x = q_rows(b, rows)
        y = jnp.concatenate([y_s[b][base + n, rows] for n in range(ND)], axis=1)
        h = (x - stat(0, b, rows)) * stat(1, b, rows) * mod(0, rows) + mod(1, rows)
        x1 = x + h * y
        x1_s[b % 3, rows] = x1
        stat_s[2][1 + b % 2, rows] = _row_mean(x1)
        wrote(stat_s[2], 't')

    def norm2_scale(b, rows):
        xc = x1_s[base + b % 3, rows] - stat(2, b, rows)
        stat_s[3][1 + b % 2, rows] = jax.lax.rsqrt(_row_mean(xc * xc) + EPS)
        wrote(stat_s[3], 't')

    def norm2_apply(b, rows):
        xc = x1_s[base + b % 3, rows] - stat(2, b, rows)
        h2 = xc * stat(3, b, rows) * mod(2, rows)
        h2_s[b % 2][1, rows] = h2
        wrote(h2_s[b % 2], 'h')

    def tied(words):
        if written:
            top = words[0:8, 0:L]
            for ref in written:
                top = top | pltpu.bitcast(ref[base, 0:8, 0:L], jnp.uint32)
            written.clear()
            if words.shape[1] > L:
                top = jnp.concatenate([top, words[0:8, L:]], axis=1)
            words = jnp.concatenate([top, words[8:]], axis=0)
        return pltpu.bitcast(words, _BF16)

    def weight(ref, tile, rows):
        return tied(ref.bitcast(jnp.uint32)[tile, rows.start // 2:rows.stop // 2])

    live = {}

    def ffn_gate(blocks, f):
        first = blocks[0] == 0
        if f == 0:
            h2 = jnp.concatenate([h2_s[b % 2][base + 1] for b in blocks], axis=0)
            live["h2"] = (h2 + mod(3, slice(0, h2.shape[0]))).astype(_BF16)
        if first and f in dict(W13_GROUPS):
            wait(*[(w, j) for j in range(f, dict(W13_GROUPS)[f]) for w in ("w1", "w3")],
                 *([("q", 2)] if f == W13_GROUPS[1][0] else []))
        live["gate"] = _dot(live["h2"], weight(w1_v, f, slice(0, D)))
        mark(live["gate"])

    def ffn_up(blocks, f):
        up = _dot(live["h2"], weight(w3_v, f, slice(0, D)))
        mark(up)
        live["act", f] = (_silu(live.pop("gate")) * up).astype(_BF16)

    def ffn_down(blocks, n, kk):
        first = blocks[0] == 0
        if first and n == 0 and kk == 0:
            wait(*[("w2", j) for j in range(ND)], ("wm", 5))
            mod_s[4] = project(5)
        act = jnp.concatenate([live["act", kk * KT + j] for j in range(KT)], axis=1)
        o = _dot(act, weight(w2_v, n, slice(kk * KT * L, (kk + 1) * KT * L)))
        mark(o)
        if kk > 0:
            o = live.pop("out") + o
        if kk + 1 < NF // KT:
            live["out"] = o
            return
        cols = slice(n * L, (n + 1) * L)
        for j, b in enumerate(blocks):
            res = x1_s[base + b % 3, :, cols] + mod(4, slice(0, R), cols) * o[j * R:(j + 1) * R]
            out_v[b * R:(b + 1) * R, cols] = res.astype(_BF16)
        if blocks[-1] + 1 == NB and n + 2 >= ND:
            send(pl.ds((NB - 1) * R, R), pl.ds(0, (ND - 1) * L) if n + 2 == ND else pl.ds(n * L, L))

    out_copies = []

    def send(rows, cols):
        cp = pltpu.make_async_copy(out_v.at[rows, cols], out_hbm.at[rows, cols],
                                   out_sems.at[len(out_copies)])
        cp.start()
        out_copies.append(cp)

    def ffn_steps(blocks):
        steps = []
        for f in range(NF):
            steps += [lambda f=f: ffn_gate(blocks, f), lambda f=f: ffn_up(blocks, f)]
        steps += [lambda n=n, kk=kk: ffn_down(blocks, n, kk)
                  for n in range(ND) for kk in range(NF // KT)]
        return steps

    def short_conv_steps(b):
        return ([(lambda r0=r0: widen_k(r0), 2 * RW * ND // 8)
                 for r0 in range(b * R, (b + 1) * R, RW)]
                + [(lambda i=i, p=p: short_conv(i, p), 9 * RP * ND // 8)
                   for i in range(b * CPB, (b + 1) * CPB) for p in range(C // RP)])

    def mac_steps(b):
        cost = sum(j + 1 for j in range(b * CPB, (b + 1) * CPB)) * 16
        return [(lambda g=g, n=n: mac(b, g, n), cost)
                for g in range(C // 16) for n in range(ND)]

    def norm_passes(b, rn=RN):
        return [[(lambda p=p, fn=fn: fn(b, slice(p * rn, (p + 1) * rn)), ops * rn * ND // 8)
                 for p in range(R // rn)]
                for fn, ops in ((norm1_mean, 2), (norm1_scale, 5), (residual, 9),
                                (norm2_scale, 4), (norm2_apply, 5))]

    def transform_steps(b):
        return [(lambda i=i, fn=fn: fn(i), 0)
                for fn in (ssm_transform, kv_transform) for i in range(b * CPB, (b + 1) * CPB)]

    def pipeline_step(*blocks):
        b = blocks[-1]
        main = ffn_steps(blocks)
        sizes = [ND] * (2 * NF) + [KT] * (len(main) - 2 * NF)
        slots = [[] for _ in main]
        if b in CONV_AT:
            for step, at in zip(transform_steps(CONV_AT[b]), XFORM_AT):
                slots[at].append(step)
        if b + 1 < NB:
            for jj in range(CPB):
                slots[INV0 + jj].append((lambda jj=jj: inverse_transform(b + 1, jj), 0))
            norm_at = NORM_FIRST if b == 1 else NORM_AT if b in MAC_AT else NORM_WIDE
            for steps, (first, stop) in zip(norm_passes(b + 1), norm_at):
                _spread(slots, steps, first, stop)
        if b + 1 in CONV_AT:
            first, stop = SC_FIRST if b == 1 else (SC0, SC1)
            if b == 1:
                for name in ("k", "v"):
                    slots[first].append((copies[name, CONV_AT[2]].wait, 0))
            _spread(slots, short_conv_steps(CONV_AT[b + 1]), first, stop)
        if b in MAC_AT:
            first, stop = MAC_FIRST if b == 1 else (XFORM_AT[-1] + MAC_LAG, len(slots))
            _fill(slots[:stop], sizes[:stop], mac_steps(MAC_AT[b]), first)
        for step, side in zip(main, slots):
            step()
            for extra, _ in side:
                extra()
        if b + 1 < NB:
            send(pl.ds(blocks[0] * R, len(blocks) * R), pl.ds(0, D))

    def run(steps):
        for step, _ in steps:
            step()

    wait("fwd", "shift", "d")
    taps = shift_v[...].astype(_F32)
    for j in range(taps.shape[0]):
        taps_s[j] = jnp.broadcast_to(taps[j:j + 1], (8, D))
    def norms(first, stop):
        for k in range(first, stop):
            for b in range(2):
                run(norm_passes(b, R)[k])

    for r in range(NPRO + 2):
        if r < NPRO:
            wait(("k", r), ("v", r), ("sk", r))
        elif r == NPRO:
            wait(("q", 0), ("q", 1), "c", "inv")
            norms(0, 2)
        else:
            wait(("wm", 0))
            gate = project(2)
            mod_s[0] = gate * (1.0 + project(1))
            mod_s[1] = gate * project(0)
            norms(2, 4)
        if 1 <= r <= NPRO:
            run(transform_steps(r - 1)[CPB:])
        if r < NPRO:
            run(transform_steps(r)[:CPB] + short_conv_steps(r))
        for b in PRO_MAC.get(r, ()):
            run(mac_steps(b))
        if r == NPRO:
            for b in range(2):
                for jj in range(CPB):
                    inverse_transform(b, jj)
        written.clear()
    wait(("wm", 4))
    mod_s[2] = 1.0 + project(4)
    norms(4, 5)
    wait(("wm", 3))
    mod_s[3] = project(3)
    pipeline_step(0, 1)
    for b in range(2, NB):
        needs = [("q", b + 1)] if b + 1 < NB else []
        if b in CONV_AT:
            needs += [("sk", CONV_AT[b])]
        if b + 1 in CONV_AT:
            needs += [("k", CONV_AT[b + 1]), ("v", CONV_AT[b + 1])]
        wait(*needs)
        pipeline_step(b)
    for cp in out_copies:
        cp.wait()


@jax.jit
def pallas_adaLN_cond__ssm_conv_h3__glu_gated_swiglu__prompt_kernel(
    A_q: jax.Array,
    A_k: jax.Array,
    A_v: jax.Array,
    A_shift_k: jax.Array,
    A_ssm_k: jax.Array,
    A_ssm_D: jax.Array,
    B_x: jax.Array,
    B_w1: jax.Array,
    B_w3: jax.Array,
    B_w2: jax.Array,
    c: jax.Array,
    w_mod: jax.Array,
):
    del B_x
    B, S, D = A_q.shape
    FH = B_w1.shape[1]
    KS = A_shift_k.shape[1]
    assert B == 1 and S % R == 0 and FH % (KT * L) == 0 and D % L == 0 and KS <= HALO - 6
    NB, CPB = S // R, R // C
    NF, ND = FH // L, D // L
    n_in = 6 + 4 * NB + 4 + 2 * NF + ND

    hbm = pl.BlockSpec(memory_space=pl.ANY)
    out = pl.pallas_call(
        _kernel,
        out_shape=jax.ShapeDtypeStruct((S, D), A_q.dtype),
        in_specs=[hbm] * 14,
        out_specs=hbm,
        scratch_shapes=[
            pltpu.VMEM((S, D), _BF16),
            pltpu.VMEM((S, D), _BF16),
            pltpu.VMEM((S, D), _BF16),
            pltpu.VMEM((KS, D), _BF16),
            pltpu.VMEM((D, S), _BF16),
            pltpu.VMEM((D,), _BF16),
            pltpu.VMEM((NF, D, L), _BF16),
            pltpu.VMEM((NF, D, L), _BF16),
            pltpu.VMEM((ND, FH, L), _BF16),
            pltpu.VMEM((1, D), _BF16),
            pltpu.VMEM((D, 6 * D), _BF16),
            pltpu.VMEM(_FWD.shape, jnp.uint32),
            pltpu.VMEM(_INV.shape, jnp.uint32),
            pltpu.SMEM((1,), jnp.int32),
            pltpu.VMEM((KS, 8, D), _F32),
            pltpu.VMEM((ND, HALO + S, L), _F32),
            [pltpu.VMEM((CPB + 1, C, D), _F32)] * NB,
            [pltpu.VMEM((CPB, 2 * C, D), _F32)] * NB,
            [pltpu.VMEM((CPB, 2 * C, D), _F32)] * NB,
            [pltpu.VMEM((1, 2 * C, D), _F32)] * 2,
            [pltpu.VMEM((CPB + 1, 2 * C, D), _F32)] * NB,
            [pltpu.VMEM((ND, R, L), _F32)] * NB,
            pltpu.VMEM((5, 8, D), _F32),
            [pltpu.VMEM((3, R, L), _F32)] * 4,
            [pltpu.VMEM((2, 8, L), _F32)] * 8,
            pltpu.VMEM((3, R, D), _F32),
            [pltpu.VMEM((2, R, D), _F32)] * 2,
            pltpu.VMEM((S, D), _BF16),
            pltpu.SemaphoreType.DMA((n_in,)),
            pltpu.SemaphoreType.DMA((NB,)),
        ],
        compiler_params=pltpu.CompilerParams(vmem_limit_bytes=120 * 1024 * 1024),
    )(
        A_q.reshape(S, D), A_k.reshape(S, D), A_v.reshape(S, D),
        A_shift_k.T, A_ssm_k, A_ssm_D,
        B_w1, B_w3, B_w2, c, w_mod,
        _FWD, _INV, np.zeros((1,), np.int32),
    )
    return out.reshape(B, S, D)
```

```python
import numpy as np

import jax
import jax.numpy as jnp
import jax.experimental.pallas as pl
import jax.experimental.pallas.tpu as pltpu

C = 128
R = 256
L = 128
KT = 4
HALO = 16
RW = 128
RP = 16
RN = 32
EPS = 1e-5

NPRO = 4
W13_GROUPS = ((0, 1), (1, 3), (3, 7), (7, 12))
XFORM_AT = (3, 5, 11, 12)
MAC_LAG = 6
MARK_LAG = 3
CONV_SLOTS, CONV_SLOTS_FIRST = (14, 24), (25, 34)
MAC_SLOTS_FIRST = (0, 18)
NORM_SLOTS = ((0, 3), (2, 5), (5, 9), (8, 11), (11, 14))
NORM_SLOTS_FIRST = ((4, 8), (7, 12), (12, 17), (16, 20), (19, 24))
NORM_SLOTS_LAST = ((0, 8), (6, 14), (14, 22), (21, 29), (28, 36))

_F32 = jnp.float32
_BF16 = jnp.bfloat16
_NT = (((1,), (1,)), ((), ()))


def _packed_bf16(x):
    bits = np.ascontiguousarray(x, np.float32).view(np.uint32)
    bits = (bits + 0x7FFF + ((bits >> 16) & 1)) >> 16
    return bits[0::2] | (bits[1::2] << 16)


def _dft_matrices():
    even = np.arange(0, C, 2)
    f = np.stack([even.reshape(-1, 8), C - 1 - even.reshape(-1, 8)], axis=1).reshape(-1)
    step = 2.0 * np.pi / (2 * C)
    ang = step * (f[:, None] + 0.5) * np.arange(C)[None, :]
    fwd = np.concatenate([np.cos(ang), -np.sin(ang)], axis=0)
    n = np.concatenate([even, even + 1])
    ang = step * n[:, None] * (even[None, :] + 0.5)
    inv = np.concatenate([np.cos(ang), -np.sin(ang)], axis=1) / C
    return _packed_bf16(fwd), _packed_bf16(inv)


_FWD, _INV = _dft_matrices()


def _dot(a, b):
    return jnp.dot(a, b, preferred_element_type=_F32)


def _row_mean(x, zero=None):
    acc = x[:, 0:L] if zero is None else x[:, 0:L] + zero
    for n in range(1, x.shape[1] // L):
        acc = acc + x[:, n * L:(n + 1) * L]
    m = jnp.sum(acc, axis=-1, keepdims=True) * (1.0 / x.shape[1])
    return jnp.broadcast_to(m, (x.shape[0], L))


def _silu(x):
    hx = 0.5 * x
    return hx * jnp.tanh(hx) + hx


def _spread(slots, steps, first, last):
    for k, step in enumerate(steps):
        slots[first + (k * (last - first)) // len(steps)].append(step)


def _fill(slots, sizes, steps, first):
    held = [sum(cost for _, cost in slot) for slot in slots]
    rate = (sum(held[first:]) + sum(cost for _, cost in steps)) / sum(sizes[first:])
    budget, k = 0.0, 0
    for s in range(first, len(slots)):
        budget += rate * sizes[s] - held[s]
        while k < len(steps) and (budget >= 0.5 * steps[k][1] or s == len(slots) - 1):
            slots[s].append(steps[k])
            budget -= steps[k][1]
            k += 1


def _kernel(q_hbm, k_hbm, v_hbm, shift_hbm, sk_hbm, d_hbm, w1_hbm, w3_hbm, w2_hbm,
            c_hbm, wm_hbm, fwd_hbm, inv_hbm, base_hbm, out_hbm,
            q_v, k_v, v_v, shift_v, sk_v, d_v, w1_v, w3_v, w2_v, c_v, wm_v, fwd_v, inv_v, base_sm,
            taps_s, k_s, kv_s, u_s, kf_s, carry_s, z_s, y_s, mod_s, stat_s, mark_s, x1_s, h2_s, out_v,
            in_sems, out_sems):
    S, D = q_hbm.shape
    FH = w1_hbm.shape[1]
    NB = S // R
    CPB = R // C
    NF = FH // L
    ND = D // L

    copies = {}

    def start(name, src, dst):
        cp = pltpu.make_async_copy(src, dst, in_sems.at[len(copies)])
        cp.start()
        copies[name] = cp

    def start_ssm(b):
        cols = pl.ds(b * R, R)
        start(("sk", b), sk_hbm.at[:, cols], sk_v.at[:, cols])

    def start_kv(b):
        rows = pl.ds(b * R, R)
        start(("k", b), k_hbm.at[rows, :], k_v.at[rows, :])
        start(("v", b), v_hbm.at[rows, :], v_v.at[rows, :])

    def start_q(b):
        rows = pl.ds(b * R, R)
        start(("q", b), q_hbm.at[rows, :], q_v.at[rows, :])

    def start_mod(j, count):
        cols = pl.ds(j * D, count * D)
        start(("wm", j), wm_hbm.at[:, cols], wm_v.at[:, cols])

    start("base", base_hbm, base_sm)
    start("fwd", fwd_hbm, fwd_v)
    start("shift", shift_hbm, shift_v)
    start("d", d_hbm, d_v)
    for b in range(NPRO):
        start_kv(b)
        start_ssm(b)
    start_q(0)
    start_q(1)
    start("c", c_hbm, c_v)
    start("inv", inv_hbm, inv_v)
    start_mod(0, 3)
    start_mod(4, 1)
    start_mod(3, 1)
    for f in range(NF):
        start(("w1", f), w1_hbm.at[:, pl.ds(f * L, L)], w1_v.at[f])
        start(("w3", f), w3_hbm.at[:, pl.ds(f * L, L)], w3_v.at[f])
        if f + 1 == W13_GROUPS[0][1]:
            start_q(2)
    start_kv(NPRO)
    for n in range(ND):
        start(("w2", n), w2_hbm.at[:, pl.ds(n * L, L)], w2_v.at[n])
    start_mod(5, 1)
    for b in range(2, NB - 1):
        start_q(b + 1)
        if b + 2 < NB:
            start_ssm(b + 2)
        if b + 3 < NB:
            start_kv(b + 3)

    def arrive(*names):
        for name in names:
            copies.pop(name).wait()

    arrive("base")
    base = base_sm[0]

    def fence():
        @pl.loop(0, base + 1)
        def _(i):
            mark_s[0][1] = jnp.zeros((8, L), _F32)

    def wait(*names):
        arrive(*names)
        fence()

    for ref in (*z_s, *kv_s):
        ref[0, 0:8, 0:L] = jnp.zeros((8, L), _F32)
    k_s[:, 0:HALO] = jnp.zeros((ND, HALO, L), _F32)

    written = []

    def wrote(ref):
        if not any(ref is r for r in written):
            written.append(ref)

    emitted = [0]

    def mark(result):
        mark_s[emitted[0] % len(mark_s)][1] = result[0:8, 0:L]
        emitted[0] += 1

    def after_mark(rows):
        return jnp.tile(mark_s[(emitted[0] - 1 - MARK_LAG) % len(mark_s)][base], (rows // 8, 1))

    for ref in mark_s:
        ref[0] = jnp.zeros((8, L), _F32)

    def mod(k, rows, cols=slice(0, D)):
        return jnp.tile(mod_s[k, :, cols], ((rows.stop - rows.start) // 8, 1))

    def project(j):
        sc = _silu(c_v[...].astype(_F32)).astype(_BF16)
        return _dot(jnp.broadcast_to(sc, (16, D)), wm_v[:, j * D:(j + 1) * D])[0:8]

    def ssm_transform(m):
        spec = jax.lax.dot_general(tied(fwd_v[...]), sk_v[:, m * C:(m + 1) * C], _NT,
                                   preferred_element_type=_F32)
        if m == 0:
            kf_s[0][0, 0:C] = spec[0:C] + d_v[...].astype(_F32).reshape(1, D)
            kf_s[0][0, C:2 * C] = spec[C:2 * C]
        else:
            kf_s[m // CPB][m % CPB] = spec

    def widen_k(r0):
        kk = k_v[r0:r0 + RW, :].astype(_F32) + jnp.tile(after_mark(RW), (1, ND))
        for n in range(ND):
            k_s[n, HALO + r0:HALO + r0 + RW] = kk[:, n * L:(n + 1) * L]

    def short_conv(i, p):
        r0 = i * C + p * RP
        sums = [None, None]
        for j in range(shift_v.shape[0]):
            first = HALO + r0 - 8 - 2 * (j // 2)
            kj = jnp.concatenate([k_s[base + n, first:first + RP + 8] for n in range(ND)], axis=1)
            if j % 2 == 0:
                kj = kj[8:]
            term = kj * jnp.tile(taps_s[base + j], (kj.shape[0] // 8, 1))
            sums[j % 2] = term if j < 2 else sums[j % 2] + term
        ks = sums[0] if sums[1] is None else sums[0] + pltpu.roll(sums[1], 1, 0)[8:]
        kv_s[i // CPB][1 + i % CPB, p * RP:(p + 1) * RP] = ks * v_v[r0:r0 + RP, :].astype(_F32)
        wrote(kv_s[i // CPB])

    def kv_transform(i):
        kv = kv_s[i // CPB][base + (1 + i % CPB)].astype(_BF16)
        u_s[i // CPB][i % CPB] = _dot(tied(fwd_v[...]), kv)

    def mac(b, g, n):
        chunks = range(b * CPB, (b + 1) * CPB)
        re = pl.ds(16 * g, 16)
        im = pl.ds(C + 16 * g, 16)
        ln = slice(n * L, (n + 1) * L)

        def tile(refs, i):
            return refs[i // CPB][base + i % CPB, re, ln], refs[i // CPB][base + i % CPB, im, ln]

        acc = {}
        kf = {}
        for i in range(chunks[-1] + 1):
            ur, ui = tile(u_s, i)
            for j in chunks:
                if j < i:
                    continue
                if j - i not in kf:
                    kf[j - i] = tile(kf_s, j - i)
                kr, ki = kf[j - i]
                pr, pi = kr * ur - ki * ui, kr * ui + ki * ur
                acc[j] = (acc[j][0] + pr, acc[j][1] + pi) if j in acc else (pr, pi)
        if b > 0:
            carry = carry_s[(b - 1) % 2]
            acc[chunks[0] - 1] = (carry[base, re, ln], carry[base, im, ln])
        if b + 1 < NB:
            carry_s[b % 2][0, re, ln], carry_s[b % 2][0, im, ln] = acc[chunks[-1]]
        for j in chunks:
            (ar, br), (ai, bi) = ((x[0:8], x[8:16]) for x in acc[j])
            if j > 0:
                pr, pi = acc[j - 1]
                ar, ai = ar - pi[0:8], ai + pr[0:8]
                br, bi = br + pi[8:16], bi - pr[8:16]
            for k, x in enumerate((ar + br, ai - bi, ar - br, ai + bi)):
                z_s[b][1 + j % CPB, pl.ds(k * (C // 2) + 8 * g, 8), ln] = x
        wrote(z_s[b])

    def inverse_transform(b, jj):
        for odd in range(2):
            z = z_s[b][base + (1 + jj), odd * C:(odd + 1) * C].astype(_BF16)
            y = _dot(tied(inv_v[odd * C // 4:(odd + 1) * C // 4]), z)
            for n in range(ND):
                y_s[b][n, pl.ds(jj * C + odd, C // 2, stride=2), :] = y[:, n * L:(n + 1) * L]

    def stat(k, b, rows):
        s = stat_s[k][base + b % 2, rows]
        return jnp.tile(s + after_mark(s.shape[0]) if k % 2 == 0 else s, (1, ND))

    def q_rows(b, rows):
        return q_v[b * R + rows.start:b * R + rows.stop, :].astype(_F32)

    def norm1_mean(b, rows):
        stat_s[0][b % 2, rows] = _row_mean(q_rows(b, rows), after_mark(rows.stop - rows.start))

    def norm1_scale(b, rows):
        xc = q_rows(b, rows) - stat(0, b, rows)
        stat_s[1][b % 2, rows] = jax.lax.rsqrt(_row_mean(xc * xc) + EPS)

    def residual(b, rows):
        x = q_rows(b, rows)
        y = jnp.concatenate([y_s[b][base + n, rows] for n in range(ND)], axis=1)
        h = (x - stat(0, b, rows)) * stat(1, b, rows) * mod(0, rows) + mod(1, rows)
        x1 = x + h * y
        x1_s[b % 3, rows] = x1
        stat_s[2][b % 2, rows] = _row_mean(x1)

    def norm2_scale(b, rows):
        xc = x1_s[base + b % 3, rows] - stat(2, b, rows)
        stat_s[3][b % 2, rows] = jax.lax.rsqrt(_row_mean(xc * xc) + EPS)

    def norm2_apply(b, rows):
        xc = x1_s[base + b % 3, rows] - stat(2, b, rows)
        h2 = xc * stat(3, b, rows) * mod(2, rows)
        h2_s[b % 2][0, rows] = h2

    def tied(words):
        if written:
            top = words[0:8, 0:L]
            for ref in written:
                top = top | pltpu.bitcast(ref[base, 0:8, 0:L], jnp.uint32)
            written.clear()
            if words.shape[1] > L:
                top = jnp.concatenate([top, words[0:8, L:]], axis=1)
            words = jnp.concatenate([top, words[8:]], axis=0)
        return pltpu.bitcast(words, _BF16)

    def weight(ref, tile, rows):
        return tied(ref.bitcast(jnp.uint32)[tile, rows.start // 2:rows.stop // 2])

    live = {}

    def ffn_gate(blocks, f):
        first = blocks[0] == 0
        if f == 0:
            h2 = jnp.concatenate([h2_s[b % 2][base] for b in blocks], axis=0)
            live["h2"] = (h2 + mod(3, slice(0, h2.shape[0]))).astype(_BF16)
        if first and f in dict(W13_GROUPS):
            wait(*[(w, j) for j in range(f, dict(W13_GROUPS)[f]) for w in ("w1", "w3")],
                 *([("q", 2)] if f == W13_GROUPS[1][0] else []))
        live["gate"] = _dot(live["h2"], weight(w1_v, f, slice(0, D)))
        mark(live["gate"])

    def ffn_up(blocks, f):
        up = _dot(live["h2"], weight(w3_v, f, slice(0, D)))
        mark(up)
        live["act", f] = (_silu(live.pop("gate")) * up).astype(_BF16)

    def ffn_down(blocks, n, kk):
        first = blocks[0] == 0
        if first and n == 0 and kk == 0:
            wait(*[("w2", j) for j in range(ND)], ("wm", 5))
            mod_s[4] = project(5)
        act = jnp.concatenate([live["act", kk * KT + j] for j in range(KT)], axis=1)
        o = _dot(act, weight(w2_v, n, slice(kk * KT * L, (kk + 1) * KT * L)))
        mark(o)
        if kk > 0:
            o = live.pop("out") + o
        if kk + 1 < NF // KT:
            live["out"] = o
            return
        cols = slice(n * L, (n + 1) * L)
        for j, b in enumerate(blocks):
            res = x1_s[base + b % 3, :, cols] + mod(4, slice(0, R), cols) * o[j * R:(j + 1) * R]
            out_v[b * R:(b + 1) * R, cols] = res.astype(_BF16)
        if blocks[-1] + 1 == NB and n + 2 >= ND:
            send(pl.ds((NB - 1) * R, R), pl.ds(0, (ND - 1) * L) if n + 2 == ND else pl.ds(n * L, L))

    out_copies = []

    def send(rows, cols):
        cp = pltpu.make_async_copy(out_v.at[rows, cols], out_hbm.at[rows, cols],
                                   out_sems.at[len(out_copies)])
        cp.start()
        out_copies.append(cp)

    def ffn_steps(blocks):
        steps = []
        for f in range(NF):
            steps += [lambda f=f: ffn_gate(blocks, f), lambda f=f: ffn_up(blocks, f)]
        steps += [lambda n=n, kk=kk: ffn_down(blocks, n, kk)
                  for n in range(ND) for kk in range(NF // KT)]
        return steps

    def short_conv_steps(b):
        return ([(lambda r0=r0: widen_k(r0), 2 * RW * ND // 8)
                 for r0 in range(b * R, (b + 1) * R, RW)]
                + [(lambda i=i, p=p: short_conv(i, p), 9 * RP * ND // 8)
                   for i in range(b * CPB, (b + 1) * CPB) for p in range(C // RP)])

    def mac_steps(b):
        cost = sum(j + 1 for j in range(b * CPB, (b + 1) * CPB)) * 16
        return [(lambda g=g, n=n: mac(b, g, n), cost)
                for g in range(C // 16) for n in range(ND)]

    def norm_passes(b, rn=RN):
        return [[(lambda p=p, fn=fn: fn(b, slice(p * rn, (p + 1) * rn)), ops * rn * ND // 8)
                 for p in range(R // rn)]
                for fn, ops in ((norm1_mean, 2), (norm1_scale, 5), (residual, 9),
                                (norm2_scale, 4), (norm2_apply, 5))]

    def transform_steps(b):
        return [(lambda i=i, fn=fn: fn(i), 0)
                for fn in (ssm_transform, kv_transform) for i in range(b * CPB, (b + 1) * CPB)]

    def pipeline_step(*blocks):
        b = blocks[-1]
        main = ffn_steps(blocks)
        sizes = [ND] * (2 * NF) + [KT] * (len(main) - 2 * NF)
        slots = [[] for _ in main]
        first = blocks[0] == 0
        if NPRO <= b + 2 < NB:
            for step, at in zip(transform_steps(b + 2), XFORM_AT):
                slots[at].append(step)
        if b + 1 < NB:
            for jj in range(CPB):
                slots[jj].append((lambda jj=jj: inverse_transform(b + 1, jj), 0))
            spans = NORM_SLOTS_FIRST if first else NORM_SLOTS if b + 2 < NB else NORM_SLOTS_LAST
            for steps, span in zip(norm_passes(b + 1), spans):
                _spread(slots, steps, *span)
        if NPRO <= b + 3 < NB:
            span = CONV_SLOTS_FIRST if first else CONV_SLOTS
            if first:
                slots[span[0]].append((lambda: arrive(("k", b + 3), ("v", b + 3)), 0))
            _spread(slots, short_conv_steps(b + 3), *span)
        if b + 2 < NB:
            lo, hi = MAC_SLOTS_FIRST if first else (XFORM_AT[-1] + MAC_LAG, len(slots))
            _fill(slots[:hi], sizes[:hi], mac_steps(b + 2), lo)
        for step, side in zip(main, slots):
            step()
            for extra, _ in side:
                extra()
        if b + 1 < NB:
            send(pl.ds(blocks[0] * R, len(blocks) * R), pl.ds(0, D))

    def run(steps):
        for step, _ in steps:
            step()

    wait("fwd", "shift", "d")
    taps = shift_v[...].astype(_F32)
    for j in range(taps.shape[0]):
        taps_s[j] = jnp.broadcast_to(taps[j:j + 1], (8, D))
    def norms(first, stop):
        for k in range(first, stop):
            for b in range(2):
                run(norm_passes(b, R)[k])

    for r in range(NPRO + 2):
        if r < NPRO:
            wait(("k", r), ("v", r), ("sk", r))
        elif r == NPRO:
            wait(("q", 0), ("q", 1), "c", "inv")
            norms(0, 2)
        else:
            wait(("wm", 0))
            gate = project(2)
            mod_s[0] = gate * (1.0 + project(1))
            mod_s[1] = gate * project(0)
            norms(2, 4)
        if 1 <= r <= NPRO:
            run(transform_steps(r - 1)[CPB:])
        if r < NPRO:
            run(transform_steps(r)[:CPB] + short_conv_steps(r))
        if 2 <= r <= NPRO:
            run(mac_steps(r - 2))
        if r == NPRO:
            for b in range(2):
                for jj in range(CPB):
                    inverse_transform(b, jj)
        written.clear()
    wait(("wm", 4))
    mod_s[2] = 1.0 + project(4)
    norms(4, 5)
    wait(("wm", 3))
    mod_s[3] = project(3)
    pipeline_step(0, 1)
    for b in range(2, NB):
        wait(*[name for name in (("q", b + 1), ("sk", b + 2), ("k", b + 3), ("v", b + 3))
               if name in copies])
        pipeline_step(b)
    assert not copies, copies
    for cp in out_copies:
        cp.wait()


@jax.jit
def pallas_adaLN_cond__ssm_conv_h3__glu_gated_swiglu__prompt_kernel(
    A_q: jax.Array,
    A_k: jax.Array,
    A_v: jax.Array,
    A_shift_k: jax.Array,
    A_ssm_k: jax.Array,
    A_ssm_D: jax.Array,
    B_x: jax.Array,
    B_w1: jax.Array,
    B_w3: jax.Array,
    B_w2: jax.Array,
    c: jax.Array,
    w_mod: jax.Array,
):
    del B_x
    B, S, D = A_q.shape
    FH = B_w1.shape[1]
    KS = A_shift_k.shape[1]
    assert B == 1 and S == 8 * R and FH == W13_GROUPS[-1][1] * L and D % L == 0 and KS <= HALO - 6
    NB, CPB = S // R, R // C
    NF, ND = FH // L, D // L
    n_in = 6 + 4 * NB + 4 + 2 * NF + ND

    hbm = pl.BlockSpec(memory_space=pl.ANY)
    out = pl.pallas_call(
        _kernel,
        out_shape=jax.ShapeDtypeStruct((S, D), A_q.dtype),
        in_specs=[hbm] * 14,
        out_specs=hbm,
        scratch_shapes=[
            pltpu.VMEM((S, D), _BF16),
            pltpu.VMEM((S, D), _BF16),
            pltpu.VMEM((S, D), _BF16),
            pltpu.VMEM((KS, D), _BF16),
            pltpu.VMEM((D, S), _BF16),
            pltpu.VMEM((D,), _BF16),
            pltpu.VMEM((NF, D, L), _BF16),
            pltpu.VMEM((NF, D, L), _BF16),
            pltpu.VMEM((ND, FH, L), _BF16),
            pltpu.VMEM((1, D), _BF16),
            pltpu.VMEM((D, 6 * D), _BF16),
            pltpu.VMEM(_FWD.shape, jnp.uint32),
            pltpu.VMEM(_INV.shape, jnp.uint32),
            pltpu.SMEM((1,), jnp.int32),
            pltpu.VMEM((KS, 8, D), _F32),
            pltpu.VMEM((ND, HALO + S, L), _F32),
            [pltpu.VMEM((CPB + 1, C, D), _F32)] * NB,
            [pltpu.VMEM((CPB, 2 * C, D), _F32)] * NB,
            [pltpu.VMEM((CPB, 2 * C, D), _F32)] * NB,
            [pltpu.VMEM((1, 2 * C, D), _F32)] * 2,
            [pltpu.VMEM((CPB + 1, 2 * C, D), _F32)] * NB,
            [pltpu.VMEM((ND, R + 8, L), _F32)] * NB,
            pltpu.VMEM((5, 8, D), _F32),
            [pltpu.VMEM((2, R, L), _F32)] * 4,
            [pltpu.VMEM((2, 8, L), _F32)] * 8,
            pltpu.VMEM((3, R, D), _F32),
            [pltpu.VMEM((1, R, D), _F32)] * 2,
            pltpu.VMEM((S, D), _BF16),
            pltpu.SemaphoreType.DMA((n_in,)),
            pltpu.SemaphoreType.DMA((NB,)),
        ],
        compiler_params=pltpu.CompilerParams(vmem_limit_bytes=120 * 1024 * 1024),
    )(
        A_q.reshape(S, D), A_k.reshape(S, D), A_v.reshape(S, D),
        A_shift_k.T, A_ssm_k, A_ssm_D,
        B_w1, B_w3, B_w2, c, w_mod,
        _FWD, _INV, np.zeros((1,), np.int32),
    )
    return out.reshape(B, S, D)
```
